```python
import jax
import jax.numpy as jnp

def _softmax(x, axis=-1):
    return jax.nn.softmax(x, axis=axis)
def _gelu(x):
    return jax.nn.gelu(x, approximate=True)
def _silu(x):
    return jax.nn.silu(x)
def _sigmoid(x):
    return jax.nn.sigmoid(x)
def _layernorm(x, axis=-1, eps=1e-5):
    m = jnp.mean(x, axis=axis, keepdims=True)
    v = jnp.var(x, axis=axis, keepdims=True)
    return (x - m) / jnp.sqrt(v + eps)
def _scatter_add(tgt, idx, src, axis=0):
    return tgt.at[idx].add(src)
def _segment_sum(src, seg, n):
    return jax.ops.segment_sum(src, seg, n)
class _Rng:
    def __init__(self, key):
        self._k = key
    def _next(self):
        self._k, sub = jax.random.split(self._k)
        return sub
    def normal(self, shape):
        return jax.random.normal(self._next(), shape, dtype=jnp.bfloat16)
    def randint(self, lo, hi, shape):
        return jax.random.randint(self._next(), shape, lo, hi, dtype=jnp.int32)
    def uniform(self, shape, lo=0.0, hi=1.0):
        return jax.random.uniform(self._next(), shape, jnp.bfloat16, lo, hi)
    def permutation(self, n):
        return jax.random.permutation(self._next(), n)


kernel_name = 'concat_heads__ssm_conv_s5__ssm_conv_h3__prompt'

def setup_inputs():
    _rng = _Rng(jax.random.key(int.from_bytes(__import__("os").urandom(4), "little")))
    _w = (lambda a: (lambda t: t.astype(jnp.bfloat16) if jnp.issubdtype(t.dtype, jnp.floating) else t)(jnp.asarray(a)))
    def _A_setup():
        B, S, D = 1, 2048, 640
        P = D
        Lambda_re = -0.5 * jnp.exp((lambda *s: _rng.normal(s) * 0.05)(P))
        Lambda_im = (lambda *s: _rng.normal(s) * 0.05)(P) * 1.0
        B_re = (lambda *s: _rng.normal(s) * 0.05)(P, D) * (D ** -0.5)
        B_im = (lambda *s: _rng.normal(s) * 0.05)(P, D) * (D ** -0.5)
        C_re = (lambda *s: _rng.normal(s) * 0.05)(D, P) * (P ** -0.5)
        C_im = (lambda *s: _rng.normal(s) * 0.05)(D, P) * (P ** -0.5)
        log_dt = (lambda *s: _rng.normal(s) * 0.05)(P) * 0.3 - 2.0
        Dskip = (lambda *s: _rng.normal(s) * 0.05)(D)
        return {
            "x": _w((lambda *s: _rng.normal(s) * 0.05)(B, S, D)),
            "Lambda_re": _w(Lambda_re),
            "Lambda_im": _w(Lambda_im),
            "B_re": _w(B_re),
            "B_im": _w(B_im),
            "C_re": _w(C_re),
            "C_im": _w(C_im),
            "log_dt": _w(log_dt),
            "Dskip": _w(Dskip),
        }
    _A_in = _A_setup()

    def _B_setup():
        B, S, D = 1, 2048, 640
        ks = 4
        return {
            "q": _w((lambda *s: _rng.normal(s) * 0.05)(B, S, D)),
            "k": _w((lambda *s: _rng.normal(s) * 0.05)(B, S, D)),
            "v": _w((lambda *s: _rng.normal(s) * 0.05)(B, S, D)),
            "shift_k": _w((lambda *s: _rng.normal(s) * 0.05)(D, ks) * 0.5),
            "ssm_k": _w((lambda *s: _rng.normal(s) * 0.05)(D, S) * (1.0 / S ** 0.5)),
            "ssm_D": _w((lambda *s: _rng.normal(s) * 0.05)(D)),
        }
    _B_in = _B_setup()

    return {
        "A_x": _A_in["x"],
        "A_Lambda_re": _A_in["Lambda_re"],
        "A_Lambda_im": _A_in["Lambda_im"],
        "A_B_re": _A_in["B_re"],
        "A_B_im": _A_in["B_im"],
        "A_C_re": _A_in["C_re"],
        "A_C_im": _A_in["C_im"],
        "A_log_dt": _A_in["log_dt"],
        "A_Dskip": _A_in["Dskip"],
        "B_q": _B_in["q"],
        "B_k": _B_in["k"],
        "B_v": _B_in["v"],
        "B_shift_k": _B_in["shift_k"],
        "B_ssm_k": _B_in["ssm_k"],
        "B_ssm_D": _B_in["ssm_D"],
    }

def reference(A_x, A_Lambda_re, A_Lambda_im, A_B_re, A_B_im, A_C_re, A_C_im, A_log_dt, A_Dskip, B_q, B_k, B_v, B_shift_k, B_ssm_k, B_ssm_D):
    def _A_ref(x, Lambda_re, Lambda_im, B_re, B_im, C_re, C_im, log_dt, Dskip):
        Bsz, L, H = x.shape
        Lam = Lambda_re + 1j * Lambda_im
        Bmat = B_re + 1j * B_im
        Cmat = C_re + 1j * C_im
        dt = jnp.exp(log_dt)
        Lam_bar = jnp.exp(dt * Lam)
        B_bar = ((Lam_bar - 1.0) / Lam)[:, None] * Bmat
        Bu = jnp.einsum("bld,pd->blp", x + 0j, B_bar)
        h = jnp.zeros_like(Bu[:, 0, :])
        hs = []
        for t in range(L):
            h = Lam_bar[None, :] * h + Bu[:, t, :]
            hs.append(h)
        hseq = jnp.stack(hs, 1)
        y = 2.0 * jnp.einsum("blp,dp->bld", hseq, Cmat).real + x * Dskip[None, None, :]
        return y

    def _B_ref(q, k, v, shift_k, ssm_k, ssm_D):
        B, S, D = q.shape
        ks = shift_k.shape[-1]
        k_pad = jnp.pad(k, ((0, 0), (ks - 1, 0), (0, 0)))
        k_shift = jnp.zeros_like(k)
        for t in range(ks):
            k_shift = k_shift + k_pad[:, t:t + S, :] * shift_k[:, ks - 1 - t][None, None, :]
        kv = k_shift * v
        L = 2 * S
        kv_pad = jnp.pad(kv, ((0, 0), (0, S), (0, 0)))
        kf_pad = jnp.pad(ssm_k, ((0, 0), (0, S)))
        kv_f = (lambda x, axes=(-2,-1): jnp.fft.rfft2(x.astype(jnp.float32), axes=axes))(kv_pad[:, None, :, :], axes=(1, 2))
        kf_f = (lambda x, axes=(-2,-1): jnp.fft.rfft2(x.astype(jnp.float32), axes=axes))(kf_pad[:, None, :], axes=(1, 2))
        kf_f = (lambda x, *d: x.transpose(*d))(kf_f, 1, 2, 0)
        y_f = kv_f * kf_f[None, :, :, :]
        y = (lambda x, s, axes=(-2,-1): jnp.fft.irfft2(x, s=s, axes=axes).astype(jnp.bfloat16))(y_f, (1, L), axes=(1, 2))[:, 0, :S, :]
        y = y + kv * ssm_D[None, None, :]
        return q * y

    a = _A_ref(A_x, A_Lambda_re, A_Lambda_im, A_B_re, A_B_im, A_C_re, A_C_im, A_log_dt, A_Dskip)
    b = _B_ref(B_q, B_k, B_v, B_shift_k, B_ssm_k, B_ssm_D)
    return jnp.concatenate([a, b], axis=-1)
```

```python
import numpy as np
import jax
import jax.numpy as jnp
from jax import lax
import jax.experimental.pallas as pl
import jax.experimental.pallas.tpu as pltpu

S, D = 2048, 640
T = 512
NP, NJ = 4, 5
HALO = 16
F32, BF16, U32 = jnp.float32, jnp.bfloat16, jnp.uint32
NT = (((1,), (1,)), ((), ()))


def _dft_tables():
    g = np.arange(128)[:, None]
    m = np.arange(128)[None, :]
    fwd = np.zeros((4, 256, 128), np.float64)
    for r in range(4):
        th = np.pi * (((4 * g + 1) * (4 * m + r)) % 2048) / 1024.0
        c = np.cos(th).reshape(16, 8, 128)
        s = np.sin(th).reshape(16, 8, 128)
        fwd[r] = np.stack([c, s], axis=1).reshape(256, 128)
    inv = np.transpose(fwd, (0, 2, 1)) / 512.0
    return fwd.astype(jnp.bfloat16), np.ascontiguousarray(inv).astype(jnp.bfloat16)


def _lo(w):
    return pltpu.bitcast(w << 16, F32)


def _hi(w):
    return pltpu.bitcast(w & jnp.uint32(0xFFFF0000), F32)


def _cmul(a, b):
    return a[0] * b[0] - a[1] * b[1], a[0] * b[1] + a[1] * b[0]


def _cadd(a, b):
    return a[0] + b[0], a[1] + b[1]


def _csub(a, b):
    return a[0] - b[0], a[1] - b[1]


def _kernel(x_hbm, lre_hbm, lim_hbm, bre_hbm, bim_hbm, cre_hbm, cim_hbm, ldt_hbm, dsk_hbm,
            q_hbm, k_hbm, v_hbm, sh_hbm, ssm_hbm, sd_hbm, f_hbm, g_hbm,
            o_hbm,
            xs, ks, vs, qs, ssm, bre, bim, cre, cim, cp, hb,
            lre_v, lim_v, ldt_v, dsk_v, sd_v, sh_v, f_v, g_v,
            lamtab, fvec, rowp, bu0, bu1, kv0, kv1, kt0, kt1, kraw,
            uh, kh, y0, y1, oa, ob, sem):
    nsem = [0]
    pending = {}

    def start(name, src, dst):
        c = pltpu.make_async_copy(src, dst, sem.at[nsem[0]])
        nsem[0] += 1
        c.start()
        pending[name] = c

    def wait(*names):
        for n in names:
            pending.pop(n).wait()

    def cols(j):
        return pl.ds(128 * j, 128)

    def rows(p):
        return pl.ds(T * p, T)

    for n, s_, d_ in (("lre", lre_hbm, lre_v), ("lim", lim_hbm, lim_v), ("ldt", ldt_hbm, ldt_v)):
        start(n, s_, d_)
    start(("b", 0, 0), bre_hbm.at[cols(0), :], bre.at[cols(0), :])
    start(("b", 0, 1), bim_hbm.at[cols(0), :], bim.at[cols(0), :])
    for j in range(NJ):
        start(("x", 0, j), x_hbm.at[rows(0), cols(j)], xs.at[j, rows(0), :])
    for j in range(1, NJ):
        start(("b", j, 0), bre_hbm.at[cols(j), :], bre.at[cols(j), :])
        start(("b", j, 1), bim_hbm.at[cols(j), :], bim.at[cols(j), :])
    for n, s_, d_ in (("dsk", dsk_hbm, dsk_v), ("sd", sd_hbm, sd_v), ("sh", sh_hbm, sh_v), ("f", f_hbm, f_v)):
        start(n, s_, d_)

    def start_b(j):
        start(("k", j), k_hbm.at[:, cols(j)], ks.at[j, pl.ds(HALO, S), :])
        start(("v", j), v_hbm.at[:, cols(j)], vs.at[j])
        start(("ssm", j), ssm_hbm.at[cols(j), :], ssm.at[cols(j), :])

    def start_x(p):
        for j in range(NJ):
            start(("x", p, j), x_hbm.at[rows(p), cols(j)], xs.at[j, rows(p), :])

    start_b(0)
    start_x(1)
    start_b(1)
    start_x(2)
    start_b(2)
    start_x(3)
    start_b(3)
    start("cre", cre_hbm, cre)
    start("cim", cim_hbm, cim)
    start_b(4)
    start("g", g_hbm, g_v)
    for j in range(NJ):
        start(("q", j), q_hbm.at[:, cols(j)], qs.at[j])

    for j in range(NJ):
        ks[j, pl.ds(0, HALO), :] = jnp.zeros((HALO, 128), BF16)

    wait("lre", "lim", "ldt")

    def bcast(ref):
        return jnp.broadcast_to(ref[...].astype(F32).reshape(1, D), (8, D))

    lr, li = bcast(lre_v), bcast(lim_v)
    dt = jnp.exp(bcast(ldt_v)).astype(BF16).astype(F32)
    mag = jnp.exp(dt * lr)
    lam = (mag * jnp.cos(dt * li), mag * jnp.sin(dt * li))
    nr, ni = lam[0] - 1.0, lam[1]
    big = jnp.abs(lr) >= jnp.abs(li)
    ratio = jnp.where(big, li / lr, lr / li)
    den = jnp.where(big, lr + li * ratio, li + lr * ratio)
    fr = jnp.where(big, nr + ni * ratio, nr * ratio + ni) / den
    fi = jnp.where(big, ni - nr * ratio, ni * ratio - nr) / den
    fvec[0] = 2.0 * fr
    fvec[1] = 2.0 * fi
    pw = [lam]
    for i in range(1, 8):
        pw.append(_cmul(pw[(i - 1) // 2], pw[i - 1 - (i - 1) // 2]))
    mu1 = pw[7]
    mu2 = _cmul(mu1, mu1)
    mu4 = _cmul(mu2, mu2)
    sub = lax.broadcasted_iota(jnp.int32, (8, D), 0)
    tab = [c for z in pw for c in z]
    for d_, mu in ((1, mu1), (2, mu2), (4, mu4)):
        tab += [jnp.where(sub >= d_, mu[0], 0.0), jnp.where(sub >= d_, mu[1], 0.0)]
    for j in range(NJ):
        for i, t_ in enumerate(tab):
            lamtab[j, i] = t_[:, 128 * j:128 * (j + 1)]

    xw = xs.bitcast(U32)
    kw = ks.bitcast(U32)
    vw = vs.bitcast(U32)
    qw = qs.bitcast(U32)
    krw = kraw.bitcast(U32)

    def xvreg(p, j, b, m):
        return xw[j, pl.ds(T // 2 * p + 32 * b + m, 8, stride=4), :]

    def a1(p, j, bu):
        lhs = jnp.concatenate([
            pltpu.bitcast(jnp.concatenate([xvreg(p, jj, b, m) for b in range(T // 64) for m in range(4)], axis=0), BF16)
            for jj in range(NJ)], axis=1)
        rhs = jnp.concatenate([bre[cols(j), :], bim[cols(j), :]], axis=0)
        r = lax.dot_general(lhs, rhs, NT, preferred_element_type=F32)
        bu[0] = r[:, :128]
        bu[1] = r[:, 128:]

    sub1 = lax.broadcasted_iota(jnp.int32, (8, 128), 0)

    def scan(p, j, bu, last):
        def tb(i):
            return lamtab[j, 2 * i], lamtab[j, 2 * i + 1]
        for b in range(T // 64):
            hs = []
            for i in range(8):
                st = pl.ds(64 * b + 16 * (i // 2) + (i % 2), 8, stride=2)
                u = (bu[0, st, :], bu[1, st, :])
                hs.append(u if i == 0 else _cadd(_cmul(tb(0), hs[-1]), u))
            if last is None:
                e = tuple(jnp.where(sub1 == 7, 0.0, c) for c in hs[7])
            else:
                e = tuple(jnp.where(sub1 == 7, l_, c) for l_, c in zip(last, hs[7]))
            e = tuple(pltpu.roll(c, 1, 0) for c in e)
            for n, d_ in enumerate((1, 2, 4)):
                e = _cadd(e, _cmul(tb(8 + n), tuple(pltpu.roll(c, d_, 0) for c in e)))
            hs = [_cadd(hs[i], _cmul(tb(i), e)) for i in range(8)]
            last = hs[7]
            for c in range(2):
                for i in range(0, 8, 2):
                    hb[pl.ds(T * p + 64 * b + 8 * i, 16), cols(2 * j + c)] = (
                        jnp.concatenate([hs[i][c], hs[i + 1][c]], axis=0).astype(BF16))
        return last

    def fold_c(i):
        for j in range(NJ):
            fr_, fi_ = fvec[0, 0:1, cols(j)], fvec[1, 0:1, cols(j)]
            a = cre[cols(i), cols(j)].astype(F32)
            b = cim[cols(i), cols(j)].astype(F32)
            cp[cols(i), cols(2 * j)] = (a * fr_ - b * fi_).astype(BF16)
            cp[cols(i), cols(2 * j + 1)] = (-(a * fi_) - b * fr_).astype(BF16)

    def a2(p, j):
        y = lax.dot_general(hb[rows(p), :], cp[cols(j), :], NT, preferred_element_type=F32)
        dsk = rowp[0, :, cols(j)]
        for b in range(T // 64):
            for m in range(4):
                w = xvreg(p, j, b, m)
                for e, xv in enumerate((_lo(w), _hi(w))):
                    i = 2 * m + e
                    r0 = 64 * b + 8 * i
                    oa[j, pl.ds(T * p + 64 * b + i, 8, stride=8), :] = y[r0:r0 + 8] + xv * dsk
        start(("oa", p, j), oa.at[j, rows(p), :], o_hbm.at[rows(p), cols(j)])

    def bprep(j, p, kv, kt):
        w = [rowp[2 + i, :, cols(j)] for i in range(4)]
        for mb in range(8):
            outs = [[] for _ in range(4)]
            for hf in range(2):
                m0 = 16 * mb + 8 * hf
                base = HALO // 2 + T // 2 * p + 2 * m0
                w0 = kw[j, pl.ds(base, 8, stride=2), :]
                w1 = kw[j, pl.ds(base + 1, 8, stride=2), :]
                p0 = kw[j, pl.ds(base - 2, 8, stride=2), :]
                p1 = kw[j, pl.ds(base - 1, 8, stride=2), :]
                kk = [_hi(p0), _lo(p1), _hi(p1), _lo(w0), _hi(w0), _lo(w1), _hi(w1)]
                v0 = vw[j, pl.ds(T // 2 * p + 2 * m0, 8, stride=2), :]
                v1 = vw[j, pl.ds(T // 2 * p + 2 * m0 + 1, 8, stride=2), :]
                vv = [_lo(v0), _hi(v0), _lo(v1), _hi(v1)]
                for r in range(4):
                    ksh = (kk[r] * w[3] + kk[r + 1] * w[2]) + (kk[r + 2] * w[1] + kk[r + 3] * w[0])
                    outs[r].append(ksh * vv[r])
            for r in range(4):
                kv[r, pl.ds(16 * mb, 16), :] = jnp.concatenate(outs[r], axis=0).astype(BF16)
        for a in range(4):
            kraw[pl.ds(128 * a, 128), :] = ssm[cols(j), pl.ds(T * p + 128 * a, 128)].T
        for mb in range(8):
            for hf in range(2):
                wa = krw[pl.ds(32 * mb + hf, 8, stride=2), :]
                wb = krw[pl.ds(32 * mb + 16 + hf, 8, stride=2), :]
                kt[2 * hf, pl.ds(16 * mb, 16), :] = jnp.concatenate([_lo(wa), _lo(wb)], axis=0).astype(BF16)
                kt[2 * hf + 1, pl.ds(16 * mb, 16), :] = jnp.concatenate([_hi(wa), _hi(wb)], axis=0).astype(BF16)

    def bfwd(src, dst, j, p, add):
        v = [jnp.dot(f_v[r], src[r], preferred_element_type=F32) for r in range(4)]
        for i in range(16):
            z = [(v[r][16 * i:16 * i + 8], v[r][16 * i + 8:16 * i + 16]) for r in range(4)]
            a, b = _cadd(z[0], z[2]), _csub(z[0], z[2])
            if add is not None:
                a, b = (a[0] + add, a[1]), (b[0] + add, b[1])
            c, d_ = _cadd(z[1], z[3]), _csub(z[1], z[3])
            res = [_cadd(a, c), (b[0] - d_[1], b[1] + d_[0]), _csub(a, c), (b[0] + d_[1], b[1] - d_[0])]
            for h in range(4):
                dst[j, i, h, p, 0] = res[h][0]
                dst[j, i, h, p, 1] = res[h][1]

    def bv(j, i, ybuf):
        ys = [[None] * 4 for _ in range(NP)]
        for h in range(4):
            kk = [(kh[j, i, h, p, 0], kh[j, i, h, p, 1]) for p in range(NP)]
            uu = [(uh[j, i, h, p, 0], uh[j, i, h, p, 1]) for p in range(NP)]
            prev = None
            for a in range(NP):
                w = _cmul(kk[0], uu[a])
                for n in range(1, a + 1):
                    w = _cadd(w, _cmul(kk[n], uu[a - n]))
                ys[a][h] = w if prev is None else (w[0] + prev[1], w[1] - prev[0])
                prev = w
        for a in range(NP):
            y = ys[a]
            p_, q_, s_, t_ = _cadd(y[0], y[2]), _csub(y[0], y[2]), _cadd(y[1], y[3]), _csub(y[1], y[3])
            res = [_cadd(p_, s_), (q_[0] + t_[1], q_[1] - t_[0]), _csub(p_, s_), (q_[0] - t_[1], q_[1] + t_[0])]
            for r in range(4):
                ybuf[a, r, pl.ds(16 * i, 16), :] = jnp.concatenate(res[r], axis=0).astype(BF16)

    def binv(j, a, ybuf):
        y = [jnp.dot(g_v[r], ybuf[a, r], preferred_element_type=F32) for r in range(4)]
        for mb in range(16):
            for hf in range(2):
                w = qw[j, pl.ds(T // 2 * a + 16 * mb + hf, 8, stride=2), :]
                for e, qv in enumerate((_lo(w), _hi(w))):
                    r = 2 * hf + e
                    ob[j, pl.ds(T * a + 32 * mb + r, 8, stride=4), :] = qv * y[r][8 * mb:8 * mb + 8]
        start(("ob", j, a), ob.at[j, rows(a), :], o_hbm.at[rows(a), cols(NJ + j)])

    bus, kvs, kts, ybs = (bu0, bu1), (kv0, kv1), (kt0, kt1), (y0, y1)
    NU = NP * NJ
    lasts = [None] * NJ
    PREP0 = 3
    A20 = NU + 1
    BV0 = PREP0 + 1 + 16
    total = max(A20 + NU, BV0 + 16 + 4 + 4)
    for n in range(total):
        u_prep, u_fwd, u_a2, u_bv, u_inv = n - PREP0, n - PREP0 - 1, n - A20, n - BV0, n - BV0 - 4
        if n < NU:
            p, j = divmod(n, NJ)
            if j == 0:
                wait(*[("x", p, jj) for jj in range(NJ)])
            if p == 0:
                wait(("b", j, 0), ("b", j, 1))
        if u_prep == 0:
            wait("dsk", "sd", "sh", "f")
            rowp[0] = bcast(dsk_v)
            rowp[1] = bcast(sd_v)
            sh = sh_v[...].astype(F32)
            for i in range(4):
                rowp[2 + i] = jnp.broadcast_to(sh[i:i + 1], (8, D))
        if 0 <= u_prep < NU and u_prep % NP == 0:
            j = u_prep // NP
            wait(("k", j), ("v", j), ("ssm", j))
        if n == NU - NJ:
            wait("cre", "cim")
        if u_inv == 0:
            wait("g")
        if 0 <= u_inv < NU and u_inv % NP == 0:
            wait(("q", u_inv // NP))
        if n < NU:
            a1(*divmod(n, NJ), bus[n % 2])
        if 0 <= u_fwd < NU:
            j, p = divmod(u_fwd, NP)
            bfwd(kvs[u_fwd % 2], uh, j, p, None)
            bfwd(kts[u_fwd % 2], kh, j, p, rowp[1, :, cols(j)] if p == 0 else None)
        if 0 <= u_a2 < NU:
            a2(*divmod(u_a2, NJ))
        if 0 <= u_inv < NU:
            j, a = divmod(u_inv, NP)
            binv(j, a, ybs[j % 2])
        if 1 <= n <= NU:
            p, j = divmod(n - 1, NJ)
            lasts[j] = scan(p, j, bus[(n - 1) % 2], lasts[j])
        if 0 <= u_prep < NU:
            bprep(*divmod(u_prep, NP), kvs[u_prep % 2], kts[u_prep % 2])
        if NU - NJ <= n < NU:
            fold_c(n - (NU - NJ))
        if 0 <= u_bv < NU:
            j, qd = divmod(u_bv, 4)
            for i in range(4 * qd, 4 * qd + 4):
                bv(j, i, ybs[j % 2])
    wait(*list(pending))


@jax.jit
def pallas_concat_heads__ssm_conv_s5__ssm_conv_h3__prompt_kernel(
    A_x, A_Lambda_re, A_Lambda_im, A_B_re, A_B_im, A_C_re, A_C_im, A_log_dt, A_Dskip,
    B_q, B_k, B_v, B_shift_k, B_ssm_k, B_ssm_D,
):
    fwd, inv = _dft_tables()
    V = pltpu.VMEM
    scratch = [
        V((NJ, S, 128), BF16), V((NJ, S + HALO, 128), BF16), V((NJ, S, 128), BF16), V((NJ, S, 128), BF16),
        V((D, S), BF16), V((D, D), BF16), V((D, D), BF16), V((D, D), BF16), V((D, D), BF16),
        V((D, 2 * D), BF16), V((S, 2 * D), BF16),
        V((D,), BF16), V((D,), BF16), V((D,), BF16), V((D,), BF16), V((D,), BF16), V((4, D), BF16),
        V((4, 256, 128), BF16), V((4, 128, 256), BF16),
        V((NJ, 22, 8, 128), F32), V((2, 8, D), F32), V((6, 8, D), F32),
        V((2, T, 128), F32), V((2, T, 128), F32),
        V((4, 128, 128), BF16), V((4, 128, 128), BF16), V((4, 128, 128), BF16), V((4, 128, 128), BF16),
        V((T, 128), BF16),
        V((NJ, 16, 4, NP, 2, 8, 128), F32), V((NJ, 16, 4, NP, 2, 8, 128), F32),
        V((NP, 4, 256, 128), BF16), V((NP, 4, 256, 128), BF16),
        V((NJ, S, 128), F32), V((NJ, S, 128), F32),
        pltpu.SemaphoreType.DMA((112,)),
    ]
    out = pl.pallas_call(
        _kernel,
        out_shape=jax.ShapeDtypeStruct((S, 2 * D), F32),
        in_specs=[pl.BlockSpec(memory_space=pl.ANY)] * 17,
        out_specs=pl.BlockSpec(memory_space=pl.ANY),
        scratch_shapes=scratch,
        compiler_params=pltpu.CompilerParams(vmem_limit_bytes=100 * 1024 * 1024),
        name="s5_h3",
    )(A_x.reshape(S, D), A_Lambda_re, A_Lambda_im, A_B_re, A_B_im, A_C_re, A_C_im, A_log_dt, A_Dskip,
      B_q.reshape(S, D), B_k.reshape(S, D), B_v.reshape(S, D), B_shift_k.T, B_ssm_k, B_ssm_D,
      jnp.asarray(fwd), jnp.asarray(inv))
    return out.reshape(1, S, 2 * D)
```

```python
import numpy as np
import jax
import jax.numpy as jnp
from jax import lax
import jax.experimental.pallas as pl
import jax.experimental.pallas.tpu as pltpu

S, D = 2048, 640
T = 512
NP, NJ = 4, 5
HALO = 16
F32, BF16, U32 = jnp.float32, jnp.bfloat16, jnp.uint32
NT = (((1,), (1,)), ((), ()))
NN = (((1,), (0,)), ((), ()))

CFG = dict(rate=60.0, lag=8, early=1, g0=0, plan=None)


def _dft_tables():
    g = np.arange(128)[:, None]
    m = np.arange(128)[None, :]
    fwd = np.zeros((4, 256, 128), np.float64)
    for r in range(4):
        th = np.pi * (((4 * g + 1) * (4 * m + r)) % 2048) / 1024.0
        c = np.cos(th).reshape(16, 8, 128)
        s = np.sin(th).reshape(16, 8, 128)
        fwd[r] = np.stack([c, s], axis=1).reshape(256, 128)
    inv = np.transpose(fwd, (0, 2, 1)) / 512.0
    perm = np.arange(128).reshape(8, 2, 8).transpose(0, 2, 1).reshape(128)
    fwd = fwd[:, :, perm]
    inv = inv.reshape(4, 128, 2, 128).transpose(0, 2, 1, 3)[..., perm]
    tab = np.concatenate([fwd.reshape(1024, 128), inv.reshape(1024, 128)], axis=0)
    return tab.astype(jnp.bfloat16)


def _lo(w):
    return pltpu.unpack_elementwise(w, index=0, packed_dtype=BF16, unpacked_dtype=F32)


def _hi(w):
    return pltpu.unpack_elementwise(w, index=1, packed_dtype=BF16, unpacked_dtype=F32)


def _pack(a, b):
    return pltpu.pack_elementwise([a, b], packed_dtype=BF16)


def _cmul(a, b):
    return a[0] * b[0] - a[1] * b[1], a[0] * b[1] + a[1] * b[0]


def _cadd(a, b):
    return a[0] + b[0], a[1] + b[1]


def _csub(a, b):
    return a[0] - b[0], a[1] - b[1]


def _lhs_sums(a11, a12, a21, a22):
    return a11 + a22, a21 + a22, a11 + a12, a21 - a11, a12 - a22


def _rhs_factors(b11, b12, b21, b22):
    return b11 + b22, b11, b12 - b22, b21 - b11, b22, b11 + b12, b21 + b22


PARAMS = ["lre", "lim", "ldt", "z"]


def _default_plan():
    a1 = [("a1", p, j) for p in range(NP) for j in range(NJ)]
    fw = [("fw", j, p) for j in range(NJ) for p in range(NP)]
    a2 = [("a2", p, j) for p in range(NP) for j in range(3)]
    iv = [("iv", j, a) for j in range(NJ) for a in range(NP)]

    def mix(x, y):
        keyed = [((i + 0.5) / len(x), 0, u) for i, u in enumerate(x)]
        keyed += [((i + 0.75) / len(y), 1, u) for i, u in enumerate(y)]
        return [u for _, _, u in sorted(keyed)]

    bw = lambda j: [("b", j, c) for c in range(2)]
    cc = [("c", 0), ("c", 1)]
    xw = lambda p: [("x", p, j) for j in range(NJ)]
    kvs = lambda j: [("k", j), ("v", j), ("ssm", j)]
    qq = lambda *js: [("q", j) for j in js]
    rows = ["dsk", "sd", "sh", "f"]
    return [
        ([], PARAMS + xw(0) + bw(0) + bw(1) + bw(2), []),
        (PARAMS, bw(3) + bw(4) + xw(1), []),
        (xw(0) + bw(0), rows + kvs(0), a1[0:1]),
        (bw(1) + bw(2), xw(2), a1[1:3]),
        (bw(3) + bw(4) + xw(1), kvs(1) + xw(3) + kvs(2), a1[3:8]),
        (rows + kvs(0) + xw(2), cc + kvs(3) + kvs(4), a1[8:9] + mix(a1[9:12], fw[0:4])),
        (kvs(1) + xw(3), ["g"] + qq(0, 1), mix(a1[12:16], fw[4:8])),
        (kvs(2) + cc, qq(2, 3, 4), mix(a1[16:20], fw[8:12])),
        (kvs(3) + kvs(4) + ["g"] + qq(0, 1), [],
         mix(a2[0:3], fw[12:16]) + mix(a2[3:5], fw[16:20] + iv[0:2])),
        (qq(2, 3, 4), [], mix(a2[5:6], iv[2:4]) + mix(a2[6:11], iv[4:20]) + a2[11:]),
    ]


def _kernel(x_hbm, lre_hbm, lim_hbm, bre_hbm, bim_hbm, cre_hbm, cim_hbm, ldt_hbm, dsk_hbm,
            q_hbm, k_hbm, v_hbm, sh_hbm, ssm_hbm, sd_hbm, tab_hbm, z_hbm,
            o_hbm,
            xs, ks, vs, qs, ssm, bs, cs, xsum, bw_, cp, hb,
            lre_v, lim_v, ldt_v, dsk_v, sd_v, sh_v, tab_v, z_v,
            lamtab, fvec, rowp, bu, kvb, ktb, kraw,
            uh, kh, yb, oa, ob, sem):
    plan = CFG["plan"] or _default_plan()

    def cols(j):
        return pl.ds(128 * j, 128)

    def rows(p):
        return pl.ds(T * p, T)

    copies = {"lre": (lre_hbm, lre_v), "lim": (lim_hbm, lim_v), "ldt": (ldt_hbm, ldt_v), "z": (z_hbm, z_v),
              "dsk": (dsk_hbm, dsk_v), "sd": (sd_hbm, sd_v), "sh": (sh_hbm, sh_v),
              "f": (tab_hbm.at[pl.ds(0, 1024), :], tab_v.at[pl.ds(0, 1024), :]),
              "g": (tab_hbm.at[pl.ds(1024, 1024), :], tab_v.at[pl.ds(1024, 1024), :]),
              ("c", 0): (cre_hbm, cs.at[0]), ("c", 1): (cim_hbm, cs.at[1])}
    for j in range(NJ):
        copies["b", j, 0] = (bre_hbm.at[cols(j), :], bs.at[0, cols(j), :])
        copies["b", j, 1] = (bim_hbm.at[cols(j), :], bs.at[1, cols(j), :])
        copies["k", j] = (k_hbm.at[:, cols(j)], ks.at[j, pl.ds(HALO, S), :])
        copies["v", j] = (v_hbm.at[:, cols(j)], vs.at[j])
        copies["q", j] = (q_hbm.at[:, cols(j)], qs.at[j])
        copies["ssm", j] = (ssm_hbm.at[cols(j), :], ssm.at[cols(j), :])
        for p in range(NP):
            copies["x", p, j] = (x_hbm.at[rows(p), cols(j)], xs.at[j, rows(p), :])
            copies["oa", p, j] = (oa.at[j, rows(p), :], o_hbm.at[rows(p), cols(j)])
            copies["ob", p, j] = (ob.at[j, rows(p), :], o_hbm.at[rows(p), cols(NJ + j)])
    group = {n: g for g, region in enumerate(plan) for n in region[0]}
    pending = {}

    def start(name):
        c = pltpu.make_async_copy(*copies[name], sem.at[group.get(name, len(plan))])
        c.start()
        pending[name] = c

    xw, kw, vw, qw, hw, tabw, cpw, bww = (r.bitcast(U32) for r in (xs, ks, vs, qs, hb, tab_v, cp, bw_))
    sub1 = lax.broadcasted_iota(jnp.int32, (8, 128), 0)

    def bcast(ref):
        return jnp.broadcast_to(ref[...].astype(F32).reshape(1, D), (8, D))

    def xvreg(p, j, b, m):
        return xw[j, pl.ds(T // 2 * p + 32 * b + m, 8, stride=4), :]

    def discretise():
        lr, li = bcast(lre_v), bcast(lim_v)
        dt = jnp.exp(bcast(ldt_v)).astype(BF16).astype(F32)
        mag = jnp.exp(dt * lr)
        lam = (mag * jnp.cos(dt * li), mag * jnp.sin(dt * li))
        nr, ni = lam[0] - 1.0, lam[1]
        big = jnp.abs(lr) >= jnp.abs(li)
        ratio = jnp.where(big, li / lr, lr / li)
        den = jnp.where(big, lr + li * ratio, li + lr * ratio)
        fvec[0] = 2.0 * jnp.where(big, nr + ni * ratio, nr * ratio + ni) / den
        fvec[1] = 2.0 * jnp.where(big, ni - nr * ratio, ni * ratio - nr) / den
        pw = [lam]
        for i in range(1, 8):
            pw.append(_cmul(pw[(i - 1) // 2], pw[i - 1 - (i - 1) // 2]))
        mu1 = pw[7]
        mu2 = _cmul(mu1, mu1)
        mu4 = _cmul(mu2, mu2)
        sub = lax.broadcasted_iota(jnp.int32, (8, D), 0)
        tab = [c for z in pw for c in z]
        for d_, mu in ((1, mu1), (2, mu2), (4, mu4)):
            tab += [jnp.where(sub >= d_, mu[0], 0.0), jnp.where(sub >= d_, mu[1], 0.0)]
        for j in range(NJ):
            for i, t_ in enumerate(tab):
                lamtab[j, i] = t_[:, 128 * j:128 * (j + 1)]
        for j in range(NJ):
            ks[j, pl.ds(0, HALO), :] = jnp.zeros((HALO, 128), BF16)

    def row_params():
        rowp[0] = bcast(dsk_v)
        rowp[1] = bcast(sd_v)
        sh = sh_v[...].astype(F32)
        for i in range(4):
            rowp[2 + i] = jnp.broadcast_to(sh[i:i + 1], (8, D))

    def x_sums(p):
        for g in range(2):
            for kt in range(2):
                for v in range(8):
                    blk = [xvreg(p, kt + 2 * cb, 4 * g + 2 * rb + v // 4, v % 4) for rb in range(2) for cb in range(2)]
                    lo, hi = _lhs_sums(*map(_lo, blk)), _lhs_sums(*map(_hi, blk))
                    ws = [_pack(a, b) for a, b in zip(lo, hi)]
                    for n, w in enumerate(ws):
                        xsum[p, g, n, kt, pl.ds(8 * v, 8), :] = w
                    yield 28, ws

    def b_factors(j):
        for kt in range(2):
            for s in range(8):
                r = pl.ds(128 * j + 16 * s, 16)
                blk = [bs[c, r, cols(kt + 2 * kb)].astype(F32) for kb in range(2) for c in range(2)]
                for n, f in enumerate(_rhs_factors(*blk)):
                    bw_[j, 2 * n + kt, pl.ds(16 * s, 16), :] = f.astype(BF16)
                bw_[j, 14 + kt, pl.ds(16 * s, 16), :] = bs[kt, r, cols(4)]
                yield 32, [bww[j, 2 * n + kt, pl.ds(8 * s, 8), :] for n in (0, 2, 3, 5, 6)]

    lasts = [None] * NJ

    def scan(p, j):
        def tb(i):
            return lamtab[j, 2 * i], lamtab[j, 2 * i + 1]
        for b in range(T // 64):
            hs = []
            for i in range(8):
                st = pl.ds(T * p + 64 * b + 16 * (i // 2) + (i % 2), 8, stride=2)
                u = (bu[j, 0, st, :], bu[j, 1, st, :])
                hs.append(u if i == 0 else _cadd(_cmul(tb(0), hs[-1]), u))
            yield 58, list(hs[7])
            if lasts[j] is None:
                e = tuple(jnp.where(sub1 == 7, 0.0, c) for c in hs[7])
            else:
                e = tuple(jnp.where(sub1 == 7, l_, c) for l_, c in zip(lasts[j], hs[7]))
            e = tuple(pltpu.roll(c, 1, 0) for c in e)
            for n, d_ in enumerate((1, 2, 4)):
                e = _cadd(e, _cmul(tb(8 + n), tuple(pltpu.roll(c, d_, 0) for c in e)))
            yield 36, list(e)
            for i0 in (4, 0):
                for i in range(i0, i0 + 4):
                    hs[i] = _cadd(hs[i], _cmul(tb(i), e))
                if i0 == 4:
                    lasts[j] = hs[7]
                blk = [jnp.concatenate([hs[i][c], hs[i + 1][c]], axis=0) for i in (i0, i0 + 2) for c in range(2)]
                r0 = 32 * b + 4 * i0
                for n, f in enumerate(_lhs_sums(*blk) + (blk[0], blk[3])):
                    hb[p, n, j, pl.ds(r0, 16), :] = f.astype(BF16)
                yield 52, [hw[p, n, j, pl.ds(r0 // 2, 8), :] for n in (0, 1, 2)]

    def fold_c(j, i):
        f_r, f_i = (jnp.concatenate([fvec[c, :, cols(j)]] * 2, axis=0) for c in range(2))

        def fold(d_, s):
            r = pl.ds(128 * d_ + 16 * s, 16)
            a, b = cs[0, r, cols(j)].astype(F32), cs[1, r, cols(j)].astype(F32)
            return a * f_r - b * f_i, -(a * f_i) - b * f_r

        for s in range(8):
            if i < 2:
                (r0, i0), (r1, i1) = fold(2 * i, s), fold(2 * i + 1, s)
                fs = _rhs_factors(r0, r1, i0, i1)
            else:
                r0, i0 = fold(4, s)
                fs = (r0 - i0, i0, r0)
            for n, f in enumerate(fs):
                cp[7 * i + n, j, pl.ds(16 * s, 16), :] = f.astype(BF16)
            yield (58 if i < 2 else 28), [cpw[7 * i + n, j, pl.ds(8 * s, 8), :] for n in ((0, 5, 6) if i < 2 else (0,))]

    def prep_kv(j, p):
        u = j * NP + p
        for mb in range(8):
            w = [rowp[2 + i, :, cols(j)] for i in range(4)]
            outs = [[] for _ in range(4)]
            for hf in range(2):
                m0 = 16 * mb + 8 * hf
                base = HALO // 2 + T // 2 * p + 2 * m0
                w0 = kw[j, pl.ds(base, 8, stride=2), :]
                w1 = kw[j, pl.ds(base + 1, 8, stride=2), :]
                p0 = kw[j, pl.ds(base - 2, 8, stride=2), :]
                p1 = kw[j, pl.ds(base - 1, 8, stride=2), :]
                kk = [_hi(p0), _lo(p1), _hi(p1), _lo(w0), _hi(w0), _lo(w1), _hi(w1)]
                v0 = vw[j, pl.ds(T // 2 * p + 2 * m0, 8, stride=2), :]
                v1 = vw[j, pl.ds(T // 2 * p + 2 * m0 + 1, 8, stride=2), :]
                vv = [_lo(v0), _hi(v0), _lo(v1), _hi(v1)]
                for r in range(4):
                    ksh = (kk[r] * w[3] + kk[r + 1] * w[2]) + (kk[r + 2] * w[1] + kk[r + 3] * w[0])
                    outs[r].append(ksh * vv[r])
                if hf == 0:
                    yield 47, [outs[r][0] for r in range(4)]
            ws = [_pack(*outs[r]) for r in range(4)]
            for r in range(4):
                kvb[u, r, pl.ds(8 * mb, 8), :] = ws[r]
            yield 51, ws

    def prep_kt(j, p):
        u = j * NP + p
        slot = kraw.at[u % 4]
        for a in range(4):
            slot[pl.ds(128 * a, 128), :] = ssm[cols(j), pl.ds(T * p + 128 * a, 128)].astype(F32).T
            for mb in (2 * a, 2 * a + 1):
                ws = [_pack(slot[pl.ds(64 * mb + r, 8, stride=4), :], slot[pl.ds(64 * mb + 32 + r, 8, stride=4), :])
                      for r in range(4)]
                for r in range(4):
                    ktb[u, r, pl.ds(8 * mb, 8), :] = ws[r]
                yield 16, ws

    def products(j, qd):
        for i in range(4 * qd, 4 * qd + 4):
            Y = [[None] * 4 for _ in range(NP)]
            for h in (0, 2, 1, 3):
                kk = [(kh[j, i, h, n, 0], kh[j, i, h, n, 1]) for n in range(NP)]
                uu = [(uh[j, i, h, n, 0], uh[j, i, h, n, 1]) for n in range(NP)]
                prev = None
                for a in range(NP):
                    w = _cmul(kk[0], uu[a])
                    for n in range(1, a + 1):
                        w = _cadd(w, _cmul(kk[n], uu[a - n]))
                    Y[a][h] = w if prev is None else (w[0] + prev[1], w[1] - prev[0])
                    prev = w
                    if a % 2:
                        yield (0, 24, 0, 58)[a], list(Y[a][h])
            for a in range(NP):
                y = Y[a]
                p_, q_, s_, t_ = _cadd(y[0], y[2]), _csub(y[0], y[2]), _cadd(y[1], y[3]), _csub(y[1], y[3])
                res = [_cadd(p_, s_), (q_[0] + t_[1], q_[1] - t_[0]), _csub(p_, s_), (q_[0] - t_[1], q_[1] + t_[0])]
                ws = [_pack(*res[r]) for r in range(4)]
                for r in range(4):
                    yb[j, a, r, pl.ds(8 * i, 8), :] = ws[r]
                yield 22, [ws[0], ws[1]]

    def mm(tie, lhs, rhs, dims):
        return lax.dot_general(pltpu.bitcast(tie(lhs), BF16), pltpu.bitcast(rhs, BF16), dims,
                               preferred_element_type=F32)

    def program(steps, dims):
        m = {}
        for key, lhs, rhs, then in steps:
            def op(tie, key=key, lhs=lhs, rhs=rhs, then=then):
                d_ = mm(tie, lhs(), rhs(), dims)
                m[key] = m[key] + d_ if key in m else d_
                if then is not None:
                    then(m)
            yield op

    def a1(p, j):
        for g in range(2):
            def plain(rb, kt, g=g):
                return lambda: jnp.concatenate(
                    [xvreg(p, kt, 4 * g + 2 * rb + v // 4, v % 4) for v in range(8)], axis=0)

            def summed(n, kt, g=g):
                return lambda: xsum[p, g, n, kt]

            def fac(n):
                return lambda: bww[j, n]

            def put(rb, c, val, g=g):
                bu[j, c, pl.ds(T * p + 256 * g + 128 * rb, 128), :] = val

            def after4(m, put=put):
                put(0, 1, m[3] + m[5] + m["l01"])
                m["t10"] = m["l10"] + m[4]
                m["t00"] = m[4] - m[5]

            def after2(m, put=put):
                put(1, 0, m["t10"] + m[2])
                m["t11"] = m[3] - m[2]

            def after1(m):
                m["t00"] = m["t00"] + m[1]
                m["t11"] = m["t11"] + m[1]

            left = {1: lambda kt: summed(0, kt), 2: lambda kt: summed(1, kt), 3: lambda kt: plain(0, kt),
                    4: lambda kt: plain(1, 2 + kt), 5: lambda kt: summed(2, kt), 6: lambda kt: summed(3, kt),
                    7: lambda kt: summed(4, kt)}

            def prod(n, key, then):
                return [(key, left[n](kt), fac(2 * (n - 1) + kt), then if kt else None) for kt in range(2)]

            steps = (prod(3, 3, None) + prod(5, 5, None)
                     + [("l01", plain(0, 4), fac(15), None), ("l10", plain(1, 4), fac(14), None)]
                     + prod(4, 4, after4) + prod(2, 2, after2) + prod(1, 1, after1)
                     + prod(7, "t00", None) + prod(6, "t11", None)
                     + [("t00", plain(0, 4), fac(14), lambda m, put=put: put(0, 0, m["t00"])),
                        ("t11", plain(1, 4), fac(15), lambda m, put=put: put(1, 1, m["t11"]))])
            for op in program(steps, NT):
                yield 21, op

    done = {}

    def a2(p, i):
        for g in range(2):
            def left(n, kt, g=g):
                return lambda: hw[p, n, kt, pl.ds(64 * g, 64), :]

            def fac(n, kt):
                return lambda: cpw[7 * i + n, kt]

            def put(j, rb, val, g=g):
                dsk = rowp[0, :, cols(j)]
                for bb in range(4):
                    b = 4 * g + bb
                    for i0 in (0, 4):
                        w = xvreg(p, j, b, i0 // 2 + rb)
                        for e, xv in enumerate((_lo(w), _hi(w))):
                            r0 = 32 * bb + 4 * i0 + 8 * e
                            oa[j, pl.ds(T * p + 64 * b + i0 + 2 * rb + e, 8, stride=8), :] = val[r0:r0 + 8] + xv * dsk
                done[p, j] = done.get((p, j), 0) + 1
                if done[p, j] == 4:
                    start(("oa", p, j))

            def prod(ln, rn, key, then):
                return [(key, left(ln, kt), fac(rn, kt), then if kt == NJ - 1 else None) for kt in range(NJ)]

            if i < 2:
                def after4(m):
                    m["t00"] = m[4] - m[5]

                def after2(m, put=put):
                    put(2 * i, 1, m[2] + m[4])
                    m["t11"] = m[3] - m[2]

                def after1(m):
                    m["t00"] = m["t00"] + m[1]
                    m["t11"] = m["t11"] + m[1]

                steps = (prod(5, 2, 3, None)
                         + prod(2, 4, 5, lambda m, put=put: put(2 * i + 1, 0, m[3] + m[5]))
                         + prod(6, 3, 4, after4) + prod(1, 1, 2, after2) + prod(0, 0, 1, after1)
                         + prod(4, 6, "t00", lambda m, put=put: put(2 * i, 0, m["t00"]))
                         + prod(3, 5, "t11", lambda m, put=put: put(2 * i + 1, 1, m["t11"])))
            else:
                steps = (prod(5, 0, 0, None) + prod(2, 1, 0, lambda m, put=put: put(4, 0, m[0]))
                         + prod(6, 0, 1, None) + prod(1, 2, 2, lambda m, put=put: put(4, 1, m[2] - m[1])))
            for op in program(steps, NT):
                yield 21, op

    def fw(j, p):
        u = j * NP + p
        for src, dst in ((kvb, uh), (ktb, kh)):
            for hf in range(2):
                v = []
                for r in range(4):
                    def op(tie, src=src, dst=dst, hf=hf, r=r, v=v):
                        v.append(mm(tie, tabw[pl.ds(128 * r + 64 * hf, 64), :], src[u, r], NN))
                        if r < 3:
                            return
                        for i in range(8):
                            z = [(v[n][16 * i:16 * i + 8], v[n][16 * i + 8:16 * i + 16]) for n in range(4)]
                            a, b = _cadd(z[0], z[2]), _csub(z[0], z[2])
                            if dst is kh and p == 0:
                                add = rowp[1, :, cols(j)]
                                a, b = (a[0] + add, a[1]), (b[0] + add, b[1])
                            c, d_ = _cadd(z[1], z[3]), _csub(z[1], z[3])
                            res = [_cadd(a, c), (b[0] - d_[1], b[1] + d_[0]), _csub(a, c), (b[0] + d_[1], b[1] - d_[0])]
                            for h in range(4):
                                dst[j, 8 * hf + i, h, p, 0] = res[h][0]
                                dst[j, 8 * hf + i, h, p, 1] = res[h][1]
                    yield 32, op

    def iv(j, a):
        for r in range(4):
            acc = [None]
            for kt in range(2):
                def op(tie, r=r, kt=kt, acc=acc):
                    d_ = mm(tie, tabw[pl.ds(512 + 128 * r + 64 * kt, 64), :], yb[j, a, r, pl.ds(64 * kt, 64), :], NN)
                    if kt == 0:
                        acc[0] = d_
                        return
                    y = acc[0] + d_
                    for mb in range(16):
                        w = qw[j, pl.ds(T // 2 * a + 16 * mb + r // 2, 8, stride=2), :]
                        qv = _hi(w) if r % 2 else _lo(w)
                        ob[j, pl.ds(T * a + 32 * mb + r, 8, stride=4), :] = qv * y[8 * mb:8 * mb + 8]
                    if r == 3:
                        start(("ob", a, j))
                yield 24, op

    make = dict(a1=a1, a2=a2, fw=fw, iv=iv)
    regions, first, last, wait_at, count = [], {}, {}, {}, 0
    for waits, starts, units in plan:
        ops = []
        for n in waits:
            wait_at[n] = count
        for unit in units:
            first[unit] = count + len(ops)
            ops += list(make[unit[0]](*unit[1:]))
            last[unit] = count + len(ops)
        regions.append((waits, starts, ops, count))
        count += len(ops)
    lag = CFG["lag"]
    tasks = []
    for p in range(NP):
        tasks.append([first["a1", p, 0], wait_at["x", p, 0], 896, x_sums(p)])
        for j in range(NJ):
            tasks.append([min(first["a2", p, i] for i in range(3)), last["a1", p, j] + lag, 1584, scan(p, j)])
            data = max(wait_at["k", j], wait_at["sh"])
            tasks.append([first["fw", j, p], data, 784, prep_kv(j, p)])
            tasks.append([first["fw", j, p] + 8, data, 128, prep_kt(j, p)])
    for j in range(NJ):
        tasks.append([first["a1", 0, j], wait_at["b", j, 0], 512, b_factors(j)])
        for i in range(3):
            tasks.append([first["a2", 0, i], wait_at["c", 0], 464 if i < 2 else 224, fold_c(j, i)])
        ready = max(last["fw", j, p] for p in range(NP)) + lag
        for qd in range(4):
            tasks.append([min(first["iv", j, a] for a in range(NP)), ready, 1664, products(j, qd)])
    tasks.sort(key=lambda t_: t_[0])

    for idx, (waits, starts, ops, n0) in enumerate(regions):
        for name in waits:
            pending.pop(name).wait()
        for name in starts:
            start(name)
        if waits == PARAMS:
            mask = z_v[...] != 0
            discretise()
        if "sh" in waits:
            row_params()
        budget = 0.0
        for k0 in range(0, len(ops), 4):
            n, rnd = n0 + k0, ops[k0:k0 + 4]
            need = max([0.0] + [sum(t2[2] for t2 in tasks[:i + 1]) * 4 / (t_[0] - n + CFG["early"])
                                for i, t_ in enumerate(tasks) if t_[1] <= n])
            budget = min(budget, 0.0) + max(4 * CFG["rate"] - sum(c for c, _ in rnd), need)
            steps = []
            for t_ in list(tasks):
                urgent = t_[0] < n + len(rnd)
                if t_[1] > n and not urgent:
                    continue
                while budget > 0 or urgent:
                    step = next(t_[3], None)
                    if step is None:
                        tasks.remove(t_)
                        break
                    budget -= step[0]
                    t_[2] -= step[0]
                    if not urgent:
                        steps.append(step)
            gates = [[[] for _ in range(8)] for _ in rnd]
            total, acc = sum(c for c, _ in steps), 0
            for i, (cost, vals) in enumerate(steps):
                acc += cost
                gates[i % len(rnd)][min(7, CFG["g0"] + int((8 - CFG["g0"]) * acc / (total + 1)))] += vals
            for (_, op), gate in zip(rnd, gates):
                def tie(lhs, gate=gate):
                    parts = [lhs[8 * i:8 * i + 8] for i in range(8)]
                    for i, vals in enumerate(gate):
                        for val in vals:
                            parts[i] = jnp.where(mask, pltpu.bitcast(val, U32), parts[i])
                    return jnp.concatenate(parts, axis=0)
                op(tie)
    assert not tasks
    for c in pending.values():
        c.wait()


@jax.jit
def pallas_concat_heads__ssm_conv_s5__ssm_conv_h3__prompt_kernel(
    A_x, A_Lambda_re, A_Lambda_im, A_B_re, A_B_im, A_C_re, A_C_im, A_log_dt, A_Dskip,
    B_q, B_k, B_v, B_shift_k, B_ssm_k, B_ssm_D,
):
    V = pltpu.VMEM
    NU = NP * NJ
    scratch = [
        V((NJ, S, 128), BF16), V((NJ, S + HALO, 128), BF16), V((NJ, S, 128), BF16), V((NJ, S, 128), BF16),
        V((D, S), BF16), V((2, D, D), BF16), V((2, D, D), BF16),
        V((NP, 2, 5, 2, 64, 128), U32), V((NJ, 16, 128, 128), BF16),
        V((17, NJ, 128, 128), BF16), V((NP, 7, NJ, T // 2, 128), BF16),
        V((D,), BF16), V((D,), BF16), V((D,), BF16), V((D,), BF16), V((D,), BF16), V((4, D), BF16),
        V((2048, 128), BF16), V((8, 128), U32),
        V((NJ, 22, 8, 128), F32), V((2, 8, D), F32), V((6, 8, D), F32),
        V((NJ, 2, S, 128), F32),
        V((NU, 4, 64, 128), U32), V((NU, 4, 64, 128), U32), V((4, T, 128), F32),
        V((NJ, 16, 4, NP, 2, 8, 128), F32), V((NJ, 16, 4, NP, 2, 8, 128), F32),
        V((NJ, NP, 4, 128, 128), U32),
        V((NJ, S, 128), F32), V((NJ, S, 128), F32),
        pltpu.SemaphoreType.DMA((16,)),
    ]
    out = pl.pallas_call(
        _kernel,
        out_shape=jax.ShapeDtypeStruct((S, 2 * D), F32),
        in_specs=[pl.BlockSpec(memory_space=pl.ANY)] * 17,
        out_specs=pl.BlockSpec(memory_space=pl.ANY),
        scratch_shapes=scratch,
        compiler_params=pltpu.CompilerParams(vmem_limit_bytes=110 * 1024 * 1024),
        name="s5_h3",
    )(A_x.reshape(S, D), A_Lambda_re, A_Lambda_im, A_B_re, A_B_im, A_C_re, A_C_im, A_log_dt, A_Dskip,
      B_q.reshape(S, D), B_k.reshape(S, D), B_v.reshape(S, D), B_shift_k.T, B_ssm_k, B_ssm_D,
      jnp.asarray(_dft_tables()), jnp.asarray(np.zeros((8, 128), np.uint32)))
    return out.reshape(1, S, 2 * D)
```

```python
import functools

import numpy as np
import jax
import jax.numpy as jnp
from jax import lax
import jax.experimental.pallas as pl
import jax.experimental.pallas.tpu as pltpu

S, D = 2048, 640
T = 512
NP, NJ = 4, 5
HALO = 16
F32, BF16, U32 = jnp.float32, jnp.bfloat16, jnp.uint32
NT = (((1,), (1,)), ((), ()))
NN = (((1,), (0,)), ((), ()))

CFG = dict(rate=70.0, fill=0.0, boost=1.0, natlag=3, natgate=0, hold=[0], holdlag=4, cap=1.5, fwcost=40, ivcost=40, lag=8, early=32, g0=0, plan=None,
           maxtie=2,
           order=["a3 a4 a5", "a6 a7 f0 a8 f1 a9 f2 f3", "a10 f4 a11 f5 a12 f6 a13 f7 a14",
                  "a15 f8 a16 f9 a17 f10 f11 a18 f12 a19 f13 f14 c0 f15",
                  "c1 i0 f16 i1 c2 f17 i2 c3 f18 i3 f19 c4 i4 i5 c5 i6 i7 c6 i8 i9 i10 c7 i11 c8 i12 i13 "
                  "c9 i14 i15 i16 c10 i17 i18 c11 i19"])


def _dft_tables():
    g = np.arange(128)[:, None]
    m = np.arange(128)[None, :]
    fwd = np.zeros((4, 256, 128), np.float64)
    for r in range(4):
        th = np.pi * (((4 * g + 1) * (4 * m + r)) % 2048) / 1024.0
        c = np.cos(th).reshape(16, 8, 128)
        s = np.sin(th).reshape(16, 8, 128)
        fwd[r] = np.stack([c, s], axis=1).reshape(256, 128)
    inv = np.transpose(fwd, (0, 2, 1)) / 512.0
    perm = np.arange(128).reshape(8, 2, 8).transpose(0, 2, 1).reshape(128)
    fwd = fwd[:, :, perm]
    inv = inv.reshape(4, 128, 2, 128).transpose(0, 2, 1, 3)[..., perm]
    tab = np.concatenate([fwd.reshape(1024, 128), inv.reshape(1024, 128)], axis=0)
    tab = tab.reshape(64, 2, 8, 2, 128).transpose(0, 2, 1, 3, 4).reshape(2048, 128)
    return tab.astype(jnp.bfloat16)


def _lo(w):
    return pltpu.unpack_elementwise(w, index=0, packed_dtype=BF16, unpacked_dtype=F32)


def _hi(w):
    return pltpu.unpack_elementwise(w, index=1, packed_dtype=BF16, unpacked_dtype=F32)


def _il(v):
    return pl.ds(16 * (v // 2) + v % 2, 8, stride=2)


def _get(ref, idx, v0, n):
    return jnp.concatenate([ref[idx + (_il(v), slice(None))] for v in range(v0, v0 + n)], axis=0)


def _pack(a, b):
    return pltpu.pack_elementwise([a, b], packed_dtype=BF16)


def _cmul(a, b):
    return a[0] * b[0] - a[1] * b[1], a[0] * b[1] + a[1] * b[0]


def _cadd(a, b):
    return a[0] + b[0], a[1] + b[1]


def _csub(a, b):
    return a[0] - b[0], a[1] - b[1]


def _lhs_sums(a11, a12, a21, a22):
    return a11 + a22, a21 + a22, a11 + a12, a21 - a11, a12 - a22


def _rhs_factors(b11, b12, b21, b22):
    return b11 + b22, b11, b12 - b22, b21 - b11, b22, b11 + b12, b21 + b22


PARAMS = ["lre", "lim", "ldt", "z"]
B_ROWS = (pl.ds(0, 128), pl.ds(128, 256), pl.ds(384, 256))


def _default_plan():
    a1 = [("a1", p, j) for p in range(NP) for j in range(NJ)]
    fw = [("fw", j, p) for j in range(NJ) for p in range(NP)]
    a2 = [("a2", p, j) for p in range(NP) for j in range(3)]
    iv = [("iv", j, a) for j in range(NJ) for a in range(NP)]

    def mix(x, y):
        keyed = [((i + 0.5) / len(x), 0, u) for i, u in enumerate(x)]
        keyed += [((i + 0.75) / len(y), 1, u) for i, u in enumerate(y)]
        return [u for _, _, u in sorted(keyed)]

    bw = lambda g: [("b", g, c, j) for c in range(2) for j in range(NJ)]
    cc = [("c", c, j) for c in range(2) for j in range(NJ)]
    xw = lambda p: [("x", p, j) for j in range(NJ)]
    kvs = lambda j: [("k", j), ("v", j), ("ssm", j)]
    qq = lambda *js: [("q", j) for j in js]
    rows = ["dsk", "sd", "sh", "f"]
    def seq(txt):
        table = dict(a=a1, f=fw, c=a2, i=iv)
        return [table[w[0]][int(w[1:])] for w in txt.split()]

    r = [seq(t_) for t_ in CFG["order"]]
    return [
        ([], PARAMS + xw(0) + bw(0) + bw(1), []),
        (PARAMS, bw(2) + xw(1), []),
        (xw(0) + bw(0), rows + kvs(0), seq("a0")),
        (bw(1), xw(2) + kvs(1), seq("a1 a2")),
        (bw(2) + xw(1), xw(3) + kvs(2), r[0]),
        (rows + kvs(0), kvs(3) + cc, r[1]),
        (xw(2) + kvs(1) + xw(3), kvs(4) + ["g"], r[2]),
        (kvs(2) + kvs(3) + cc, qq(0, 1, 2, 3, 4), r[3]),
        (kvs(4) + ["g"] + qq(0, 1, 2, 3, 4), [], r[4]),
    ]


def _kernel(x_hbm, lre_hbm, lim_hbm, bre_hbm, bim_hbm, cre_hbm, cim_hbm, ldt_hbm, dsk_hbm,
            q_hbm, k_hbm, v_hbm, sh_hbm, ssm_hbm, sd_hbm, tab_hbm, z_hbm,
            o_hbm,
            xs, ks, vs, qs, ssm, bs, cs,
            lre_v, lim_v, ldt_v, dsk_v, sd_v, sh_v, tab_v, z_v,
            lamtab, fvec, rowp, bu, kraw, oa, ob, wprev, sem, *rest):
    rest = list(rest)
    xsums, bfs, cps, hbs, kvbs, ktbs, uhs, khs, ybs = (
        [rest.pop(0) for _ in range(n)] for n in (NP, NJ, 3, NP, NJ * NP, NJ * NP, NJ, NJ, NJ))

    plan = CFG["plan"] or _default_plan()

    def cols(j):
        return pl.ds(128 * j, 128)

    def rows(p):
        return pl.ds(T * p, T)

    copies = {"lre": (lre_hbm, lre_v), "lim": (lim_hbm, lim_v), "ldt": (ldt_hbm, ldt_v), "z": (z_hbm, z_v),
              "dsk": (dsk_hbm, dsk_v), "sd": (sd_hbm, sd_v), "sh": (sh_hbm, sh_v),
              "f": (tab_hbm.at[pl.ds(0, 1024), :], tab_v.at[pl.ds(0, 1024), :]),
              "g": (tab_hbm.at[pl.ds(1024, 1024), :], tab_v.at[pl.ds(1024, 1024), :]),
              }
    for j in range(NJ):
        for c, (b_hbm, c_hbm) in enumerate(((bre_hbm, cre_hbm), (bim_hbm, cim_hbm))):
            copies["c", c, j] = (c_hbm.at[:, cols(j)], cs.at[c, j])
            for g, r in enumerate(B_ROWS):
                copies["b", g, c, j] = (b_hbm.at[r, cols(j)], bs.at[c, j, r, :])
        copies["k", j] = (k_hbm.at[:, cols(j)], ks.at[j, pl.ds(HALO, S), :])
        copies["v", j] = (v_hbm.at[:, cols(j)], vs.at[j])
        copies["q", j] = (q_hbm.at[:, cols(j)], qs.at[j])
        copies["ssm", j] = (ssm_hbm.at[cols(j), :], ssm.at[cols(j), :])
        for p in range(NP):
            copies["x", p, j] = (x_hbm.at[rows(p), cols(j)], xs.at[j, rows(p), :])
            for g in range(2):
                r = pl.ds(T * p + T // 2 * g, T // 2)
                copies["oa", p, g, j] = (oa.at[j, r, :], o_hbm.at[r, cols(j)])
            copies["ob", p, j] = (ob.at[j, rows(p), :], o_hbm.at[rows(p), cols(NJ + j)])
    group = {n: g for g, region in enumerate(plan) for n in region[0]}
    pending = {}

    def start(name):
        c = pltpu.make_async_copy(*copies[name], sem.at[group.get(name, len(plan))])
        c.start()
        pending[name] = c

    xw, kw, vw, qw, tabw = (r.bitcast(U32) for r in (xs, ks, vs, qs, tab_v))
    bw, cw = bs.bitcast(U32), cs.bitcast(U32)
    sub1 = lax.broadcasted_iota(jnp.int32, (8, 128), 0)

    def bcast(ref):
        return jnp.broadcast_to(ref[...].astype(F32).reshape(1, D), (8, D))

    def xvreg(p, j, b, m):
        return xw[j, pl.ds(T // 2 * p + 32 * b + m, 8, stride=4), :]

    def discretise():
        lr, li = bcast(lre_v), bcast(lim_v)
        dt = jnp.exp(bcast(ldt_v)).astype(BF16).astype(F32)
        mag = jnp.exp(dt * lr)
        lam = (mag * jnp.cos(dt * li), mag * jnp.sin(dt * li))
        nr, ni = lam[0] - 1.0, lam[1]
        big = jnp.abs(lr) >= jnp.abs(li)
        ratio = jnp.where(big, li / lr, lr / li)
        den = jnp.where(big, lr + li * ratio, li + lr * ratio)
        fvec[0] = 2.0 * jnp.where(big, nr + ni * ratio, nr * ratio + ni) / den
        fvec[1] = 2.0 * jnp.where(big, ni - nr * ratio, ni * ratio - nr) / den
        pw = [lam]
        for i in range(1, 8):
            pw.append(_cmul(pw[(i - 1) // 2], pw[i - 1 - (i - 1) // 2]))
        mu1 = pw[7]
        mu2 = _cmul(mu1, mu1)
        mu4 = _cmul(mu2, mu2)
        sub = lax.broadcasted_iota(jnp.int32, (8, D), 0)
        tab = [c for z in pw for c in z]
        for d_, mu in ((1, mu1), (2, mu2), (4, mu4)):
            tab += [jnp.where(sub >= d_, mu[0], 0.0), jnp.where(sub >= d_, mu[1], 0.0)]
        for j in range(NJ):
            for i, t_ in enumerate(tab):
                lamtab[j, i] = t_[:, 128 * j:128 * (j + 1)]
        for j in range(NJ):
            ks[j, pl.ds(0, HALO), :] = jnp.zeros((HALO, 128), BF16)

    def row_params():
        rowp[0] = bcast(dsk_v)
        rowp[1] = bcast(sd_v)
        sh = sh_v[...].astype(F32)
        for i in range(4):
            rowp[2 + i] = jnp.broadcast_to(sh[i:i + 1], (8, D))

    def x_sums(p):
        for g in range(2):
            for kt in range(2):
                for v in range(8):
                    blk = [xvreg(p, kt + 2 * cb, 4 * g + 2 * rb + v // 4, v % 4) for rb in range(2) for cb in range(2)]
                    lo, hi = _lhs_sums(*map(_lo, blk)), _lhs_sums(*map(_hi, blk))
                    ws = [_pack(a, b) for a, b in zip(lo, hi)]
                    for n, w in enumerate(ws):
                        xsums[p][5 * g + n, kt, _il(v), :] = w
                    yield 28, ws

    def b_factors(j):
        for s in range(8):
            r = pl.ds(64 * j + 8 * s, 8)
            for kt in range(2):
                blk = [bw[c, kt + 2 * kb, r, :] for kb in range(2) for c in range(2)]
                lo, hi = _rhs_factors(*map(_lo, blk)), _rhs_factors(*map(_hi, blk))
                ws = [blk[0] if n == 1 else blk[3] if n == 4 else _pack(lo[n], hi[n]) for n in range(7)]
                for n, w in enumerate(ws):
                    bfs[j][2 * n + kt, _il(s), :] = w
                bfs[j][14 + kt, _il(s), :] = bw[kt, 4, r, :]
                yield 34, [ws[n] for n in (0, 2, 3, 5, 6)]

    lasts = [None] * NJ

    def scan(p, j):
        def tb(i):
            return lamtab[j, 2 * i], lamtab[j, 2 * i + 1]
        for b in range(T // 64):
            hs = []
            for i in range(8):
                st = pl.ds(T * p + 64 * b + 16 * (i // 2) + (i % 2), 8, stride=2)
                u = (bu[j, 0, st, :], bu[j, 1, st, :])
                hs.append(u if i == 0 else _cadd(_cmul(tb(0), hs[-1]), u))
            yield 58, list(hs[7])
            if lasts[j] is None:
                e = tuple(jnp.where(sub1 == 7, 0.0, c) for c in hs[7])
            else:
                e = tuple(jnp.where(sub1 == 7, l_, c) for l_, c in zip(lasts[j], hs[7]))
            e = tuple(pltpu.roll(c, 1, 0) for c in e)
            for n, d_ in enumerate((1, 2, 4)):
                e = _cadd(e, _cmul(tb(8 + n), tuple(pltpu.roll(c, d_, 0) for c in e)))
            yield 36, list(e)
            for i0 in (1, 0):
                for i in range(i0, 8, 2):
                    hs[i] = _cadd(hs[i], _cmul(tb(i), e))
                    if i == 7:
                        lasts[j] = hs[7]
                lo, hi = ([hs[i][c] for i in (i1, i1 + 2) for c in range(2)] for i1 in (i0, i0 + 4))
                lo, hi = (_lhs_sums(*blk) + (blk[0], blk[3]) for blk in (lo, hi))
                ws = [_pack(a_, b_) for a_, b_ in zip(lo, hi)]
                for n, w in enumerate(ws):
                    hbs[p][n, j, _il(2 * b + i0), :] = w
                yield 52, ws[:3]

    def fold_c(j, i):
        f_r, f_i = fvec[0, :, cols(j)], fvec[1, :, cols(j)]
        f_n = -f_i

        def fold(d_, s):
            a, b = (cw[c, j, pl.ds(64 * d_ + 8 * s, 8), :] for c in range(2))
            return [(a_ * f_r - b_ * f_i, a_ * f_n - b_ * f_r) for a_, b_ in ((_lo(a), _lo(b)), (_hi(a), _hi(b)))]

        for s in range(8):
            if i < 2:
                fs = [_rhs_factors(r0, r1, i0, i1) for (r0, i0), (r1, i1) in zip(fold(2 * i, s), fold(2 * i + 1, s))]
            else:
                fs = [(r0 - i0, i0, r0) for r0, i0 in fold(4, s)]
            ws = [_pack(a_, b_) for a_, b_ in zip(*fs)]
            for n, w in enumerate(ws):
                cps[i][n, j, _il(s), :] = w
            yield (58, [ws[0], ws[5], ws[6]]) if i < 2 else (28, ws[:1])

    def prep_kv(j, p):
        u = j * NP + p
        for mb in range(8):
            w = [rowp[2 + i, :, cols(j)] for i in range(4)]
            outs = [[] for _ in range(4)]
            for hf in range(2):
                m0 = 16 * mb + 8 * hf
                base = HALO // 2 + T // 2 * p + 2 * m0
                w0 = kw[j, pl.ds(base, 8, stride=2), :]
                w1 = kw[j, pl.ds(base + 1, 8, stride=2), :]
                p0 = kw[j, pl.ds(base - 2, 8, stride=2), :]
                p1 = kw[j, pl.ds(base - 1, 8, stride=2), :]
                kk = [_hi(p0), _lo(p1), _hi(p1), _lo(w0), _hi(w0), _lo(w1), _hi(w1)]
                v0 = vw[j, pl.ds(T // 2 * p + 2 * m0, 8, stride=2), :]
                v1 = vw[j, pl.ds(T // 2 * p + 2 * m0 + 1, 8, stride=2), :]
                vv = [_lo(v0), _hi(v0), _lo(v1), _hi(v1)]
                for r in range(4):
                    ksh = (kk[r] * w[3] + kk[r + 1] * w[2]) + (kk[r + 2] * w[1] + kk[r + 3] * w[0])
                    outs[r].append(ksh * vv[r])
                if hf == 0:
                    yield 47, [outs[r][0] for r in range(4)]
            ws = [_pack(*outs[r]) for r in range(4)]
            for r in range(4):
                kvbs[u][r, _il(mb), :] = ws[r]
            yield 51, ws

    def prep_kt(j, p):
        u = j * NP + p
        slot = kraw.at[u % 4]
        for a in range(4):
            slot[pl.ds(128 * a, 128), :] = ssm[cols(j), pl.ds(T * p + 128 * a, 128)].astype(F32).T
            for mb in (2 * a, 2 * a + 1):
                ws = [_pack(slot[pl.ds(64 * mb + r, 8, stride=4), :], slot[pl.ds(64 * mb + 32 + r, 8, stride=4), :])
                      for r in range(4)]
                for r in range(4):
                    ktbs[u][r, _il(mb), :] = ws[r]
                yield 16, ws

    def bin_(ref, i, h, n):
        return tuple(ref[i, pl.ds(64 * h + 16 * n + c, 8, stride=2), :] for c in range(2))

    recent = [None, None]

    def hold(ref, i):
        if recent[1] is not None:
            for r0 in CFG["hold"]:
                r = pl.ds(r0, 8, stride=33)
                ref[i, r, :] = jnp.where(recent[0], recent[1], ref[i, r, :])

    def product(j, i, a, prev):
        half = []
        for hs in ((0, 2), (1, 3)):
            y = []
            for h in hs:
                w = None
                for n in range(a + 1):
                    t_ = _cmul(bin_(khs[j], i, h, n), bin_(uhs[j], i, h, a - n))
                    w = t_ if w is None else _cadd(w, t_)
                y.append((w[0] + prev[h][1], w[1] - prev[h][0]) if a else w)
                prev[h] = w
                if a > 1 and h == hs[0]:
                    yield 8 * a + 8, list(y[0])
            half += [_cadd(*y), _csub(*y)]
            if hs[0] == 0 and a:
                yield (8 * a + 14 if a > 1 else 38), list(half[0])
        p_, q_, s_, t_ = half
        res = [_cadd(p_, s_), (q_[0] + t_[1], q_[1] - t_[0]), _csub(p_, s_), (q_[0] - t_[1], q_[1] + t_[0])]
        ws = [_pack(*res[r]) for r in range(4)]
        for r in range(4):
            ybs[j][a, r, _il(i), :] = ws[r]
        yield (46, 50, 36, 44)[a], [ws[0], ws[1]]

    def products(j, qd):
        for i in range(4 * qd, 4 * qd + 4):
            prev = [None] * 4
            hold(uhs[j], i)
            for a in range(NP):
                yield from product(j, i, a, prev)

    def products_of_block(j, a):
        for i in range(16):
            hold(uhs[j], i)
            prev = [bin_(wprev, i, h, (a - 1) % 2) if a else None for h in range(4)]
            yield from product(j, i, a, prev)
            if a < NP - 1:
                for h in range(4):
                    for c in range(2):
                        wprev[i, pl.ds(64 * h + 16 * (a % 2) + c, 8, stride=2), :] = prev[h][c]

    def mm(tie, lhs, rhs, dims):
        return lax.dot_general(pltpu.bitcast(tie(lhs), BF16), pltpu.bitcast(rhs, BF16), dims,
                               preferred_element_type=F32)

    def program(steps, dims):
        m = {}
        for n, (key, lhs, rhs, then) in enumerate(steps):
            def op(tie, key=key, lhs=lhs, rhs=rhs, then=then, n=n):
                d_ = mm(tie, lhs(), rhs(), dims)
                m[key] = m[key] + d_ if key in m else d_
                out = m[key][120:128]
                if then is not None:
                    then(m)
                return out
            yield op

    def a1(p, j):
        for g in range(2):
            def plain(rb, kt, g=g):
                return lambda: jnp.concatenate(
                    [xvreg(p, kt, 4 * g + 2 * rb + v // 4, v % 4) for v in range(8)], axis=0)

            def summed(n, kt, g=g):
                return lambda: _get(xsums[p], (5 * g + n, kt), 0, 8)

            def fac(n):
                return lambda: _get(bfs[j], (n,), 0, 8)

            def put(rb, c, val, g=g):
                bu[j, c, pl.ds(T * p + 256 * g + 128 * rb, 128), :] = val

            def after4(m, put=put):
                put(0, 1, m[3] + m[5] + m["l01"])
                m["t10"] = m["l10"] + m[4]
                m["t00"] = m[4] - m[5]

            def after2(m, put=put):
                put(1, 0, m["t10"] + m[2])
                m["t11"] = m[3] - m[2]

            def after1(m):
                m["t00"] = m["t00"] + m[1]
                m["t11"] = m["t11"] + m[1]

            left = {1: lambda kt: summed(0, kt), 2: lambda kt: summed(1, kt), 3: lambda kt: plain(0, kt),
                    4: lambda kt: plain(1, 2 + kt), 5: lambda kt: summed(2, kt), 6: lambda kt: summed(3, kt),
                    7: lambda kt: summed(4, kt)}

            def prod(n, key, then):
                return [(key, left[n](kt), fac(2 * (n - 1) + kt), then if kt else None) for kt in range(2)]

            steps = (prod(3, 3, None) + prod(5, 5, None)
                     + [("l01", plain(0, 4), fac(15), None), ("l10", plain(1, 4), fac(14), None)]
                     + prod(4, 4, after4) + prod(2, 2, after2) + prod(1, 1, after1)
                     + prod(7, "t00", None) + prod(6, "t11", None)
                     + [("t00", plain(0, 4), fac(14), lambda m, put=put: put(0, 0, m["t00"])),
                        ("t11", plain(1, 4), fac(15), lambda m, put=put: put(1, 1, m["t11"]))])
            for op in program(steps, NT):
                yield 21, op

    done = {}

    def a2(p, unit):
        parts = [(0, unit, None), (1, unit, None), (0, 2, unit)] if unit < 2 else [(1, 2, 0), (1, 2, 1)]
        for g, i, half in parts:
            def left(n, kt, g=g):
                return lambda: _get(hbs[p], (n, kt), 8 * g, 8)

            def fac(n, kt, i=i):
                return lambda: _get(cps[i], (n, kt), 0, 8)

            def put(j, rb, val, g=g):
                dsk = rowp[0, :, cols(j)]
                for v in range(16):
                    i = 2 * rb + (v // 2) % 2
                    t0 = T * p + 64 * (4 * g + v // 4) + 32 * (v % 2) + i
                    w = xw[j, pl.ds(t0 // 2, 8, stride=2), :]
                    oa[j, pl.ds(t0, 8, stride=4), :] = val[8 * v:8 * v + 8] + (_hi(w) if i % 2 else _lo(w)) * dsk
                done[p, g, j] = done.get((p, g, j), 0) + 1
                if done[p, g, j] == 2:
                    start(("oa", p, g, j))

            def prod(ln, rn, key, then):
                return [(key, left(ln, kt), fac(rn, kt), then if kt == NJ - 1 else None) for kt in range(NJ)]

            if i < 2:
                def after4(m):
                    m["t00"] = m[4] - m[5]

                def after2(m, put=put, i=i):
                    put(2 * i, 1, m[2] + m[4])
                    m["t11"] = m[3] - m[2]

                def after1(m):
                    m["t00"] = m["t00"] + m[1]
                    m["t11"] = m["t11"] + m[1]

                steps = (prod(5, 2, 3, None)
                         + prod(2, 4, 5, lambda m, put=put, i=i: put(2 * i + 1, 0, m[3] + m[5]))
                         + prod(6, 3, 4, after4) + prod(1, 1, 2, after2) + prod(0, 0, 1, after1)
                         + prod(4, 6, "t00", lambda m, put=put, i=i: put(2 * i, 0, m["t00"]))
                         + prod(3, 5, "t11", lambda m, put=put, i=i: put(2 * i + 1, 1, m["t11"])))
            elif half == 0:
                steps = prod(5, 0, 0, None) + prod(2, 1, 0, lambda m, put=put: put(4, 0, m[0]))
            else:
                steps = prod(6, 0, 0, None) + prod(1, 2, 1, lambda m, put=put: put(4, 1, m[1] - m[0]))
            for op in program(steps, NT):
                yield 21, op

    def fw(j, p):
        u = j * NP + p
        for src, dst in ((kvbs[u], uhs[j]), (ktbs[u], khs[j])):
            for hf in range(2):
                v = []
                for r in range(4):
                    def op(tie, src=src, dst=dst, hf=hf, r=r, v=v):
                        v.append(mm(tie, _get(tabw, (), 16 * r + 8 * hf, 8), _get(src, (r,), 0, 8), NN))
                        if r < 3:
                            return
                        for i in range(8):
                            z = [(v[n][16 * i:16 * i + 8], v[n][16 * i + 8:16 * i + 16]) for n in range(4)]
                            a, b = _cadd(z[0], z[2]), _csub(z[0], z[2])
                            if dst is khs[j] and p == 0:
                                add = rowp[1, :, cols(j)]
                                a, b = (a[0] + add, a[1]), (b[0] + add, b[1])
                            c, d_ = _cadd(z[1], z[3]), _csub(z[1], z[3])
                            res = [_cadd(a, c), (b[0] - d_[1], b[1] + d_[0]), _csub(a, c), (b[0] + d_[1], b[1] - d_[0])]
                            for h in range(4):
                                dst[8 * hf + i, pl.ds(64 * h + 16 * p, 8, stride=2), :] = res[h][0]
                                dst[8 * hf + i, pl.ds(64 * h + 16 * p + 1, 8, stride=2), :] = res[h][1]
                        return res[3][1] + res[2][0]
                    yield CFG["fwcost"], op

    def iv(j, a):
        for r in range(4):
            acc = [None]
            for kt in range(2):
                def op(tie, r=r, kt=kt, acc=acc):
                    d_ = mm(tie, _get(tabw, (), 64 + 16 * r + 8 * kt, 8), _get(ybs[j], (a, r), 8 * kt, 8), NN)
                    if kt == 0:
                        acc[0] = d_
                        return
                    y = acc[0] + d_
                    for mb in range(16):
                        w = qw[j, pl.ds(T // 2 * a + 16 * mb + r // 2, 8, stride=2), :]
                        qv = _hi(w) if r % 2 else _lo(w)
                        out = qv * y[8 * mb:8 * mb + 8]
                        ob[j, pl.ds(T * a + 32 * mb + r, 8, stride=4), :] = out
                    if r == 3:
                        start(("ob", a, j))
                    return out
                yield CFG["ivcost"], op

    make = dict(a1=a1, a2=a2, fw=fw, iv=iv)
    regions, first, last, wait_at, count = [], {}, {}, {}, 0
    for waits, starts, units in plan:
        ops = []
        for n in waits:
            wait_at[n] = count
        for unit in units:
            first[unit] = count + len(ops)
            ops += list(make[unit[0]](*unit[1:]))
            last[unit] = count + len(ops)
        regions.append((waits, starts, ops, count))
        count += len(ops)
    lag = CFG["lag"]
    tasks = []
    for p in range(NP):
        tasks.append([first["a1", p, 0], wait_at["x", p, 0], 896, x_sums(p)])
        for j in range(NJ):
            tasks.append([min(first["a2", p, i] for i in range(3)), last["a1", p, j] + lag, 1584, scan(p, j)])
            data = max(wait_at["k", j], wait_at["sh"])
            tasks.append([first["fw", j, p], data, 784, prep_kv(j, p)])
            tasks.append([first["fw", j, p] + 8, data, 128, prep_kt(j, p)])
    for j in range(NJ):
        tasks.append([first["a1", 0, j], wait_at["b", (j + 1) // 2, 0, 0], 512, b_factors(j)])
        for i in range(3):
            tasks.append([first["a2", 0, i % 2], wait_at["c", 0, 0], 464 if i < 2 else 224, fold_c(j, i)])
        ready = max(last["fw", j, p] for p in range(NP)) + lag
        for qd in range(4):
            if j == NJ - 1:
                tasks.append([first["iv", j, qd], ready, 16 * (46, 88, 110, 150)[qd], products_of_block(j, qd)])
                continue
            tasks.append([min(first["iv", j, a] for a in range(NP)), ready, 1632, products(j, qd)])
    tasks.sort(key=lambda t_: t_[0])

    cum = [0.0]
    for _, _, ops, _ in regions:
        for c, _ in ops:
            cum.append(cum[-1] + max(CFG["rate"] - c, 0.0))
    for idx, (waits, starts, ops, n0) in enumerate(regions):
        for name in waits:
            pending.pop(name).wait()
        for name in starts:
            start(name)
        if waits == PARAMS:
            mask = recent[0] = jnp.full((8, 128), z_v[0], jnp.int32) != 0
            discretise()
        if "sh" in waits:
            row_params()
        budget = 0.0
        back = []
        for k0 in range(0, len(ops), 4):
            n, rnd = n0 + k0, ops[k0:k0 + 4]
            room = cum[n + len(rnd)] - cum[n]
            need = max([0.0] + [sum(t2[2] for t2 in tasks[:i + 1]) / max(cum[max(t_[0] - CFG["early"], 0)] - cum[n], room, 1)
                                for i, t_ in enumerate(tasks)])
            budget = min(budget, 0.0) + room * max(CFG["fill"], min(need * CFG["boost"], CFG["cap"]))
            steps = []
            recent[1] = back[-CFG["holdlag"]][-1] if len(back) >= CFG["holdlag"] else None
            for t_ in list(tasks):
                urgent = t_[0] < n + len(rnd)
                if t_[1] > n and not urgent:
                    continue
                while budget > 0 or urgent:
                    step = next(t_[3], None)
                    if step is None:
                        tasks.remove(t_)
                        break
                    budget -= step[0]
                    t_[2] -= step[0]
                    if not urgent:
                        steps.append((step[0], step[1][-CFG["maxtie"]:]))
            gates = [[[] for _ in range(8)] for _ in rnd]
            total, acc = sum(c for c, _ in steps), 0
            for i, (cost, vals) in enumerate(steps):
                acc += cost
                gates[i % len(rnd)][min(7, CFG["g0"] + int((8 - CFG["g0"]) * acc / (total + 1)))] += vals
            if CFG["natlag"] and len(back) >= CFG["natlag"]:
                for gate, val in zip(gates, back[-CFG["natlag"]]):
                    if val is not None:
                        gate[CFG["natgate"]].append(val)
            back.append([])
            for (_, op), gate in zip(rnd, gates):
                def tie(lhs, gate=gate):
                    parts = [lhs[8 * i:8 * i + 8] for i in range(8)]
                    for i, vals in enumerate(gate):
                        if vals:
                            both = functools.reduce(jnp.bitwise_or, [pltpu.bitcast(val, U32) for val in vals])
                            parts[i] = jnp.where(mask, both, parts[i])
                    return jnp.concatenate(parts, axis=0)
                back[-1].append(op(tie))
    assert not tasks
    for c in pending.values():
        c.wait()


@jax.jit
def pallas_concat_heads__ssm_conv_s5__ssm_conv_h3__prompt_kernel(
    A_x, A_Lambda_re, A_Lambda_im, A_B_re, A_B_im, A_C_re, A_C_im, A_log_dt, A_Dskip,
    B_q, B_k, B_v, B_shift_k, B_ssm_k, B_ssm_D,
):
    V = pltpu.VMEM
    NU = NP * NJ
    scratch = [
        V((NJ, S, 128), BF16), V((NJ, S + HALO, 128), BF16), V((NJ, S, 128), BF16), V((NJ, S, 128), BF16),
        V((D, S), BF16), V((2, NJ, D, 128), BF16), V((2, NJ, D, 128), BF16),
        V((D,), BF16), V((D,), BF16), V((D,), BF16), V((D,), BF16), V((D,), BF16), V((4, D), BF16),
        V((2048, 128), BF16), pltpu.SMEM((1,), jnp.int32),
        V((NJ, 22, 8, 128), F32), V((2, 8, D), F32), V((6, 8, D), F32),
        V((NJ, 2, S, 128), F32), V((4, T, 128), F32),
        V((NJ, S, 128), F32), V((NJ, S, 128), F32), V((16, 256, 128), F32),
        pltpu.SemaphoreType.DMA((16,)),
    ]
    scratch += [V((10, 2, 64, 128), U32)] * NP + [V((16, 64, 128), U32)] * NJ
    scratch += [V((7, NJ, 64, 128), U32)] * 3 + [V((7, NJ, T // 4, 128), U32)] * NP
    scratch += [V((4, 64, 128), U32)] * (2 * NU)
    scratch += [V((16, 256, 128), F32)] * (2 * NJ) + [V((NP, 4, 128, 128), U32)] * NJ
    out = pl.pallas_call(
        _kernel,
        out_shape=jax.ShapeDtypeStruct((S, 2 * D), F32),
        in_specs=[pl.BlockSpec(memory_space=pl.ANY)] * 17,
        out_specs=pl.BlockSpec(memory_space=pl.ANY),
        scratch_shapes=scratch,
        compiler_params=pltpu.CompilerParams(vmem_limit_bytes=110 * 1024 * 1024),
        name="s5_h3",
    )(A_x.reshape(S, D), A_Lambda_re, A_Lambda_im, A_B_re, A_B_im, A_C_re, A_C_im, A_log_dt, A_Dskip,
      B_q.reshape(S, D), B_k.reshape(S, D), B_v.reshape(S, D), B_shift_k.T, B_ssm_k, B_ssm_D,
      jnp.asarray(_dft_tables()), jnp.asarray(np.zeros((1,), np.int32)))
    return out.reshape(1, S, 2 * D)
```

```python
import functools

import numpy as np
import jax
import jax.numpy as jnp
from jax import lax
import jax.experimental.pallas as pl
import jax.experimental.pallas.tpu as pltpu

S, D = 2048, 640
T = 512
NP, NJ = 4, 5
HALO = 16
F32, BF16, U32 = jnp.float32, jnp.bfloat16, jnp.uint32
NT = (((1,), (1,)), ((), ()))
NN = (((1,), (0,)), ((), ()))

CFG = dict(
    rate=70.0, boost=1.0, cap=1.5, fwcost=40, ivcost=40, lag=8, early=32, maxtie=2, glag=8,
    natlag=3, hold=[0], holdlag=4, waitlag=3, flag=False, more=["scan"], blocks=[[0, 1], [2], [3]], plainfirst=[0, 1, 3],
    ahead={"par": "b1", "x0": "ss0", "b1": "ss1", "x1": "ss2", "ss0": "ss3", "x3": "q4"},
    loads="par b0 x0 b1 b2 x1 rows kv0 ss0 x2 kv1 ss1 x3 kv2 ss2 c kv3 ss3 kv4 ss4 g q0 q1 q2 q3 q4",
    order="W:b0 W:x0 a0 W:b1 a1 a2 W:b2 W:x1 a3 a4 a5 W:rows W:kv0 W:ss0 a6 a7 f0 a8 f1 a9 f2 f3 "
          "W:x2 W:kv1 W:ss1 W:x3 a10 f4 a11 f5 a12 f6 a13 f7 a14 "
          "W:kv2 W:ss2 W:c W:kv3 W:ss3 a15 f8 a16 f9 a17 f10 f11 a18 f12 a19 f13 f14 c0 f15 "
          "W:kv4 W:ss4 W:g W:q0 W:q1 W:q2 W:q3 W:q4 c1 i0 f16 i1 c2 f17 i2 c3 f18 i3 f19 c4 i4 i5 c5 i6 i7 "
          "c6 i8 i9 i10 c7 i11 c8 i12 i13 c9x i14 c9y i15 c9z i16 i17 c10x i18 c10y i19 c10z c11",
)


def _dft_tables():
    g = np.arange(128)[:, None]
    m = np.arange(128)[None, :]
    fwd = np.zeros((4, 256, 128), np.float64)
    for r in range(4):
        th = np.pi * (((4 * g + 1) * (4 * m + r)) % 2048) / 1024.0
        c = np.cos(th).reshape(16, 8, 128)
        s = np.sin(th).reshape(16, 8, 128)
        fwd[r] = np.stack([c, s], axis=1).reshape(256, 128)
    inv = np.transpose(fwd, (0, 2, 1)) / 512.0
    perm = np.arange(128).reshape(8, 2, 8).transpose(0, 2, 1).reshape(128)
    fwd = fwd[:, :, perm]
    inv = inv.reshape(4, 128, 2, 128).transpose(0, 2, 1, 3)[..., perm]
    tab = np.concatenate([fwd.reshape(1024, 128), inv.reshape(1024, 128)], axis=0)
    tab = tab.reshape(64, 2, 8, 2, 128).transpose(0, 2, 1, 3, 4).reshape(2048, 128)
    return tab.astype(jnp.bfloat16)


def _lo(w):
    return pltpu.unpack_elementwise(w, index=0, packed_dtype=BF16, unpacked_dtype=F32)


def _hi(w):
    return pltpu.unpack_elementwise(w, index=1, packed_dtype=BF16, unpacked_dtype=F32)


def _il(v):
    return pl.ds(16 * (v // 2) + v % 2, 8, stride=2)


def _get(ref, idx, v0, n):
    return jnp.concatenate([ref[idx + (_il(v), slice(None))] for v in range(v0, v0 + n)], axis=0)


def _pack(a, b):
    return pltpu.pack_elementwise([a, b], packed_dtype=BF16)


def _cmul(a, b):
    return a[0] * b[0] - a[1] * b[1], a[0] * b[1] + a[1] * b[0]


def _cadd(a, b):
    return a[0] + b[0], a[1] + b[1]


def _csub(a, b):
    return a[0] - b[0], a[1] - b[1]


def _lhs_sums(a11, a12, a21, a22):
    return a11 + a22, a21 + a22, a11 + a12, a21 - a11, a12 - a22


def _rhs_factors(b11, b12, b21, b22):
    return b11 + b22, b11, b12 - b22, b21 - b11, b22, b11 + b12, b21 + b22


B_ROWS = (pl.ds(0, 128), pl.ds(128, 256), pl.ds(384, 256))


def _load_groups():
    groups = {"par": ["lre", "lim", "ldt", "z"], "rows": ["dsk", "sd", "sh", "f"], "g": ["g"],
              "c": [("c", c, j) for j in range(NJ) for c in range(2)]}
    for g in range(len(B_ROWS)):
        groups[f"b{g}"] = [("b", g, c, kt) for kt in range(NJ) for c in range(2)]
    for j in range(NJ):
        groups[f"kv{j}"] = [("k", j), ("v", j)]
        groups[f"ss{j}"] = [("ssm", j)]
        groups[f"q{j}"] = [("q", j)]
    for p in range(NP):
        groups[f"x{p}"] = [("x", p, j) for j in range(NJ)]
    return groups


def _kernel(x_hbm, lre_hbm, lim_hbm, bre_hbm, bim_hbm, cre_hbm, cim_hbm, ldt_hbm, dsk_hbm,
            q_hbm, k_hbm, v_hbm, sh_hbm, ssm_hbm, sd_hbm, tab_hbm, z_hbm,
            o_hbm,
            xs, ks, vs, qs, ssm, bs, cs,
            lre_v, lim_v, ldt_v, dsk_v, sd_v, sh_v, tab_v, z_v,
            lamtab, fvec, rowp, bu, kraw, oa, ob, wprev, sem, *rest):
    rest = list(rest)
    xsums, bfs, cps, hbs, kvbs, ktbs, uhs, khs, ybs = (
        [rest.pop(0) for _ in range(n)] for n in (NP, NJ, 3, NP, NJ * NP, NJ * NP, NJ, NJ, NJ))


    def cols(j):
        return pl.ds(128 * j, 128)

    def rows(p):
        return pl.ds(T * p, T)

    copies = {"lre": (lre_hbm, lre_v), "lim": (lim_hbm, lim_v), "ldt": (ldt_hbm, ldt_v), "z": (z_hbm, z_v),
              "dsk": (dsk_hbm, dsk_v), "sd": (sd_hbm, sd_v), "sh": (sh_hbm, sh_v),
              "f": (tab_hbm.at[pl.ds(0, 1024), :], tab_v.at[pl.ds(0, 1024), :]),
              "g": (tab_hbm.at[pl.ds(1024, 1024), :], tab_v.at[pl.ds(1024, 1024), :]),
              }
    for j in range(NJ):
        for c, (b_hbm, c_hbm) in enumerate(((bre_hbm, cre_hbm), (bim_hbm, cim_hbm))):
            copies["c", c, j] = (c_hbm.at[:, cols(j)], cs.at[c, j])
            for g, r in enumerate(B_ROWS):
                copies["b", g, c, j] = (b_hbm.at[r, cols(j)], bs.at[c, j, r, :])
        copies["k", j] = (k_hbm.at[:, cols(j)], ks.at[j, pl.ds(HALO, S), :])
        copies["v", j] = (v_hbm.at[:, cols(j)], vs.at[j])
        copies["q", j] = (q_hbm.at[:, cols(j)], qs.at[j])
        copies["ssm", j] = (ssm_hbm.at[cols(j), :], ssm.at[cols(j), :])
        for p in range(NP):
            copies["x", p, j] = (x_hbm.at[rows(p), cols(j)], xs.at[j, rows(p), :])
            for g in range(2):
                r = pl.ds(T * p + T // 2 * g, T // 2)
                copies["oa", p, g, j] = (oa.at[j, r, :], o_hbm.at[r, cols(j)])
            copies["ob", p, j] = (ob.at[j, rows(p), :], o_hbm.at[rows(p), cols(NJ + j)])
    groups = _load_groups()
    loads = CFG["loads"].split()
    batch, slot = 0, {n: 0 for n in groups["par"]}
    words = CFG["order"].split()
    for prev_, word in zip([""] + words, words):
        if word.startswith("W:"):
            batch += not prev_.startswith("W:")
            slot.update({n: batch for n in groups[word[2:]]})
    pending = {}

    def start(name):
        c = pltpu.make_async_copy(*copies[name], sem.at[slot.get(name, batch + 1)])
        c.start()
        pending[name] = c

    def wait(key):
        for name in groups[key]:
            pending.pop(name).wait()

    xw, kw, vw, qw, tabw = (r.bitcast(U32) for r in (xs, ks, vs, qs, tab_v))
    bw, cw = bs.bitcast(U32), cs.bitcast(U32)
    sub1 = lax.broadcasted_iota(jnp.int32, (8, 128), 0)

    def bcast(ref):
        return jnp.broadcast_to(ref[...].astype(F32).reshape(1, D), (8, D))

    def xvreg(p, j, b, m):
        return xw[j, pl.ds(T // 2 * p + 32 * b + m, 8, stride=4), :]

    def discretise():
        lr, li = bcast(lre_v), bcast(lim_v)
        dt = jnp.exp(bcast(ldt_v)).astype(BF16).astype(F32)
        mag = jnp.exp(dt * lr)
        lam = (mag * jnp.cos(dt * li), mag * jnp.sin(dt * li))
        nr, ni = lam[0] - 1.0, lam[1]
        big = jnp.abs(lr) >= jnp.abs(li)
        ratio = jnp.where(big, li / lr, lr / li)
        den = jnp.where(big, lr + li * ratio, li + lr * ratio)
        fvec[0] = 2.0 * jnp.where(big, nr + ni * ratio, nr * ratio + ni) / den
        fvec[1] = 2.0 * jnp.where(big, ni - nr * ratio, ni * ratio - nr) / den
        pw = [lam]
        for i in range(1, 8):
            pw.append(_cmul(pw[(i - 1) // 2], pw[i - 1 - (i - 1) // 2]))
        mu1 = pw[7]
        mu2 = _cmul(mu1, mu1)
        mu4 = _cmul(mu2, mu2)
        sub = lax.broadcasted_iota(jnp.int32, (8, D), 0)
        tab = [c for z in pw for c in z]
        for d_, mu in ((1, mu1), (2, mu2), (4, mu4)):
            tab += [jnp.where(sub >= d_, mu[0], 0.0), jnp.where(sub >= d_, mu[1], 0.0)]
        for j in range(NJ):
            for i, t_ in enumerate(tab):
                lamtab[j, i] = t_[:, 128 * j:128 * (j + 1)]
        for j in range(NJ):
            ks[j, pl.ds(0, HALO), :] = jnp.zeros((HALO, 128), BF16)

    def row_params():
        rowp[0] = bcast(dsk_v)
        rowp[1] = bcast(sd_v)
        sh = sh_v[...].astype(F32)
        for i in range(4):
            rowp[2 + i] = jnp.broadcast_to(sh[i:i + 1], (8, D))

    def x_sums(p):
        for g in range(2):
            for kt in range(2):
                for v in range(8):
                    blk = [xvreg(p, kt + 2 * cb, 4 * g + 2 * rb + v // 4, v % 4) for rb in range(2) for cb in range(2)]
                    lo, hi = _lhs_sums(*map(_lo, blk)), _lhs_sums(*map(_hi, blk))
                    ws = [_pack(a, b) for a, b in zip(lo, hi)]
                    for n, w in enumerate(ws):
                        xsums[p][5 * g + n, kt, _il(v), :] = w
                    yield 25, ws

    def b_factors(j):
        for s in range(8):
            r = pl.ds(64 * j + 8 * s, 8)
            for kt in range(2):
                blk = [bw[c, kt + 2 * kb, r, :] for kb in range(2) for c in range(2)]
                lo, hi = _rhs_factors(*map(_lo, blk)), _rhs_factors(*map(_hi, blk))
                ws = [blk[0] if n == 1 else blk[3] if n == 4 else _pack(lo[n], hi[n]) for n in range(7)]
                for n, w in enumerate(ws):
                    bfs[j][2 * n + kt, _il(s), :] = w
                bfs[j][14 + kt, _il(s), :] = bw[kt, 4, r, :]
                yield 34, [ws[n] for n in (0, 2, 3, 5, 6)]

    lasts = [None] * NJ

    def scan(p, j):
        def tb(i):
            return lamtab[j, 2 * i], lamtab[j, 2 * i + 1]
        for b in range(T // 64):
            hold2("scan", bu, (j, 0), T * p + 64 * b, 9)
            hs = []
            for i in range(8):
                st = pl.ds(T * p + 64 * b + 16 * (i // 2) + (i % 2), 8, stride=2)
                u = (bu[j, 0, st, :], bu[j, 1, st, :])
                hs.append(u if i == 0 else _cadd(_cmul(tb(0), hs[-1]), u))
            yield 58, list(hs[7])
            if lasts[j] is None:
                e = tuple(jnp.where(sub1 == 7, 0.0, c) for c in hs[7])
            else:
                e = tuple(jnp.where(sub1 == 7, l_, c) for l_, c in zip(lasts[j], hs[7]))
            e = tuple(pltpu.roll(c, 1, 0) for c in e)
            for n, d_ in enumerate((1, 2, 4)):
                e = _cadd(e, _cmul(tb(8 + n), tuple(pltpu.roll(c, d_, 0) for c in e)))
            yield 36, list(e)
            for i0 in (1, 0):
                for i in range(i0, 8, 2):
                    hs[i] = _cadd(hs[i], _cmul(tb(i), e))
                    if i == 7:
                        lasts[j] = hs[7]
                lo, hi = ([hs[i][c] for i in (i1, i1 + 2) for c in range(2)] for i1 in (i0, i0 + 4))
                lo, hi = (_lhs_sums(*blk) + (blk[0], blk[3]) for blk in (lo, hi))
                ws = [_pack(a_, b_) for a_, b_ in zip(lo, hi)]
                for n, w in enumerate(ws):
                    hbs[p][n, j, _il(2 * b + i0), :] = w
                yield 52, ws[:3]

    def fold_c(j, i):
        f_r, f_i = fvec[0, :, cols(j)], fvec[1, :, cols(j)]
        f_n = -f_i

        def fold(d_, s):
            a, b = (cw[c, j, pl.ds(64 * d_ + 8 * s, 8), :] for c in range(2))
            return [(a_ * f_r - b_ * f_i, a_ * f_n - b_ * f_r) for a_, b_ in ((_lo(a), _lo(b)), (_hi(a), _hi(b)))]

        for s in range(8):
            if s % 8 == 0:
                hold2("c", cw, (0, j), 128 * i, 9)
                hold2("c", cw, (1, j), 128 * i, 9)
            if i < 2:
                fs = [_rhs_factors(r0, r1, i0, i1) for (r0, i0), (r1, i1) in zip(fold(2 * i, s), fold(2 * i + 1, s))]
            else:
                fs = [(r0 - i0, i0, r0) for r0, i0 in fold(4, s)]
            ws = [_pack(a_, b_) for a_, b_ in zip(*fs)]
            for n, w in enumerate(ws):
                cps[i][n, j, _il(s), :] = w
            yield (58, [ws[0], ws[5], ws[6]]) if i < 2 else (28, ws[:1])

    def prep_kv(j, p):
        u = j * NP + p
        for mb in range(8):
            if mb % 2 == 0:
                hold2("kv", vw, (j,), T // 2 * p + 32 * mb, 9)
                hold2("kv", kw, (j,), HALO // 2 + T // 2 * p + 32 * mb, 9)
            w = [rowp[2 + i, :, cols(j)] for i in range(4)]
            outs = [[] for _ in range(4)]
            for hf in range(2):
                m0 = 16 * mb + 8 * hf
                base = HALO // 2 + T // 2 * p + 2 * m0
                w0 = kw[j, pl.ds(base, 8, stride=2), :]
                w1 = kw[j, pl.ds(base + 1, 8, stride=2), :]
                p0 = kw[j, pl.ds(base - 2, 8, stride=2), :]
                p1 = kw[j, pl.ds(base - 1, 8, stride=2), :]
                kk = [_hi(p0), _lo(p1), _hi(p1), _lo(w0), _hi(w0), _lo(w1), _hi(w1)]
                v0 = vw[j, pl.ds(T // 2 * p + 2 * m0, 8, stride=2), :]
                v1 = vw[j, pl.ds(T // 2 * p + 2 * m0 + 1, 8, stride=2), :]
                vv = [_lo(v0), _hi(v0), _lo(v1), _hi(v1)]
                for r in range(4):
                    ksh = (kk[r] * w[3] + kk[r + 1] * w[2]) + (kk[r + 2] * w[1] + kk[r + 3] * w[0])
                    outs[r].append(ksh * vv[r])
                if hf == 0:
                    yield 47, [outs[r][0] for r in range(4)]
            ws = [_pack(*outs[r]) for r in range(4)]
            for r in range(4):
                kvbs[u][r, _il(mb), :] = ws[r]
            yield 51, ws

    def prep_kt(j, p):
        u = j * NP + p
        slot = kraw.at[u % 4]
        for a in range(4):
            slot[pl.ds(128 * a, 128), :] = ssm[cols(j), pl.ds(T * p + 128 * a, 128)].astype(F32).T
            for mb in (2 * a, 2 * a + 1):
                ws = [_pack(slot[pl.ds(64 * mb + r, 8, stride=4), :], slot[pl.ds(64 * mb + 32 + r, 8, stride=4), :])
                      for r in range(4)]
                for r in range(4):
                    ktbs[u][r, _il(mb), :] = ws[r]
                yield 16, ws

    def bin_(ref, i, h, n):
        return tuple(ref[i, pl.ds(64 * h + 16 * n + c, 8, stride=2), :] for c in range(2))

    recent = [None, None]

    def hold2(kind, ref, idx, r0, stride):
        if recent[1] is not None and kind in CFG["more"]:
            r = idx + (pl.ds(r0, 8, stride=stride), slice(None))
            ref[r] = jnp.where(recent[0], pltpu.bitcast(recent[1], ref.dtype), ref[r])

    def hold(ref, i):
        if recent[1] is not None:
            for r0 in CFG["hold"]:
                r = pl.ds(r0, 8, stride=33)
                ref[i, r, :] = jnp.where(recent[0], recent[1], ref[i, r, :])

    def product(j, i, a, prev):
        half = []
        for hs in ((0, 2), (1, 3)):
            y = []
            for h in hs:
                w = None
                for n in range(a + 1):
                    t_ = _cmul(bin_(khs[j], i, h, n), bin_(uhs[j], i, h, a - n))
                    w = t_ if w is None else _cadd(w, t_)
                y.append((w[0] + prev[h][1], w[1] - prev[h][0]) if a else w)
                prev[h] = w
                if a > 1 and h == hs[0]:
                    yield 8 * a + 8, list(y[0])
            half += [_cadd(*y), _csub(*y)]
            if hs[0] == 0 and a:
                yield (8 * a + 14 if a > 1 else 38), list(half[0])
        p_, q_, s_, t_ = half
        res = [_cadd(p_, s_), (q_[0] + t_[1], q_[1] - t_[0]), _csub(p_, s_), (q_[0] - t_[1], q_[1] + t_[0])]
        ws = [_pack(*res[r]) for r in range(4)]
        for r in range(4):
            ybs[j][a, r, _il(i), :] = ws[r]
        yield (46, 50, 36, 44)[a], [ws[0], ws[1]]

    def products(j, qd):
        for i in range(4 * qd, 4 * qd + 4):
            prev = [None] * 4
            hold(uhs[j], i)
            for a in range(NP):
                yield from product(j, i, a, prev)

    def products_of_blocks(j, blocks):
        for i in range(16):
            hold(uhs[j], i)
            prev = [bin_(wprev, i, h, blocks[0] - 1) if blocks[0] else None for h in range(4)]
            for a in blocks:
                yield from product(j, i, a, prev)
            if a < NP - 1:
                for h in range(4):
                    for c in range(2):
                        wprev[i, pl.ds(64 * h + 16 * a + c, 8, stride=2), :] = prev[h][c]

    def mm(tie, lhs, rhs, dims):
        return lax.dot_general(pltpu.bitcast(tie(lhs), BF16), pltpu.bitcast(rhs, BF16), dims,
                               preferred_element_type=F32)

    def program(steps, dims):
        m = {}
        for n, (key, lhs, rhs, then) in enumerate(steps):
            def op(tie, key=key, lhs=lhs, rhs=rhs, then=then, n=n):
                d_ = mm(tie, lhs(), rhs(), dims)
                m[key] = m[key] + d_ if key in m else d_
                out = m[key][120:128]
                if then is not None:
                    then(m)
                return out
            yield op

    def a1(p, j):
        for g in range(2):
            def plain(rb, kt, g=g):
                return lambda: jnp.concatenate(
                    [xvreg(p, kt, 4 * g + 2 * rb + v // 4, v % 4) for v in range(8)], axis=0)

            def summed(n, kt, g=g):
                return lambda: _get(xsums[p], (5 * g + n, kt), 0, 8)

            def fac(n):
                return lambda: _get(bfs[j], (n,), 0, 8)

            def put(rb, c, val, g=g):
                bu[j, c, pl.ds(T * p + 256 * g + 128 * rb, 128), :] = val

            def after4(m, put=put):
                put(0, 1, m[3] + m[5] + m["l01"])
                m["t10"] = m["l10"] + m[4]
                m["t00"] = m[4] - m[5]

            def after2(m, put=put):
                put(1, 0, m["t10"] + m[2])
                m["t11"] = m[3] - m[2]

            def after1(m):
                m["t00"] = m["t00"] + m[1]
                m["t11"] = m["t11"] + m[1]

            left = {1: lambda kt: summed(0, kt), 2: lambda kt: summed(1, kt), 3: lambda kt: plain(0, kt),
                    4: lambda kt: plain(1, 2 + kt), 5: lambda kt: summed(2, kt), 6: lambda kt: summed(3, kt),
                    7: lambda kt: summed(4, kt)}

            def prod(n, key, then):
                return [(key, left[n](kt), fac(2 * (n - 1) + kt), then if kt else None) for kt in range(2)]

            steps = (prod(3, 3, None) + prod(5, 5, None)
                     + [("l01", plain(0, 4), fac(15), None), ("l10", plain(1, 4), fac(14), None)]
                     + prod(4, 4, after4) + prod(2, 2, after2) + prod(1, 1, after1)
                     + prod(7, "t00", None) + prod(6, "t11", None)
                     + [("t00", plain(0, 4), fac(14), lambda m, put=put: put(0, 0, m["t00"])),
                        ("t11", plain(1, 4), fac(15), lambda m, put=put: put(1, 1, m["t11"]))])
            if p == 0 and j in CFG["plainfirst"] and g == 0:
                def direct(c):
                    return lambda: bw[c, 4, pl.ds(64 * j, 64), :]

                heads = [("l" + str(rb) + str(c), plain(rb, 4), direct(c), None) for rb in range(2) for c in range(2)]
                steps = [t_ for t_ in steps[:-2] if t_[0] not in ("l01", "l10")]
                key, lhs, rhs, _ = steps.pop()

                def finish(m, put=put):
                    put(0, 0, m["t00"] + m["l00"])
                    put(1, 1, m["t11"] + m["l11"])

                steps = heads + steps + [(key, lhs, rhs, finish)]
            for op in program(steps, NT):
                yield 21, op

    done = {}

    def a2(p, unit, which):
        parts = [(0, unit, None), (1, unit, None), (0, 2, unit)] if unit < 2 else [(1, 2, 0), (1, 2, 1)]
        if which:
            parts = [parts["xyz".index(which)]]
        for g, i, half in parts:
            def left(n, kt, g=g):
                return lambda: _get(hbs[p], (n, kt), 8 * g, 8)

            def fac(n, kt, i=i):
                return lambda: _get(cps[i], (n, kt), 0, 8)

            def put(j, rb, val, g=g):
                dsk = rowp[0, :, cols(j)]
                for v in range(16):
                    i = 2 * rb + (v // 2) % 2
                    t0 = T * p + 64 * (4 * g + v // 4) + 32 * (v % 2) + i
                    w = xw[j, pl.ds(t0 // 2, 8, stride=2), :]
                    oa[j, pl.ds(t0, 8, stride=4), :] = val[8 * v:8 * v + 8] + (_hi(w) if i % 2 else _lo(w)) * dsk
                done[p, g, j] = done.get((p, g, j), 0) + 1
                if done[p, g, j] == 2:
                    start(("oa", p, g, j))

            def prod(ln, rn, key, then):
                return [(key, left(ln, kt), fac(rn, kt), then if kt == NJ - 1 else None) for kt in range(NJ)]

            if i < 2:
                def after4(m):
                    m["t00"] = m[4] - m[5]

                def after2(m, put=put, i=i):
                    put(2 * i, 1, m[2] + m[4])
                    m["t11"] = m[3] - m[2]

                def after1(m):
                    m["t00"] = m["t00"] + m[1]
                    m["t11"] = m["t11"] + m[1]

                steps = (prod(5, 2, 3, None)
                         + prod(2, 4, 5, lambda m, put=put, i=i: put(2 * i + 1, 0, m[3] + m[5]))
                         + prod(6, 3, 4, after4) + prod(1, 1, 2, after2) + prod(0, 0, 1, after1)
                         + prod(4, 6, "t00", lambda m, put=put, i=i: put(2 * i, 0, m["t00"]))
                         + prod(3, 5, "t11", lambda m, put=put, i=i: put(2 * i + 1, 1, m["t11"])))
            elif half == 0:
                steps = prod(5, 0, 0, None) + prod(2, 1, 0, lambda m, put=put: put(4, 0, m[0]))
            else:
                steps = prod(6, 0, 0, None) + prod(1, 2, 1, lambda m, put=put: put(4, 1, m[1] - m[0]))
            for op in program(steps, NT):
                yield 21, op

    def fw(j, p):
        u = j * NP + p
        for src, dst in ((kvbs[u], uhs[j]), (ktbs[u], khs[j])):
            for hf in range(2):
                v = []
                for r in range(4):
                    def op(tie, src=src, dst=dst, hf=hf, r=r, v=v):
                        v.append(mm(tie, _get(tabw, (), 16 * r + 8 * hf, 8), _get(src, (r,), 0, 8), NN))
                        if r < 3:
                            return
                        for i in range(8):
                            z = [(v[n][16 * i:16 * i + 8], v[n][16 * i + 8:16 * i + 16]) for n in range(4)]
                            a, b = _cadd(z[0], z[2]), _csub(z[0], z[2])
                            if dst is khs[j] and p == 0:
                                add = rowp[1, :, cols(j)]
                                a, b = (a[0] + add, a[1]), (b[0] + add, b[1])
                            c, d_ = _cadd(z[1], z[3]), _csub(z[1], z[3])
                            res = [_cadd(a, c), (b[0] - d_[1], b[1] + d_[0]), _csub(a, c), (b[0] + d_[1], b[1] - d_[0])]
                            for h in range(4):
                                dst[8 * hf + i, pl.ds(64 * h + 16 * p, 8, stride=2), :] = res[h][0]
                                dst[8 * hf + i, pl.ds(64 * h + 16 * p + 1, 8, stride=2), :] = res[h][1]
                        return res[3][1] + res[2][0]
                    yield CFG["fwcost"], op

    def iv(j, a):
        for r in range(4):
            acc = [None]
            for kt in range(2):
                def op(tie, r=r, kt=kt, acc=acc):
                    d_ = mm(tie, _get(tabw, (), 64 + 16 * r + 8 * kt, 8), _get(ybs[j], (a, r), 8 * kt, 8), NN)
                    if kt == 0:
                        acc[0] = d_
                        return
                    y = acc[0] + d_
                    for mb in range(16):
                        w = qw[j, pl.ds(T // 2 * a + 16 * mb + r // 2, 8, stride=2), :]
                        qv = _hi(w) if r % 2 else _lo(w)
                        out = qv * y[8 * mb:8 * mb + 8]
                        ob[j, pl.ds(T * a + 32 * mb + r, 8, stride=4), :] = out
                    if r == 3:
                        start(("ob", a, j))
                    return out
                yield CFG["ivcost"], op

    ops, first, last, wait_at, waits = [], {}, {}, {}, {}
    for word in CFG["order"].split():
        if word.startswith("W:"):
            wait_at[word[2:]] = len(ops)
            waits.setdefault(len(ops), []).append(word[2:])
            continue
        k = int(word[1:].rstrip("xyz"))
        make, unit = {"a": (a1, divmod(k, NJ)), "c": (a2, divmod(k, 3)),
                      "f": (fw, divmod(k, NP)), "i": (iv, divmod(k, NP))}[word[0]]
        first.setdefault((word[0],) + unit, len(ops))
        ops += list(make(*unit, word[1:].lstrip("0123456789")) if word[0] == "c" else make(*unit))
        last[(word[0],) + unit] = len(ops)
    lag = CFG["lag"]
    tasks = []
    for p in range(NP):
        tasks.append([first["a", p, 0], wait_at[f"x{p}"], 800, x_sums(p)])
        for j in range(NJ):
            tasks.append([min(first["c", p, i] for i in range(3)), last["a", p, j] + lag, 1584, scan(p, j)])
            tasks.append([first["f", j, p], max(wait_at[f"kv{j}"], wait_at["rows"]), 784, prep_kv(j, p)])
            tasks.append([first["f", j, p] + 8, wait_at[f"ss{j}"], 128, prep_kt(j, p)])
    for j in range(NJ):
        tasks.append([first["a", 0, j], wait_at[f"b{(j + 1) // 2}"], 512, b_factors(j)])
        for i in range(3):
            tasks.append([min(first["c", 0, i], first["c", 0, 0] if i == 2 else len(ops)), wait_at["c"], 464 if i < 2 else 224, fold_c(j, i)])
        ready = max(last["f", j, p] for p in range(NP)) + lag
        if j == NJ - 1:
            for blocks in CFG["blocks"]:
                cost = 16 * sum((48, 90, 112, 152)[a] for a in blocks)
                tasks.append([min(first["i", j, a] for a in blocks), ready, cost, products_of_blocks(j, blocks)])
        else:
            for qd in range(4):
                tasks.append([min(first["i", j, a] for a in range(NP)), ready, 1632, products(j, qd)])
    tasks.sort(key=lambda t_: t_[0])
    cum = [0.0]
    for c, _ in ops:
        cum.append(cum[-1] + max(CFG["rate"] - c, 0.0))

    queue = list(loads)

    def start_through(key):
        while key in queue:
            for name in groups[queue.pop(0)]:
                start(name)

    start_through("x0")
    wait("par")
    start_through(CFG["ahead"].get("par"))
    recent[0] = jnp.full((8, 128), z_v[0], jnp.int32) != 0
    discretise()
    budget, back, later = 0.0, [], {}
    for n in range(0, len(ops), 4):
        for key in waits.get(n, ()):
            wait(key)
        for key in waits.get(n, ()):
            later.clear()
            start_through(CFG["ahead"].get(key))
            if key == "rows":
                row_params()
        room = cum[n + 4] - cum[n]
        need = max([0.0] + [sum(t2[2] for t2 in tasks[:i + 1]) / max(cum[max(t_[0] - CFG["early"], 0)] - cum[n], room, 1)
                            for i, t_ in enumerate(tasks)])
        budget = min(budget, 0.0) + room * min(need * CFG["boost"], CFG["cap"])
        steps = []
        recent[1] = back[-CFG["holdlag"]][-1] if len(back) >= CFG["holdlag"] else None
        for t_ in list(tasks):
            urgent = t_[0] < n + 4
            if t_[1] > n and not urgent:
                continue
            while budget > 0 or urgent:
                step = next(t_[3], None)
                if step is None:
                    tasks.remove(t_)
                    break
                budget -= step[0]
                t_[2] -= step[0]
                if not urgent:
                    steps.append((step[0], step[1][-CFG["maxtie"]:]))
        gates = [[[] for _ in range(8)] for _ in range(4)]
        total, acc = sum(c for c, _ in steps), 0
        for i, (cost, vals) in enumerate(steps):
            acc += cost
            pos = 8 * (n // 4) + CFG["glag"] + int(8 * acc / (total + 1))
            later.setdefault(pos, []).append((i % 4, vals))
        for pos in range(8 * (n // 4), 8 * (n // 4) + 8):
            for i, vals in later.pop(pos, ()):
                gates[i][pos % 8] += vals
        if len(back) >= CFG["natlag"]:
            for gate, val in zip(gates, back[-CFG["natlag"]]):
                gate[0].append(val)
        back.append([])
        for (_, op), gate in zip(ops[n:n + 4], gates):
            def tie(lhs, gate=gate):
                parts = [lhs[8 * i:8 * i + 8] for i in range(8)]
                for i, vals in enumerate(gate):
                    if vals:
                        both = functools.reduce(jnp.bitwise_or, [pltpu.bitcast(val, U32) for val in vals])
                        parts[i] = jnp.where(recent[0], both, parts[i])
                return jnp.concatenate(parts, axis=0)
            out = op(tie)
            if out is not None:
                back[-1].append(out)
    assert not tasks
    for c in pending.values():
        c.wait()


@jax.jit
def pallas_concat_heads__ssm_conv_s5__ssm_conv_h3__prompt_kernel(
    A_x, A_Lambda_re, A_Lambda_im, A_B_re, A_B_im, A_C_re, A_C_im, A_log_dt, A_Dskip,
    B_q, B_k, B_v, B_shift_k, B_ssm_k, B_ssm_D,
):
    V = pltpu.VMEM
    NU = NP * NJ
    scratch = [
        V((NJ, S, 128), BF16), V((NJ, S + HALO, 128), BF16), V((NJ, S, 128), BF16), V((NJ, S, 128), BF16),
        V((D, S), BF16), V((2, NJ, D, 128), BF16), V((2, NJ, D, 128), BF16),
        V((D,), BF16), V((D,), BF16), V((D,), BF16), V((D,), BF16), V((D,), BF16), V((4, D), BF16),
        V((2048, 128), BF16), pltpu.SMEM((1,), jnp.int32),
        V((NJ, 22, 8, 128), F32), V((2, 8, D), F32), V((6, 8, D), F32),
        V((NJ, 2, S, 128), F32), V((4, T, 128), F32),
        V((NJ, S, 128), F32), V((NJ, S, 128), F32), V((16, 256, 128), F32),
        pltpu.SemaphoreType.DMA((9,)),
    ]
    scratch += [V((10, 2, 64, 128), U32)] * NP + [V((16, 64, 128), U32)] * NJ
    scratch += [V((7, NJ, 64, 128), U32)] * 3 + [V((7, NJ, T // 4, 128), U32)] * NP
    scratch += [V((4, 64, 128), U32)] * (2 * NU)
    scratch += [V((16, 256, 128), F32)] * (2 * NJ) + [V((NP, 4, 128, 128), U32)] * NJ
    out = pl.pallas_call(
        _kernel,
        out_shape=jax.ShapeDtypeStruct((S, 2 * D), F32),
        in_specs=[pl.BlockSpec(memory_space=pl.ANY)] * 17,
        out_specs=pl.BlockSpec(memory_space=pl.ANY),
        scratch_shapes=scratch,
        compiler_params=pltpu.CompilerParams(vmem_limit_bytes=110 * 1024 * 1024),
        name="s5_h3",
    )(A_x.reshape(S, D), A_Lambda_re, A_Lambda_im, A_B_re, A_B_im, A_C_re, A_C_im, A_log_dt, A_Dskip,
      B_q.reshape(S, D), B_k.reshape(S, D), B_v.reshape(S, D), B_shift_k.T, B_ssm_k, B_ssm_D,
      jnp.asarray(_dft_tables()), jnp.asarray(np.zeros((1,), np.int32)))
    return out.reshape(1, S, 2 * D)
```

```python
import functools

import numpy as np
import jax
import jax.numpy as jnp
from jax import lax
import jax.experimental.pallas as pl
import jax.experimental.pallas.tpu as pltpu

S, D = 2048, 640
T = 512
NP, NJ = 4, 5
HALO = 16
F32, BF16, U32 = jnp.float32, jnp.bfloat16, jnp.uint32
NT = (((1,), (1,)), ((), ()))
NN = (((1,), (0,)), ((), ()))
B_ROWS = (pl.ds(0, 128), pl.ds(128, 256), pl.ds(384, 256))

ORDER = ("W:x0c a0 W:b1 a1 a2 W:b2 W:x1 a3 a4 a5 a6 "
         "W:rows W:x2 W:kv0 a7 a8 f0 a9 a10 f1 a11 f2 a12 f3 a13 "
         "W:x3 W:kv1 W:kv2 W:c a14 a15 f4 a16 f5 f6 a17 f7 a18 f8 a19 f9 c0 f10 f11 c1 "
         "W:kv3 W:kv4 W:g W:q c2 i0 i1 f12 i2 c3 f13 i3 f14 f15 c4 i4 f16 f17 i5 c5 f18 i6 f19 i7 "
         "c6 i8 i9 i10 c7 i11 c8 i12 i13 c9x i14 c9y i15 c9z i16 i17 c10x i18 c10y i19 c10z c11")
LOADS = "par b0 x0a x0b x0c b1 b2 x1 rows x2 kv0 x3 kv1 kv2 c kv3 kv4 g q"
CFG = dict(
    ahead={"par": "b1", "x0c": "kv0", "b1": "kv1", "x1": "kv2", "kv0": "kv4", "x3": "q"},
    rate=70.0,
    cap=1.5,
    fwcost=40, ivcost=40, projcost=21,
    lag=8,
    early=16,
    quiet=8,
    scandue=45,
    gate=8, scangate=8, natlag=3, holdlag=4, scanlag=10,
)


def _dft_tables():
    g = np.arange(128)[:, None]
    m = np.arange(128)[None, :]
    fwd = np.zeros((4, 256, 128), np.float64)
    for r in range(4):
        th = np.pi * (((4 * g + 1) * (4 * m + r)) % 2048) / 1024.0
        c = np.cos(th).reshape(16, 8, 128)
        s = np.sin(th).reshape(16, 8, 128)
        fwd[r] = np.stack([c, s], axis=1).reshape(256, 128)
    inv = np.transpose(fwd, (0, 2, 1)) / 512.0
    perm = np.arange(128).reshape(8, 2, 8).transpose(0, 2, 1).reshape(128)
    fwd = fwd[:, :, perm]
    inv = inv.reshape(4, 128, 2, 128).transpose(0, 2, 1, 3)[..., perm]
    tab = np.concatenate([fwd.reshape(1024, 128), inv.reshape(1024, 128)], axis=0)
    tab = tab.reshape(64, 2, 8, 2, 128).transpose(0, 2, 1, 3, 4).reshape(2048, 128)
    return tab.astype(jnp.bfloat16)


def _lo(w):
    return pltpu.unpack_elementwise(w, index=0, packed_dtype=BF16, unpacked_dtype=F32)


def _hi(w):
    return pltpu.unpack_elementwise(w, index=1, packed_dtype=BF16, unpacked_dtype=F32)


def _pack(a, b):
    return pltpu.pack_elementwise([a, b], packed_dtype=BF16)


def _il(v):
    return pl.ds(16 * (v // 2) + v % 2, 8, stride=2)


def _get(ref, idx, v0):
    return jnp.concatenate([ref[idx + (_il(v), slice(None))] for v in range(v0, v0 + 8)], axis=0)


def _cmul(a, b):
    return a[0] * b[0] - a[1] * b[1], a[0] * b[1] + a[1] * b[0]


def _cadd(a, b):
    return a[0] + b[0], a[1] + b[1]


def _csub(a, b):
    return a[0] - b[0], a[1] - b[1]


def _lhs_sums(a11, a12, a21, a22):
    return a11 + a22, a21 + a22, a11 + a12, a21 - a11, a12 - a22


def _rhs_factors(b11, b12, b21, b22):
    return b11 + b22, b11, b12 - b22, b21 - b11, b22, b11 + b12, b21 + b22


def _load_groups():
    groups = {"par": ["lre", "lim", "ldt", "z"], "rows": ["dsk", "sd", "sh", "f"], "g": ["g"],
              "c": [("c", c, j) for j in range(NJ) for c in range(2)],
              "q": [("q", j) for j in range(NJ)],
              "x0a": [("x", 0, 0), ("x", 0, 2)], "x0b": [("x", 0, 1), ("x", 0, 3)], "x0c": [("x", 0, 4)]}
    for g in range(len(B_ROWS)):
        groups[f"b{g}"] = [("b", g, c, kt) for kt in range(NJ) for c in range(2)]
    for j in range(NJ):
        groups[f"kv{j}"] = [("k", j), ("v", j), ("ssm", j)]
    for p in range(1, NP):
        groups[f"x{p}"] = [("x", p, j) for j in range(NJ)]
    return groups


def _kernel(x_hbm, lre_hbm, lim_hbm, bre_hbm, bim_hbm, cre_hbm, cim_hbm, ldt_hbm, dsk_hbm,
            q_hbm, k_hbm, v_hbm, sh_hbm, ssm_hbm, sd_hbm, tab_hbm, z_hbm,
            o_hbm,
            xs, ks, vs, qs, ssm, bs, cs,
            lre_v, lim_v, ldt_v, dsk_v, sd_v, sh_v, tab_v, z_v,
            lamtab, fvec, rowp, kraw, oa, ob, wprev, sem, *rest):
    rest = list(rest)
    xsums, bfs, cps, hbs, kvbs, ktbs, uhs, khs, ybs, bus = (
        [rest.pop(0) for _ in range(n)] for n in (NP, NJ, 3, NP, NJ * NP, NJ * NP, NJ, NJ, NJ, NJ))

    def cols(j):
        return pl.ds(128 * j, 128)

    def rows(p):
        return pl.ds(T * p, T)

    copies = {"lre": (lre_hbm, lre_v), "lim": (lim_hbm, lim_v), "ldt": (ldt_hbm, ldt_v), "z": (z_hbm, z_v),
              "dsk": (dsk_hbm, dsk_v), "sd": (sd_hbm, sd_v), "sh": (sh_hbm, sh_v),
              "f": (tab_hbm.at[pl.ds(0, 1024), :], tab_v.at[pl.ds(0, 1024), :]),
              "g": (tab_hbm.at[pl.ds(1024, 1024), :], tab_v.at[pl.ds(1024, 1024), :])}
    for j in range(NJ):
        for c, (b_hbm, c_hbm) in enumerate(((bre_hbm, cre_hbm), (bim_hbm, cim_hbm))):
            copies["c", c, j] = (c_hbm.at[:, cols(j)], cs.at[c, j])
            for g, r in enumerate(B_ROWS):
                copies["b", g, c, j] = (b_hbm.at[r, cols(j)], bs.at[c, j, r, :])
        copies["k", j] = (k_hbm.at[:, cols(j)], ks.at[j, pl.ds(HALO, S), :])
        copies["v", j] = (v_hbm.at[:, cols(j)], vs.at[j])
        copies["q", j] = (q_hbm.at[:, cols(j)], qs.at[j])
        copies["ssm", j] = (ssm_hbm.at[cols(j), :], ssm.at[cols(j), :])
        for p in range(NP):
            copies["x", p, j] = (x_hbm.at[rows(p), cols(j)], xs.at[j, rows(p), :])
            for g in range(2):
                r = pl.ds(T * p + T // 2 * g, T // 2)
                copies["oa", p, g, j] = (oa.at[j, r, :], o_hbm.at[r, cols(j)])
            copies["ob", p, j] = (ob.at[j, rows(p), :], o_hbm.at[rows(p), cols(NJ + j)])

    groups = _load_groups()
    words = ORDER.split()
    slot = {n: batch for batch, key in enumerate(("par", "b0", "x0a", "x0b")) for n in groups[key]}
    batch = 3
    for before, word in zip([""] + words, words):
        if word.startswith("W:"):
            batch += not before.startswith("W:")
            slot.update({n: batch for n in groups[word[2:]]})
    queue, pending = LOADS.split(), {}

    def start(name):
        c = pltpu.make_async_copy(*copies[name], sem.at[slot.get(name, batch + 1)])
        c.start()
        pending[name] = c

    def start_through(key):
        while key in queue:
            for name in groups[queue.pop(0)]:
                start(name)

    def wait(key):
        for name in groups[key]:
            pending.pop(name).wait()

    xw, kw, vw, qw, tabw, bw, cw = (r.bitcast(U32) for r in (xs, ks, vs, qs, tab_v, bs, cs))
    sub1 = lax.broadcasted_iota(jnp.int32, (8, 128), 0)

    def bcast(ref):
        return jnp.broadcast_to(ref[...].astype(F32).reshape(1, D), (8, D))

    def xvreg(p, j, b, m):
        return xw[j, pl.ds(T // 2 * p + 32 * b + m, 8, stride=4), :]

    aid = dict(never=None, scan=None, product=None)

    def hold(kind, ref, idx, stride):
        if aid[kind] is not None:
            r = idx + (stride, slice(None))
            ref[r] = jnp.where(aid["never"], aid[kind], ref[r])

    def discretise():
        lr, li = bcast(lre_v), bcast(lim_v)
        dt = jnp.exp(bcast(ldt_v)).astype(BF16).astype(F32)
        mag = jnp.exp(dt * lr)
        lam = (mag * jnp.cos(dt * li), mag * jnp.sin(dt * li))
        nr, ni = lam[0] - 1.0, lam[1]
        big = jnp.abs(lr) >= jnp.abs(li)
        ratio = jnp.where(big, li / lr, lr / li)
        den = jnp.where(big, lr + li * ratio, li + lr * ratio)
        fvec[0] = 2.0 * jnp.where(big, nr + ni * ratio, nr * ratio + ni) / den
        fvec[1] = 2.0 * jnp.where(big, ni - nr * ratio, ni * ratio - nr) / den
        pw = [lam]
        for i in range(1, 8):
            pw.append(_cmul(pw[(i - 1) // 2], pw[i - 1 - (i - 1) // 2]))
        mu1 = pw[7]
        mu2 = _cmul(mu1, mu1)
        mu4 = _cmul(mu2, mu2)
        sub = lax.broadcasted_iota(jnp.int32, (8, D), 0)
        tab = [c for z in pw for c in z]
        for d_, mu in ((1, mu1), (2, mu2), (4, mu4)):
            tab += [jnp.where(sub >= d_, mu[0], 0.0), jnp.where(sub >= d_, mu[1], 0.0)]
        for j in range(NJ):
            for i, t_ in enumerate(tab):
                lamtab[j, i] = t_[:, 128 * j:128 * (j + 1)]
            ks[j, pl.ds(0, HALO), :] = jnp.zeros((HALO, 128), BF16)

    def row_params():
        rowp[0] = bcast(dsk_v)
        rowp[1] = bcast(sd_v)
        sh = sh_v[...].astype(F32)
        for i in range(4):
            rowp[2 + i] = jnp.broadcast_to(sh[i:i + 1], (8, D))
        yield 100, []

    def x_sums(p, kts):
        for g in range(2):
            for kt in kts:
                for v in range(8):
                    blk = [xvreg(p, kt + 2 * cb, 4 * g + 2 * rb + v // 4, v % 4) for rb in range(2) for cb in range(2)]
                    lo, hi = _lhs_sums(*map(_lo, blk)), _lhs_sums(*map(_hi, blk))
                    ws = [_pack(a, b) for a, b in zip(lo, hi)]
                    for n, w in enumerate(ws):
                        xsums[p][5 * g + n, kt, _il(v), :] = w
                    yield 25, ws

    def b_factors(j):
        for s in range(8):
            r = pl.ds(64 * j + 8 * s, 8)
            for kt in range(2):
                blk = [bw[c, kt + 2 * kb, r, :] for kb in range(2) for c in range(2)]
                lo, hi = _rhs_factors(*map(_lo, blk)), _rhs_factors(*map(_hi, blk))
                ws = [blk[0] if n == 1 else blk[3] if n == 4 else _pack(lo[n], hi[n]) for n in range(7)]
                for n, w in enumerate(ws):
                    bfs[j][2 * n + kt, _il(s), :] = w
                bfs[j][14 + kt, _il(s), :] = bw[kt, 4, r, :]
                yield 34, [ws[n] for n in (0, 2, 3, 5, 6)]

    lasts = [None] * NJ

    def scan(p, j):
        def power(i):
            return lamtab[j, 2 * i], lamtab[j, 2 * i + 1]

        for b in range(T // 64):
            hold("scan", bus[j], (0,), pl.ds(T * p + 64 * b, 8, stride=9))
            hs = []
            for i in range(8):
                st = pl.ds(T * p + 64 * b + 16 * (i // 2) + (i % 2), 8, stride=2)
                u = (bus[j][0, st, :], bus[j][1, st, :])
                hs.append(u if i == 0 else _cadd(_cmul(power(0), hs[-1]), u))
            yield 58, list(hs[7]), CFG["scangate"]
            e = tuple(jnp.where(sub1 == 7, c0, c1) for c0, c1 in zip(lasts[j] or (0.0, 0.0), hs[7]))
            e = tuple(pltpu.roll(c, 1, 0) for c in e)
            for n, d_ in enumerate((1, 2, 4)):
                e = _cadd(e, _cmul(power(8 + n), tuple(pltpu.roll(c, d_, 0) for c in e)))
            yield 36, list(e), CFG["scangate"]
            for i0 in (1, 0):
                for i in range(i0, 8, 2):
                    hs[i] = _cadd(hs[i], _cmul(power(i), e))
                    if i == 7:
                        lasts[j] = hs[7]
                lo, hi = ([hs[i][c] for i in (i1, i1 + 2) for c in range(2)] for i1 in (i0, i0 + 4))
                lo, hi = (_lhs_sums(*blk) + (blk[0], blk[3]) for blk in (lo, hi))
                ws = [_pack(a_, b_) for a_, b_ in zip(lo, hi)]
                for n, w in enumerate(ws):
                    hbs[p][n, j, _il(2 * b + i0), :] = w
                yield 52, ws[:3], CFG["scangate"]

    def fold_c(j, i):
        f_r, f_i = fvec[0, :, cols(j)], fvec[1, :, cols(j)]
        f_n = -f_i

        def fold(d_, s):
            a, b = (cw[c, j, pl.ds(64 * d_ + 8 * s, 8), :] for c in range(2))
            return [(a_ * f_r - b_ * f_i, a_ * f_n - b_ * f_r) for a_, b_ in ((_lo(a), _lo(b)), (_hi(a), _hi(b)))]

        for s in range(8):
            if i < 2:
                fs = [_rhs_factors(r0, r1, i0, i1) for (r0, i0), (r1, i1) in zip(fold(2 * i, s), fold(2 * i + 1, s))]
            else:
                fs = [(r0 - i0, i0, r0) for r0, i0 in fold(4, s)]
            ws = [_pack(a_, b_) for a_, b_ in zip(*fs)]
            for n, w in enumerate(ws):
                cps[i][n, j, _il(s), :] = w
            yield (58, [ws[0], ws[5], ws[6]]) if i < 2 else (28, ws[:1])

    def prep_kv(j, p):
        for mb in range(8):
            w = [rowp[2 + i, :, cols(j)] for i in range(4)]
            outs = [[] for _ in range(4)]
            for hf in range(2):
                at = T // 2 * p + 32 * mb + 16 * hf
                p0, p1, w0, w1 = (kw[j, pl.ds(HALO // 2 + at + o, 8, stride=2), :] for o in (-2, -1, 0, 1))
                kk = [_hi(p0), _lo(p1), _hi(p1), _lo(w0), _hi(w0), _lo(w1), _hi(w1)]
                v0, v1 = (vw[j, pl.ds(at + o, 8, stride=2), :] for o in (0, 1))
                vv = [_lo(v0), _hi(v0), _lo(v1), _hi(v1)]
                for r in range(4):
                    ksh = (kk[r] * w[3] + kk[r + 1] * w[2]) + (kk[r + 2] * w[1] + kk[r + 3] * w[0])
                    outs[r].append(ksh * vv[r])
                if hf == 0:
                    yield 47, [outs[r][0] for r in range(4)]
            ws = [_pack(*outs[r]) for r in range(4)]
            for r in range(4):
                kvbs[j * NP + p][r, _il(mb), :] = ws[r]
            yield 51, ws

    def prep_filter(j, p):
        raw = kraw.at[(j * NP + p) % 4]
        for a in range(4):
            raw[pl.ds(128 * a, 128), :] = ssm[cols(j), pl.ds(T * p + 128 * a, 128)].astype(F32).T
            for mb in (2 * a, 2 * a + 1):
                ws = [_pack(raw[pl.ds(64 * mb + r, 8, stride=4), :], raw[pl.ds(64 * mb + 32 + r, 8, stride=4), :])
                      for r in range(4)]
                for r in range(4):
                    ktbs[j * NP + p][r, _il(mb), :] = ws[r]
                yield 16, ws

    def bin_(ref, i, h, n):
        return tuple(ref[i, pl.ds(64 * h + 16 * n + c, 8, stride=2), :] for c in range(2))

    def product(j, i, a, prev):
        half = []
        for hs in ((0, 2), (1, 3)):
            y = []
            for h in hs:
                w = None
                for n in range(a + 1):
                    t_ = _cmul(bin_(khs[j], i, h, n), bin_(uhs[j], i, h, a - n))
                    w = t_ if w is None else _cadd(w, t_)
                y.append((w[0] + prev[h][1], w[1] - prev[h][0]) if a else w)
                prev[h] = w
                if a > 1 and h == hs[0]:
                    yield 8 * a + 8, list(y[0])
            half += [_cadd(*y), _csub(*y)]
            if hs[0] == 0 and a:
                yield (8 * a + 14 if a > 1 else 38), list(half[0])
        p_, q_, s_, t_ = half
        res = [_cadd(p_, s_), (q_[0] + t_[1], q_[1] - t_[0]), _csub(p_, s_), (q_[0] - t_[1], q_[1] + t_[0])]
        ws = [_pack(*res[r]) for r in range(4)]
        for r in range(4):
            ybs[j][a, r, _il(i), :] = ws[r]
        yield (46, 50, 36, 44)[a], ws[:2]

    def products(j, blocks, groups_):
        for i in groups_:
            hold("product", uhs[j], (i,), pl.ds(0, 8, stride=33))
            prev = [bin_(wprev, i, h, blocks[0] - 1) if blocks[0] else None for h in range(4)]
            for a in blocks:
                yield from product(j, i, a, prev)
            if a < NP - 1:
                for h in range(4):
                    for c in range(2):
                        wprev[i, pl.ds(64 * h + 16 * a + c, 8, stride=2), :] = prev[h][c]

    def mm(tie, lhs, rhs, dims):
        return lax.dot_general(pltpu.bitcast(tie(lhs), BF16), pltpu.bitcast(rhs, BF16), dims,
                               preferred_element_type=F32)

    def program(steps):
        m = {}
        for key, lhs, rhs, then in steps:
            def op(tie, key=key, lhs=lhs, rhs=rhs, then=then):
                d_ = mm(tie, lhs(), rhs(), NT)
                m[key] = m[key] + d_ if key in m else d_
                out = m[key][120:128]
                if then is not None:
                    then(m)
                return out
            yield CFG["projcost"], op

    def project_in(p, j):
        for g in range(2):
            def plain(rb, kt, g=g):
                return lambda: jnp.concatenate(
                    [xvreg(p, kt, 4 * g + 2 * rb + v // 4, v % 4) for v in range(8)], axis=0)

            def put(rb, c, val, g=g):
                bus[j][c, pl.ds(T * p + 256 * g + 128 * rb, 128), :] = val

            def prod(n, key, then):
                def left(kt, g=g):
                    if n in (3, 4):
                        return plain(n - 3, 2 * (n - 3) + kt)
                    return lambda: _get(xsums[p], (5 * g + {1: 0, 2: 1, 5: 2, 6: 3, 7: 4}[n], kt), 0)
                return [(key, left(kt), lambda kt=kt: _get(bfs[j], (2 * (n - 1) + kt,), 0), then if kt else None)
                        for kt in range(2)]

            lead = p == 0 and j in (0, 1, 3) and g == 0

            def after4(m, put=put):
                put(0, 1, m[3] + m[5] + m["l01"])
                m["t10"] = m["l10"] + m[4]
                m["t00"] = m[4] - m[5]

            def after2(m, put=put):
                put(1, 0, m["t10"] + m[2])
                m["t11"] = m[3] - m[2]

            def after1(m):
                m["t00"] = m["t00"] + m[1]
                m["t11"] = m["t11"] + m[1]

            def finish(m, put=put):
                put(0, 0, m["t00"] + m["l00"])
                put(1, 1, m["t11"] + m["l11"])

            def fifth(key, rb, c, then=None):
                if lead:
                    return key, plain(rb, 4), lambda: bw[c, 4, pl.ds(64 * j, 64), :], then
                return key, plain(rb, 4), lambda: _get(bfs[j], (14 + c,), 0), then

            middle = (prod(4, 4, after4) + prod(2, 2, after2) + prod(1, 1, after1) + prod(7, "t00", None)
                      + prod(6, "t11", finish if lead else None))
            if lead:
                steps = ([fifth(f"l{rb}{c}", rb, c) for rb in range(2) for c in range(2)]
                         + prod(3, 3, None) + prod(5, 5, None) + middle)
            else:
                steps = (prod(3, 3, None) + prod(5, 5, None) + [fifth("l01", 0, 1), fifth("l10", 1, 0)] + middle
                         + [fifth("t00", 0, 0, lambda m, put=put: put(0, 0, m["t00"])),
                            fifth("t11", 1, 1, lambda m, put=put: put(1, 1, m["t11"]))])
            yield from program(steps)

    done = {}

    def project_out(p, unit, part):
        parts = [(0, unit, None), (1, unit, None), (0, 2, unit)] if unit < 2 else [(1, 2, 0), (1, 2, 1)]
        for g, i, half in [parts["xyz".index(part)]] if part else parts:
            def put(j, rb, val, g=g):
                dsk = rowp[0, :, cols(j)]
                for v in range(16):
                    step = 2 * rb + (v // 2) % 2
                    t0 = T * p + 64 * (4 * g + v // 4) + 32 * (v % 2) + step
                    w = xw[j, pl.ds(t0 // 2, 8, stride=2), :]
                    oa[j, pl.ds(t0, 8, stride=4), :] = val[8 * v:8 * v + 8] + (_hi(w) if step % 2 else _lo(w)) * dsk
                done[p, g, j] = done.get((p, g, j), 0) + 1
                if done[p, g, j] == 2:
                    start(("oa", p, g, j))

            def prod(ln, rn, key, then):
                return [(key, lambda kt=kt, g=g: _get(hbs[p], (ln, kt), 8 * g),
                         lambda kt=kt, i=i: _get(cps[i], (rn, kt), 0), then if kt == NJ - 1 else None)
                        for kt in range(NJ)]

            if i < 2:
                def after4(m):
                    m["t00"] = m[4] - m[5]

                def after2(m, put=put, i=i):
                    put(2 * i, 1, m[2] + m[4])
                    m["t11"] = m[3] - m[2]

                def after1(m):
                    m["t00"] = m["t00"] + m[1]
                    m["t11"] = m["t11"] + m[1]

                steps = (prod(5, 2, 3, None)
                         + prod(2, 4, 5, lambda m, put=put, i=i: put(2 * i + 1, 0, m[3] + m[5]))
                         + prod(6, 3, 4, after4) + prod(1, 1, 2, after2) + prod(0, 0, 1, after1)
                         + prod(4, 6, "t00", lambda m, put=put, i=i: put(2 * i, 0, m["t00"]))
                         + prod(3, 5, "t11", lambda m, put=put, i=i: put(2 * i + 1, 1, m["t11"])))
            elif half == 0:
                steps = prod(5, 0, 0, None) + prod(2, 1, 0, lambda m, put=put: put(4, 0, m[0]))
            else:
                steps = prod(6, 0, 0, None) + prod(1, 2, 1, lambda m, put=put: put(4, 1, m[1] - m[0]))
            yield from program(steps)

    def forward(j, p):
        for src, dst in ((kvbs[j * NP + p], uhs[j]), (ktbs[j * NP + p], khs[j])):
            for hf in range(2):
                v = []
                for r in range(4):
                    def op(tie, src=src, dst=dst, hf=hf, r=r, v=v):
                        v.append(mm(tie, _get(tabw, (), 16 * r + 8 * hf), _get(src, (r,), 0), NN))
                        if r < 3:
                            return None
                        for i in range(8):
                            z = [(v[n][16 * i:16 * i + 8], v[n][16 * i + 8:16 * i + 16]) for n in range(4)]
                            a, b = _cadd(z[0], z[2]), _csub(z[0], z[2])
                            if dst is khs[j] and p == 0:
                                tap = rowp[1, :, cols(j)]
                                a, b = (a[0] + tap, a[1]), (b[0] + tap, b[1])
                            c, d_ = _cadd(z[1], z[3]), _csub(z[1], z[3])
                            res = [_cadd(a, c), (b[0] - d_[1], b[1] + d_[0]), _csub(a, c), (b[0] + d_[1], b[1] - d_[0])]
                            for h in range(4):
                                for e in range(2):
                                    dst[8 * hf + i, pl.ds(64 * h + 16 * p + e, 8, stride=2), :] = res[h][e]
                        return res[3][1] + res[2][0]
                    yield CFG["fwcost"], op

    def inverse(j, a):
        for r in range(4):
            acc = []
            for kt in range(2):
                def op(tie, r=r, kt=kt, acc=acc):
                    acc.append(mm(tie, _get(tabw, (), 64 + 16 * r + 8 * kt), _get(ybs[j], (a, r), 8 * kt), NN))
                    if kt == 0:
                        return None
                    y = acc[0] + acc[1]
                    for mb in range(16):
                        w = qw[j, pl.ds(T // 2 * a + 16 * mb + r // 2, 8, stride=2), :]
                        out = (_hi(w) if r % 2 else _lo(w)) * y[8 * mb:8 * mb + 8]
                        ob[j, pl.ds(T * a + 32 * mb + r, 8, stride=4), :] = out
                    if r == 3:
                        start(("ob", a, j))
                    return out
                yield CFG["ivcost"], op

    ops, first, last, wait_at, waits = [], {}, {}, {}, {}
    for word in words:
        if word.startswith("W:"):
            wait_at[word[2:]] = len(ops)
            waits.setdefault(len(ops), []).append(word[2:])
            continue
        k = int(word[1:].rstrip("xyz"))
        make, unit = {"a": (project_in, divmod(k, NJ)), "c": (project_out, divmod(k, 3)),
                      "f": (forward, divmod(k, NP)), "i": (inverse, divmod(k, NP))}[word[0]]
        key = (word[0],) + unit
        first.setdefault(key, len(ops))
        ops += list(make(*unit, word[1:].lstrip("0123456789")) if word[0] == "c" else make(*unit))
        last[key] = len(ops)

    lag = CFG["lag"]
    tasks = [[wait_at["rows"] + 4, wait_at["rows"], 100, row_params()]]
    for p in range(NP):
        if p:
            tasks.append([first["a", p, 0], wait_at[f"x{p}"], 800, x_sums(p, (0, 1))])
        for j in range(NJ):
            due = min(first["c", p, i] for i in range(3)) - CFG["scandue"] * p
            tasks.append([due, last["a", p, j] + lag, 1584, scan(p, j)])
            tasks.append([first["f", j, p], max(wait_at[f"kv{j}"], wait_at["rows"] + 4), 784, prep_kv(j, p)])
            tasks.append([first["f", j, p] + 8, wait_at[f"kv{j}"], 128, prep_filter(j, p)])
    for j in range(NJ):
        if j:
            tasks.append([first["a", 0, j], wait_at[f"b{(j + 1) // 2}"], 512, b_factors(j)])
        for i in range(3):
            due = min(first["c", 0, i], first["c", 0, 0] if i == 2 else len(ops))
            tasks.append([due, wait_at["c"], 464 if i < 2 else 224, fold_c(j, i)])
        ready = max(last["f", j, p] for p in range(NP)) + lag
        for blocks, part in ([((0, 1), range(16)), ((2,), range(16)), ((3,), range(16))] if j == NJ - 1 else
                             [((0, 1, 2, 3), range(4 * i, 4 * i + 4)) for i in range(4)]):
            cost = len(part) * sum((48, 90, 112, 152)[a] for a in blocks) if j == NJ - 1 else 1632
            tasks.append([min(first["i", j, a] for a in blocks), ready, cost, products(j, blocks, part)])
    tasks.sort(key=lambda t_: t_[0])
    cum = [0.0]
    for n, (c, _) in enumerate(ops):
        quiet = any(n + ahead in waits for ahead in range(1, CFG["quiet"] + 1))
        cum.append(cum[-1] + (0.0 if quiet else max(CFG["rate"] - c, 0.0)))

    start_through("x0c")
    wait("par")
    start_through(CFG["ahead"]["par"])
    aid["never"] = jnp.full((8, 128), z_v[0], jnp.int32) != 0
    discretise()
    for key, task in (("b0", b_factors(0)), ("x0a", x_sums(0, (0,))), ("x0b", x_sums(0, (1,)))):
        wait(key)
        for _ in task:
            pass

    budget, back, later = 0.0, [], {}
    for n in range(0, len(ops), 4):
        for key in waits.get(n, ()):
            wait(key)
        for key in waits.get(n, ()):
            later.clear()
            start_through(CFG["ahead"].get(key))
        room = cum[n + 4] - cum[n]
        need = max([0.0] + [sum(t2[2] for t2 in tasks[:i + 1]) / max(cum[max(t_[0] - CFG["early"], 0)] - cum[n], room, 1)
                            for i, t_ in enumerate(tasks)])
        budget = min(budget, 0.0) + room * min(need, CFG["cap"])
        for kind, behind in (("product", CFG["holdlag"]), ("scan", CFG["scanlag"])):
            aid[kind] = back[-behind][-1] if len(back) >= behind else None
        steps = []
        for t_ in list(tasks):
            urgent = t_[0] < n + 4
            if t_[1] > n and not urgent:
                continue
            while budget > 0 or urgent:
                step = next(t_[3], None)
                if step is None:
                    tasks.remove(t_)
                    break
                if not urgent:
                    budget -= step[0]
                    t_[2] -= step[0]
                    steps.append((step[0], step[1][-2:], sum(step[2:])))
        total, acc = sum(t_[0] for t_ in steps), 0
        for i, (cost, vals, slack) in enumerate(steps):
            acc += cost
            later.setdefault(2 * n + CFG["gate"] + slack + int(8 * acc / (total + 1)), []).append((i % 4, vals))
        gates = [[[] for _ in range(8)] for _ in range(4)]
        for pos in range(8):
            for i, vals in later.pop(2 * n + pos, ()):
                gates[i][pos] += vals
        if len(back) >= CFG["natlag"]:
            for gate, val in zip(gates, back[-CFG["natlag"]]):
                gate[0].append(val)
        back.append([])
        for (_, op), gate in zip(ops[n:n + 4], gates):
            def tie(lhs, gate=gate):
                parts = [lhs[8 * i:8 * i + 8] for i in range(8)]
                for i, vals in enumerate(gate):
                    if vals:
                        both = functools.reduce(jnp.bitwise_or, [pltpu.bitcast(val, U32) for val in vals])
                        parts[i] = jnp.where(aid["never"], both, parts[i])
                return jnp.concatenate(parts, axis=0)

            out = op(tie)
            if out is not None:
                back[-1].append(out)
    assert not tasks and not queue
    for c in pending.values():
        c.wait()


@jax.jit
def pallas_concat_heads__ssm_conv_s5__ssm_conv_h3__prompt_kernel(
    A_x, A_Lambda_re, A_Lambda_im, A_B_re, A_B_im, A_C_re, A_C_im, A_log_dt, A_Dskip,
    B_q, B_k, B_v, B_shift_k, B_ssm_k, B_ssm_D,
):
    V = pltpu.VMEM
    scratch = [
        V((NJ, S, 128), BF16), V((NJ, S + HALO, 128), BF16), V((NJ, S, 128), BF16), V((NJ, S, 128), BF16),
        V((D, S), BF16), V((2, NJ, D, 128), BF16), V((2, NJ, D, 128), BF16),
        V((D,), BF16), V((D,), BF16), V((D,), BF16), V((D,), BF16), V((D,), BF16), V((4, D), BF16),
        V((2048, 128), BF16), pltpu.SMEM((1,), jnp.int32),
        V((NJ, 22, 8, 128), F32), V((2, 8, D), F32), V((6, 8, D), F32), V((4, T, 128), F32),
        V((NJ, S, 128), F32), V((NJ, S, 128), F32), V((16, 256, 128), F32),
        pltpu.SemaphoreType.DMA((12,)),
    ]
    scratch += [V((10, 2, 64, 128), U32)] * NP + [V((16, 64, 128), U32)] * NJ
    scratch += [V((7, NJ, 64, 128), U32)] * 3 + [V((7, NJ, T // 4, 128), U32)] * NP
    scratch += [V((4, 64, 128), U32)] * (2 * NP * NJ)
    scratch += [V((16, 256, 128), F32)] * (2 * NJ) + [V((NP, 4, 128, 128), U32)] * NJ
    scratch += [V((2, S, 128), F32)] * NJ
    out = pl.pallas_call(
        _kernel,
        out_shape=jax.ShapeDtypeStruct((S, 2 * D), F32),
        in_specs=[pl.BlockSpec(memory_space=pl.ANY)] * 17,
        out_specs=pl.BlockSpec(memory_space=pl.ANY),
        scratch_shapes=scratch,
        compiler_params=pltpu.CompilerParams(vmem_limit_bytes=110 * 1024 * 1024),
        name="s5_h3",
    )(A_x.reshape(S, D), A_Lambda_re, A_Lambda_im, A_B_re, A_B_im, A_C_re, A_C_im, A_log_dt, A_Dskip,
      B_q.reshape(S, D), B_k.reshape(S, D), B_v.reshape(S, D), B_shift_k.T, B_ssm_k, B_ssm_D,
      jnp.asarray(_dft_tables()), jnp.asarray(np.zeros((1,), np.int32)))
    return out.reshape(1, S, 2 * D)
```

```python
import functools

import numpy as np
import jax
import jax.numpy as jnp
from jax import lax
import jax.experimental.pallas as pl
import jax.experimental.pallas.tpu as pltpu

S, D = 2048, 640
T = 512
NP, NJ = 4, 5
HALO = 16
F32, BF16, U32 = jnp.float32, jnp.bfloat16, jnp.uint32
NT = (((1,), (1,)), ((), ()))
NN = (((1,), (0,)), ((), ()))
B_ROWS = (pl.ds(0, 128), pl.ds(128, 256), pl.ds(384, 256))

C_ROWS = (pl.ds(0, 256), pl.ds(256, 256), pl.ds(512, 128))

ORDER = ("W:x0c a0 W:b1 a1 a2 W:b2 W:x1 a3 a4 a5 a6 "
         "W:rows W:x2 W:kv0 a7 f0 a8 a9 a10 f1 a11 f2 f3 a12 a13 "
         "W:x3 W:kv1 W:kv2 W:ca a14 a15 f4 a16 f5 f6 a17 f7 f8 a18 a19 f9 f10 c0 f11 c2 "
         "W:cb W:kv3 W:kv4 W:g W:q c3 i0 i1 f12 c1 i2 f13 i3 f14 c4 f15 i4 f16 i5 f17 c5 f18 i6 f19 i7 "
         "c6 i8 i9 c7 i10 i11 c8 i12 i13 c9x i14 c9y i15 c9z i16 i17 c10x i18 c10y i19 c10z c11")
LOADS = "par b0 x0a x0b x0c b1 b2 x1 rows x2 kv0 x3 kv1 kv2 ca cb kv3 kv4 g q"
CFG = dict(
    ahead={"par": "b1", "x0c": "kv0", "b1": "kv1", "x1": "kv2", "kv0": "kv4", "x3": "q"},
    rate=70.0,
    cap=1.5,
    fwcost=40, ivcost=40, projcost=21,
    lag=8,
    early=16,
    quiet=8,
    scandue=80,
    gate=16, scangate=8, natlag=5, holdlag=3, scanlag=12,
)


def _dft_tables():
    g = np.arange(128)[:, None]
    m = np.arange(128)[None, :]
    fwd = np.zeros((4, 256, 128), np.float64)
    for r in range(4):
        th = np.pi * (((4 * g + 1) * (4 * m + r)) % 2048) / 1024.0
        c = np.cos(th).reshape(16, 8, 128)
        s = np.sin(th).reshape(16, 8, 128)
        fwd[r] = np.stack([c, s], axis=1).reshape(256, 128)
    inv = np.transpose(fwd, (0, 2, 1)) / 512.0
    perm = np.arange(128).reshape(8, 2, 8).transpose(0, 2, 1).reshape(128)
    fwd = fwd[:, :, perm]
    inv = inv.reshape(4, 128, 2, 128).transpose(0, 2, 1, 3)[..., perm]
    tab = np.concatenate([fwd.reshape(1024, 128), inv.reshape(1024, 128)], axis=0)
    tab = tab.reshape(64, 2, 8, 2, 128).transpose(0, 2, 1, 3, 4).reshape(2048, 128)
    return tab.astype(jnp.bfloat16)


def _lo(w):
    return pltpu.unpack_elementwise(w, index=0, packed_dtype=BF16, unpacked_dtype=F32)


def _hi(w):
    return pltpu.unpack_elementwise(w, index=1, packed_dtype=BF16, unpacked_dtype=F32)


def _pack(a, b):
    return pltpu.pack_elementwise([a, b], packed_dtype=BF16)


def _il(v):
    return pl.ds(16 * (v // 2) + v % 2, 8, stride=2)


def _get(ref, idx, v0):
    return jnp.concatenate([ref[idx + (_il(v), slice(None))] for v in range(v0, v0 + 8)], axis=0)


def _cmul(a, b):
    return a[0] * b[0] - a[1] * b[1], a[0] * b[1] + a[1] * b[0]


def _cadd(a, b):
    return a[0] + b[0], a[1] + b[1]


def _csub(a, b):
    return a[0] - b[0], a[1] - b[1]


def _lhs_sums(a11, a12, a21, a22):
    return a11 + a22, a21 + a22, a11 + a12, a21 - a11, a12 - a22


def _rhs_factors(b11, b12, b21, b22):
    return b11 + b22, b11, b12 - b22, b21 - b11, b22, b11 + b12, b21 + b22


def _load_groups():
    groups = {"par": ["lre", "lim", "ldt", "z"], "rows": ["dsk", "sd", "sh", "f"], "g": ["g"],
              "ca": [("c", g, c, j) for g in (0, 2) for j in range(NJ) for c in range(2)],
              "cb": [("c", 1, c, j) for j in range(NJ) for c in range(2)],
              "q": [("q", j) for j in range(NJ)],
              "x0a": [("x", 0, 0), ("x", 0, 2)], "x0b": [("x", 0, 1), ("x", 0, 3)], "x0c": [("x", 0, 4)]}
    for g in range(len(B_ROWS)):
        groups[f"b{g}"] = [("b", g, c, kt) for kt in range(NJ) for c in range(2)]
    for j in range(NJ):
        groups[f"kv{j}"] = [("k", j), ("v", j), ("ssm", j)]
    for p in range(1, NP):
        groups[f"x{p}"] = [("x", p, j) for j in range(NJ)]
    return groups


def _kernel(x_hbm, lre_hbm, lim_hbm, bre_hbm, bim_hbm, cre_hbm, cim_hbm, ldt_hbm, dsk_hbm,
            q_hbm, k_hbm, v_hbm, sh_hbm, ssm_hbm, sd_hbm, tab_hbm, z_hbm,
            o_hbm,
            xs, ks, vs, qs, ssm, bs, cs,
            lre_v, lim_v, ldt_v, dsk_v, sd_v, sh_v, tab_v, z_v,
            lamtab, fvec, rowp, kraw, oa, ob, wprev, sem, *rest):
    rest = list(rest)
    xsums, bfs, cps, hbs, kvbs, ktbs, uhs, khs, ybs, bus = (
        [rest.pop(0) for _ in range(n)] for n in (NP, NJ, 3, NP, NJ * NP, NJ * NP, NJ, NJ, NJ, NJ))

    def cols(j):
        return pl.ds(128 * j, 128)

    def rows(p):
        return pl.ds(T * p, T)

    copies = {"lre": (lre_hbm, lre_v), "lim": (lim_hbm, lim_v), "ldt": (ldt_hbm, ldt_v), "z": (z_hbm, z_v),
              "dsk": (dsk_hbm, dsk_v), "sd": (sd_hbm, sd_v), "sh": (sh_hbm, sh_v),
              "f": (tab_hbm.at[pl.ds(0, 1024), :], tab_v.at[pl.ds(0, 1024), :]),
              "g": (tab_hbm.at[pl.ds(1024, 1024), :], tab_v.at[pl.ds(1024, 1024), :])}
    for j in range(NJ):
        for c, (b_hbm, c_hbm) in enumerate(((bre_hbm, cre_hbm), (bim_hbm, cim_hbm))):
            for g, r in enumerate(C_ROWS):
                copies["c", g, c, j] = (c_hbm.at[r, cols(j)], cs.at[c, j, r, :])
            for g, r in enumerate(B_ROWS):
                copies["b", g, c, j] = (b_hbm.at[r, cols(j)], bs.at[c, j, r, :])
        copies["k", j] = (k_hbm.at[:, cols(j)], ks.at[j, pl.ds(HALO, S), :])
        copies["v", j] = (v_hbm.at[:, cols(j)], vs.at[j])
        copies["q", j] = (q_hbm.at[:, cols(j)], qs.at[j])
        copies["ssm", j] = (ssm_hbm.at[cols(j), :], ssm.at[cols(j), :])
        for p in range(NP):
            copies["x", p, j] = (x_hbm.at[rows(p), cols(j)], xs.at[j, rows(p), :])
            for g in range(2):
                r = pl.ds(T * p + T // 2 * g, T // 2)
                copies["oa", p, g, j] = (oa.at[j, r, :], o_hbm.at[r, cols(j)])
            copies["ob", p, j] = (ob.at[j, rows(p), :], o_hbm.at[rows(p), cols(NJ + j)])

    groups = _load_groups()
    words = ORDER.split()
    slot = {n: batch for batch, key in enumerate(("par", "b0", "x0a", "x0b")) for n in groups[key]}
    batch = 3
    for before, word in zip([""] + words, words):
        if word.startswith("W:"):
            batch += not before.startswith("W:")
            slot.update({n: batch for n in groups[word[2:]]})
    queue, pending = LOADS.split(), {}

    def start(name):
        c = pltpu.make_async_copy(*copies[name], sem.at[slot.get(name, batch + 1)])
        c.start()
        pending[name] = c

    def start_through(key):
        while key in queue:
            for name in groups[queue.pop(0)]:
                start(name)

    def wait(key):
        for name in groups[key]:
            pending.pop(name).wait()

    xw, kw, vw, qw, tabw, bw, cw = (r.bitcast(U32) for r in (xs, ks, vs, qs, tab_v, bs, cs))
    sub1 = lax.broadcasted_iota(jnp.int32, (8, 128), 0)

    def bcast(ref):
        return jnp.broadcast_to(ref[...].astype(F32).reshape(1, D), (8, D))

    def xvreg(p, j, b, m):
        return xw[j, pl.ds(T // 2 * p + 32 * b + m, 8, stride=4), :]

    aid = dict(never=None, scan=None, product=None)

    def hold(kind, ref, idx, stride):
        if aid[kind] is not None:
            r = idx + (stride, slice(None))
            ref[r] = jnp.where(aid["never"], aid[kind], ref[r])

    def discretise():
        lr, li = bcast(lre_v), bcast(lim_v)
        dt = jnp.exp(bcast(ldt_v)).astype(BF16).astype(F32)
        mag = jnp.exp(dt * lr)
        lam = (mag * jnp.cos(dt * li), mag * jnp.sin(dt * li))
        nr, ni = lam[0] - 1.0, lam[1]
        big = jnp.abs(lr) >= jnp.abs(li)
        ratio = jnp.where(big, li / lr, lr / li)
        den = jnp.where(big, lr + li * ratio, li + lr * ratio)
        fvec[0] = 2.0 * jnp.where(big, nr + ni * ratio, nr * ratio + ni) / den
        fvec[1] = 2.0 * jnp.where(big, ni - nr * ratio, ni * ratio - nr) / den
        pw = [lam]
        for i in range(1, 8):
            pw.append(_cmul(pw[(i - 1) // 2], pw[i - 1 - (i - 1) // 2]))
        mu1 = pw[7]
        mu2 = _cmul(mu1, mu1)
        mu4 = _cmul(mu2, mu2)
        sub = lax.broadcasted_iota(jnp.int32, (8, D), 0)
        tab = [c for z in pw for c in z]
        for d_, mu in ((1, mu1), (2, mu2), (4, mu4)):
            tab += [jnp.where(sub >= d_, mu[0], 0.0), jnp.where(sub >= d_, mu[1], 0.0)]
        for j in range(NJ):
            for i, t_ in enumerate(tab):
                lamtab[j, i] = t_[:, 128 * j:128 * (j + 1)]
            ks[j, pl.ds(0, HALO), :] = jnp.zeros((HALO, 128), BF16)

    def row_params():
        rowp[0] = bcast(dsk_v)
        rowp[1] = bcast(sd_v)
        sh = sh_v[...].astype(F32)
        for i in range(4):
            rowp[2 + i] = jnp.broadcast_to(sh[i:i + 1], (8, D))
        yield 100, []

    def x_sums(p, kts):
        for g in range(2):
            for kt in kts:
                for v in range(8):
                    blk = [xvreg(p, kt + 2 * cb, 4 * g + 2 * rb + v // 4, v % 4) for rb in range(2) for cb in range(2)]
                    lo, hi = _lhs_sums(*map(_lo, blk)), _lhs_sums(*map(_hi, blk))
                    ws = [_pack(a, b) for a, b in zip(lo, hi)]
                    for n, w in enumerate(ws):
                        xsums[p][5 * g + n, kt, _il(v), :] = w
                    yield 25, ws

    def b_factors(j):
        for s in range(8):
            r = pl.ds(64 * j + 8 * s, 8)
            for kt in range(2):
                blk = [bw[c, kt + 2 * kb, r, :] for kb in range(2) for c in range(2)]
                lo, hi = _rhs_factors(*map(_lo, blk)), _rhs_factors(*map(_hi, blk))
                ws = [blk[0] if n == 1 else blk[3] if n == 4 else _pack(lo[n], hi[n]) for n in range(7)]
                for n, w in enumerate(ws):
                    bfs[j][2 * n + kt, _il(s), :] = w
                bfs[j][14 + kt, _il(s), :] = bw[kt, 4, r, :]
                yield 34, [ws[n] for n in (0, 2, 3, 5, 6)]

    lasts = [None] * NJ

    def scan(p, j):
        def power(i):
            return lamtab[j, 2 * i], lamtab[j, 2 * i + 1]

        for b in range(T // 64):
            hold("scan", bus[j], (0,), pl.ds(T * p + 64 * b, 8, stride=9))
            hs = []
            for i in range(8):
                st = pl.ds(T * p + 64 * b + 16 * (i // 2) + (i % 2), 8, stride=2)
                u = (bus[j][0, st, :], bus[j][1, st, :])
                hs.append(u if i == 0 else _cadd(_cmul(power(0), hs[-1]), u))
            yield 58, list(hs[7]), CFG["scangate"]
            e = tuple(jnp.where(sub1 == 7, c0, c1) for c0, c1 in zip(lasts[j] or (0.0, 0.0), hs[7]))
            e = tuple(pltpu.roll(c, 1, 0) for c in e)
            for n, d_ in enumerate((1, 2, 4)):
                e = _cadd(e, _cmul(power(8 + n), tuple(pltpu.roll(c, d_, 0) for c in e)))
            yield 36, list(e), CFG["scangate"]
            for i0 in (1, 0):
                for i in range(i0, 8, 2):
                    hs[i] = _cadd(hs[i], _cmul(power(i), e))
                    if i == 7:
                        lasts[j] = hs[7]
                lo, hi = ([hs[i][c] for i in (i1, i1 + 2) for c in range(2)] for i1 in (i0, i0 + 4))
                lo, hi = (_lhs_sums(*blk) + (blk[0], blk[3]) for blk in (lo, hi))
                ws = [_pack(a_, b_) for a_, b_ in zip(lo, hi)]
                for n, w in enumerate(ws):
                    hbs[p][n, j, _il(2 * b + i0), :] = w
                yield 52, ws[:3], CFG["scangate"]

    def fold_c(j, i):
        f_r, f_i = fvec[0, :, cols(j)], fvec[1, :, cols(j)]
        f_n = -f_i

        def fold(d_, s):
            a, b = (cw[c, j, pl.ds(64 * d_ + 8 * s, 8), :] for c in range(2))
            return [(a_ * f_r - b_ * f_i, a_ * f_n - b_ * f_r) for a_, b_ in ((_lo(a), _lo(b)), (_hi(a), _hi(b)))]

        for s in range(8):
            if i < 2:
                fs = [_rhs_factors(r0, r1, i0, i1) for (r0, i0), (r1, i1) in zip(fold(2 * i, s), fold(2 * i + 1, s))]
            else:
                fs = [(r0 - i0, i0, r0) for r0, i0 in fold(4, s)]
            ws = [_pack(a_, b_) for a_, b_ in zip(*fs)]
            for n, w in enumerate(ws):
                cps[i][n, j, _il(s), :] = w
            yield (58, [ws[0], ws[5], ws[6]]) if i < 2 else (28, ws[:1])

    def prep_kv(j, p):
        for mb in range(8):
            w = [rowp[2 + i, :, cols(j)] for i in range(4)]
            outs = [[] for _ in range(4)]
            for hf in range(2):
                at = T // 2 * p + 32 * mb + 16 * hf
                p0, p1, w0, w1 = (kw[j, pl.ds(HALO // 2 + at + o, 8, stride=2), :] for o in (-2, -1, 0, 1))
                kk = [_hi(p0), _lo(p1), _hi(p1), _lo(w0), _hi(w0), _lo(w1), _hi(w1)]
                v0, v1 = (vw[j, pl.ds(at + o, 8, stride=2), :] for o in (0, 1))
                vv = [_lo(v0), _hi(v0), _lo(v1), _hi(v1)]
                for r in range(4):
                    ksh = (kk[r] * w[3] + kk[r + 1] * w[2]) + (kk[r + 2] * w[1] + kk[r + 3] * w[0])
                    outs[r].append(ksh * vv[r])
                if hf == 0:
                    yield 47, [outs[r][0] for r in range(4)]
            ws = [_pack(*outs[r]) for r in range(4)]
            for r in range(4):
                kvbs[j * NP + p][r, _il(mb), :] = ws[r]
            yield 51, ws

    def prep_filter(j, p):
        raw = kraw.at[(j * NP + p) % 4]
        for a in range(4):
            raw[pl.ds(128 * a, 128), :] = ssm[cols(j), pl.ds(T * p + 128 * a, 128)].astype(F32).T
            for mb in (2 * a, 2 * a + 1):
                ws = [_pack(raw[pl.ds(64 * mb + r, 8, stride=4), :], raw[pl.ds(64 * mb + 32 + r, 8, stride=4), :])
                      for r in range(4)]
                for r in range(4):
                    ktbs[j * NP + p][r, _il(mb), :] = ws[r]
                yield 16, ws

    def bin_(ref, i, h, n):
        return tuple(ref[i, pl.ds(64 * h + 16 * n + c, 8, stride=2), :] for c in range(2))

    def product(j, i, a, prev):
        half = []
        for hs in ((0, 2), (1, 3)):
            y = []
            for h in hs:
                w = None
                for n in range(a + 1):
                    t_ = _cmul(bin_(khs[j], i, h, n), bin_(uhs[j], i, h, a - n))
                    w = t_ if w is None else _cadd(w, t_)
                y.append((w[0] + prev[h][1], w[1] - prev[h][0]) if a else w)
                prev[h] = w
                if a > 1 and h == hs[0]:
                    yield 8 * a + 8, list(y[0])
            half += [_cadd(*y), _csub(*y)]
            if hs[0] == 0 and a:
                yield (8 * a + 14 if a > 1 else 38), list(half[0])
        p_, q_, s_, t_ = half
        res = [_cadd(p_, s_), (q_[0] + t_[1], q_[1] - t_[0]), _csub(p_, s_), (q_[0] - t_[1], q_[1] + t_[0])]
        ws = [_pack(*res[r]) for r in range(4)]
        for r in range(4):
            ybs[j][a, r, _il(i), :] = ws[r]
        yield (46, 50, 36, 44)[a], ws[:2]

    def products(j, blocks, groups_):
        for i in groups_:
            hold("product", uhs[j], (i,), pl.ds(0, 8, stride=33))
            prev = [bin_(wprev, i, h, blocks[0] - 1) if blocks[0] else None for h in range(4)]
            for a in blocks:
                yield from product(j, i, a, prev)
            if a < NP - 1:
                for h in range(4):
                    for c in range(2):
                        wprev[i, pl.ds(64 * h + 16 * a + c, 8, stride=2), :] = prev[h][c]

    def mm(tie, lhs, rhs, dims):
        return lax.dot_general(pltpu.bitcast(tie(lhs), BF16), pltpu.bitcast(rhs, BF16), dims,
                               preferred_element_type=F32)

    def program(steps):
        m = {}
        for key, lhs, rhs, then in steps:
            def op(tie, key=key, lhs=lhs, rhs=rhs, then=then):
                d_ = mm(tie, lhs(), rhs(), NT)
                m[key] = m[key] + d_ if key in m else d_
                out = m[key][120:128]
                if then is not None:
                    then(m)
                return out
            yield CFG["projcost"], op

    def project_in(p, j):
        for g in range(2):
            def plain(rb, kt, g=g):
                return lambda: jnp.concatenate(
                    [xvreg(p, kt, 4 * g + 2 * rb + v // 4, v % 4) for v in range(8)], axis=0)

            def put(rb, c, val, g=g):
                bus[j][c, pl.ds(T * p + 256 * g + 128 * rb, 128), :] = val

            def prod(n, key, then):
                def left(kt, g=g):
                    if n in (3, 4):
                        return plain(n - 3, 2 * (n - 3) + kt)
                    return lambda: _get(xsums[p], (5 * g + {1: 0, 2: 1, 5: 2, 6: 3, 7: 4}[n], kt), 0)
                return [(key, left(kt), lambda kt=kt: _get(bfs[j], (2 * (n - 1) + kt,), 0), then if kt else None)
                        for kt in range(2)]

            lead = p == 0 and j in (0, 1, 3) and g == 0

            def after4(m, put=put):
                put(0, 1, m[3] + m[5] + m["l01"])
                m["t10"] = m["l10"] + m[4]
                m["t00"] = m[4] - m[5]

            def after2(m, put=put):
                put(1, 0, m["t10"] + m[2])
                m["t11"] = m[3] - m[2]

            def after1(m):
                m["t00"] = m["t00"] + m[1]
                m["t11"] = m["t11"] + m[1]

            def finish(m, put=put):
                put(0, 0, m["t00"] + m["l00"])
                put(1, 1, m["t11"] + m["l11"])

            def fifth(key, rb, c, then=None):
                if lead:
                    return key, plain(rb, 4), lambda: bw[c, 4, pl.ds(64 * j, 64), :], then
                return key, plain(rb, 4), lambda: _get(bfs[j], (14 + c,), 0), then

            middle = (prod(4, 4, after4) + prod(2, 2, after2) + prod(1, 1, after1) + prod(7, "t00", None)
                      + prod(6, "t11", finish if lead else None))
            if lead:
                steps = ([fifth(f"l{rb}{c}", rb, c) for rb in range(2) for c in range(2)]
                         + prod(3, 3, None) + prod(5, 5, None) + middle)
            else:
                steps = (prod(3, 3, None) + prod(5, 5, None) + [fifth("l01", 0, 1), fifth("l10", 1, 0)] + middle
                         + [fifth("t00", 0, 0, lambda m, put=put: put(0, 0, m["t00"])),
                            fifth("t11", 1, 1, lambda m, put=put: put(1, 1, m["t11"]))])
            yield from program(steps)

    done = {}

    def project_out(p, unit, part):
        parts = [(0, unit, None), (1, unit, None), (0, 2, unit)] if unit < 2 else [(1, 2, 0), (1, 2, 1)]
        for g, i, half in [parts["xyz".index(part)]] if part else parts:
            def put(j, rb, val, g=g):
                dsk = rowp[0, :, cols(j)]
                for v in range(16):
                    step = 2 * rb + (v // 2) % 2
                    t0 = T * p + 64 * (4 * g + v // 4) + 32 * (v % 2) + step
                    w = xw[j, pl.ds(t0 // 2, 8, stride=2), :]
                    oa[j, pl.ds(t0, 8, stride=4), :] = val[8 * v:8 * v + 8] + (_hi(w) if step % 2 else _lo(w)) * dsk
                done[p, g, j] = done.get((p, g, j), 0) + 1
                if done[p, g, j] == 2:
                    start(("oa", p, g, j))

            def prod(ln, rn, key, then):
                return [(key, lambda kt=kt, g=g: _get(hbs[p], (ln, kt), 8 * g),
                         lambda kt=kt, i=i: _get(cps[i], (rn, kt), 0), then if kt == NJ - 1 else None)
                        for kt in range(NJ)]

            if i < 2:
                def after4(m):
                    m["t00"] = m[4] - m[5]

                def after2(m, put=put, i=i):
                    put(2 * i, 1, m[2] + m[4])
                    m["t11"] = m[3] - m[2]

                def after1(m):
                    m["t00"] = m["t00"] + m[1]
                    m["t11"] = m["t11"] + m[1]

                steps = (prod(5, 2, 3, None)
                         + prod(2, 4, 5, lambda m, put=put, i=i: put(2 * i + 1, 0, m[3] + m[5]))
                         + prod(6, 3, 4, after4) + prod(1, 1, 2, after2) + prod(0, 0, 1, after1)
                         + prod(4, 6, "t00", lambda m, put=put, i=i: put(2 * i, 0, m["t00"]))
                         + prod(3, 5, "t11", lambda m, put=put, i=i: put(2 * i + 1, 1, m["t11"])))
            elif half == 0:
                steps = prod(5, 0, 0, None) + prod(2, 1, 0, lambda m, put=put: put(4, 0, m[0]))
            else:
                steps = prod(6, 0, 0, None) + prod(1, 2, 1, lambda m, put=put: put(4, 1, m[1] - m[0]))
            yield from program(steps)

    def forward(j, p):
        for src, dst in ((kvbs[j * NP + p], uhs[j]), (ktbs[j * NP + p], khs[j])):
            for hf in range(2):
                v = []
                for r in range(4):
                    def op(tie, src=src, dst=dst, hf=hf, r=r, v=v):
                        v.append(mm(tie, _get(tabw, (), 16 * r + 8 * hf), _get(src, (r,), 0), NN))
                        if r < 3:
                            return None
                        for i in range(8):
                            z = [(v[n][16 * i:16 * i + 8], v[n][16 * i + 8:16 * i + 16]) for n in range(4)]
                            a, b = _cadd(z[0], z[2]), _csub(z[0], z[2])
                            if dst is khs[j] and p == 0:
                                tap = rowp[1, :, cols(j)]
                                a, b = (a[0] + tap, a[1]), (b[0] + tap, b[1])
                            c, d_ = _cadd(z[1], z[3]), _csub(z[1], z[3])
                            res = [_cadd(a, c), (b[0] - d_[1], b[1] + d_[0]), _csub(a, c), (b[0] + d_[1], b[1] - d_[0])]
                            for h in range(4):
                                for e in range(2):
                                    dst[8 * hf + i, pl.ds(64 * h + 16 * p + e, 8, stride=2), :] = res[h][e]
                        return res[3][1] + res[2][0]
                    yield CFG["fwcost"], op

    def inverse(j, a):
        for r in range(4):
            acc = []
            for kt in range(2):
                def op(tie, r=r, kt=kt, acc=acc):
                    acc.append(mm(tie, _get(tabw, (), 64 + 16 * r + 8 * kt), _get(ybs[j], (a, r), 8 * kt), NN))
                    if kt == 0:
                        return None
                    y = acc[0] + acc[1]
                    for mb in range(16):
                        w = qw[j, pl.ds(T // 2 * a + 16 * mb + r // 2, 8, stride=2), :]
                        out = (_hi(w) if r % 2 else _lo(w)) * y[8 * mb:8 * mb + 8]
                        ob[j, pl.ds(T * a + 32 * mb + r, 8, stride=4), :] = out
                    if r == 3:
                        start(("ob", a, j))
                    return out
                yield CFG["ivcost"], op

    ops, first, last, wait_at, waits = [], {}, {}, {}, {}
    for word in words:
        if word.startswith("W:"):
            wait_at[word[2:]] = len(ops)
            waits.setdefault(len(ops), []).append(word[2:])
            continue
        k = int(word[1:].rstrip("xyz"))
        make, unit = {"a": (project_in, divmod(k, NJ)), "c": (project_out, divmod(k, 3)),
                      "f": (forward, divmod(k, NP)), "i": (inverse, divmod(k, NP))}[word[0]]
        key = (word[0],) + unit
        first.setdefault(key, len(ops))
        ops += list(make(*unit, word[1:].lstrip("0123456789")) if word[0] == "c" else make(*unit))
        last[key] = len(ops)

    lag = CFG["lag"]
    tasks = [[wait_at["rows"] + 4, wait_at["rows"], 100, row_params()]]
    for p in range(NP):
        if p:
            tasks.append([first["a", p, 0], wait_at[f"x{p}"], 800, x_sums(p, (0, 1))])
        for j in range(NJ):
            due = min(first["c", p, i] for i in range(3)) - CFG["scandue"] * p
            tasks.append([due, last["a", p, j] + lag, 1584, scan(p, j)])
            tasks.append([first["f", j, p], max(wait_at[f"kv{j}"], wait_at["rows"] + 4), 784, prep_kv(j, p)])
            tasks.append([first["f", j, p] + 8, wait_at[f"kv{j}"], 128, prep_filter(j, p)])
    for j in range(NJ):
        if j:
            tasks.append([first["a", 0, j], wait_at[f"b{(j + 1) // 2}"], 512, b_factors(j)])
        for i in range(3):
            due = min(first["c", p, n] for p in range(NP) for n in ((0,), (1,), (0, 1, 2))[i])
            tasks.append([due, wait_at["cb" if i == 1 else "ca"], 464 if i < 2 else 224, fold_c(j, i)])
        ready = max(last["f", j, p] for p in range(NP)) + lag
        for blocks, part in ([((0, 1), range(16)), ((2,), range(16)), ((3,), range(16))] if j == NJ - 1 else
                             [((0, 1, 2, 3), range(4 * i, 4 * i + 4)) for i in range(4)]):
            cost = len(part) * sum((48, 90, 112, 152)[a] for a in blocks) if j == NJ - 1 else 1632
            tasks.append([min(first["i", j, a] for a in blocks), ready, cost, products(j, blocks, part)])
    tasks.sort(key=lambda t_: t_[0])
    cum = [0.0]
    for n, (c, _) in enumerate(ops):
        quiet = any(n + ahead in waits for ahead in range(1, CFG["quiet"] + 1))
        cum.append(cum[-1] + (0.0 if quiet else max(CFG["rate"] - c, 0.0)))

    start_through("x0c")
    wait("par")
    start_through(CFG["ahead"]["par"])
    aid["never"] = jnp.full((8, 128), z_v[0], jnp.int32) != 0
    discretise()
    for key, task in (("b0", b_factors(0)), ("x0a", x_sums(0, (0,))), ("x0b", x_sums(0, (1,)))):
        wait(key)
        for _ in task:
            pass

    budget, back, later = 0.0, [], {}
    for n in range(0, len(ops), 4):
        for key in waits.get(n, ()):
            wait(key)
        for key in waits.get(n, ()):
            later.clear()
            start_through(CFG["ahead"].get(key))
        room = cum[n + 4] - cum[n]
        need = max([0.0] + [sum(t2[2] for t2 in tasks[:i + 1]) / max(cum[max(t_[0] - CFG["early"], 0)] - cum[n], room, 1)
                            for i, t_ in enumerate(tasks)])
        budget = min(budget, 0.0) + room * min(need, CFG["cap"])
        for kind, behind in (("product", CFG["holdlag"]), ("scan", CFG["scanlag"])):
            aid[kind] = back[-behind][-1] if len(back) >= behind else None
        steps = []
        for t_ in list(tasks):
            urgent = t_[0] < n + 4
            if t_[1] > n and not urgent:
                continue
            while budget > 0 or urgent:
                step = next(t_[3], None)
                if step is None:
                    tasks.remove(t_)
                    break
                if not urgent:
                    budget -= step[0]
                    t_[2] -= step[0]
                    steps.append((step[0], step[1][-2:], sum(step[2:])))
        total, acc = sum(t_[0] for t_ in steps), 0
        for i, (cost, vals, slack) in enumerate(steps):
            acc += cost
            later.setdefault(2 * n + CFG["gate"] + slack + int(8 * acc / (total + 1)), []).append((i % 4, vals))
        gates = [[[] for _ in range(8)] for _ in range(4)]
        for pos in range(8):
            for i, vals in later.pop(2 * n + pos, ()):
                gates[i][pos] += vals
        if len(back) >= CFG["natlag"]:
            for gate, val in zip(gates, back[-CFG["natlag"]]):
                gate[0].append(val)
        back.append([])
        for (_, op), gate in zip(ops[n:n + 4], gates):
            def tie(lhs, gate=gate):
                parts = [lhs[8 * i:8 * i + 8] for i in range(8)]
                for i, vals in enumerate(gate):
                    if vals:
                        both = functools.reduce(jnp.bitwise_or, [pltpu.bitcast(val, U32) for val in vals])
                        parts[i] = jnp.where(aid["never"], both, parts[i])
                return jnp.concatenate(parts, axis=0)

            out = op(tie)
            if out is not None:
                back[-1].append(out)
    assert not tasks and not queue
    for c in pending.values():
        c.wait()


@jax.jit
def pallas_concat_heads__ssm_conv_s5__ssm_conv_h3__prompt_kernel(
    A_x, A_Lambda_re, A_Lambda_im, A_B_re, A_B_im, A_C_re, A_C_im, A_log_dt, A_Dskip,
    B_q, B_k, B_v, B_shift_k, B_ssm_k, B_ssm_D,
):
    V = pltpu.VMEM
    scratch = [
        V((NJ, S, 128), BF16), V((NJ, S + HALO, 128), BF16), V((NJ, S, 128), BF16), V((NJ, S, 128), BF16),
        V((D, S), BF16), V((2, NJ, D, 128), BF16), V((2, NJ, D, 128), BF16),
        V((D,), BF16), V((D,), BF16), V((D,), BF16), V((D,), BF16), V((D,), BF16), V((4, D), BF16),
        V((2048, 128), BF16), pltpu.SMEM((1,), jnp.int32),
        V((NJ, 22, 8, 128), F32), V((2, 8, D), F32), V((6, 8, D), F32), V((4, T, 128), F32),
        V((NJ, S, 128), F32), V((NJ, S, 128), F32), V((16, 256, 128), F32),
        pltpu.SemaphoreType.DMA((12,)),
    ]
    scratch += [V((10, 2, 64, 128), U32)] * NP + [V((16, 64, 128), U32)] * NJ
    scratch += [V((7, NJ, 64, 128), U32)] * 3 + [V((7, NJ, T // 4, 128), U32)] * NP
    scratch += [V((4, 64, 128), U32)] * (2 * NP * NJ)
    scratch += [V((16, 256, 128), F32)] * (2 * NJ) + [V((NP, 4, 128, 128), U32)] * NJ
    scratch += [V((2, S, 128), F32)] * NJ
    out = pl.pallas_call(
        _kernel,
        out_shape=jax.ShapeDtypeStruct((S, 2 * D), F32),
        in_specs=[pl.BlockSpec(memory_space=pl.ANY)] * 17,
        out_specs=pl.BlockSpec(memory_space=pl.ANY),
        scratch_shapes=scratch,
        compiler_params=pltpu.CompilerParams(vmem_limit_bytes=110 * 1024 * 1024),
        name="s5_h3",
    )(A_x.reshape(S, D), A_Lambda_re, A_Lambda_im, A_B_re, A_B_im, A_C_re, A_C_im, A_log_dt, A_Dskip,
      B_q.reshape(S, D), B_k.reshape(S, D), B_v.reshape(S, D), B_shift_k.T, B_ssm_k, B_ssm_D,
      jnp.asarray(_dft_tables()), jnp.asarray(np.zeros((1,), np.int32)))
    return out.reshape(1, S, 2 * D)
```

```python
import functools

import numpy as np
import jax
import jax.numpy as jnp
from jax import lax
import jax.experimental.pallas as pl
import jax.experimental.pallas.tpu as pltpu

S, D = 2048, 640
T = 512
NP, NJ = 4, 5
HALO = 16
F32, BF16, U32 = jnp.float32, jnp.bfloat16, jnp.uint32
NT = (((1,), (1,)), ((), ()))
NN = (((1,), (0,)), ((), ()))
B_ROWS = (pl.ds(0, 128), pl.ds(128, 256), pl.ds(384, 256))

C_ROWS = (pl.ds(0, 256), pl.ds(256, 256), pl.ds(512, 128))

ORDER = ("W:x0c a0 W:b1 a1 a2 W:b2 W:x1 a3 a4 a5 a6 "
         "W:rows W:x2 W:kv0 a7 f0 a8 a9 a10 f1 a11 f2 f3 a12 a13 "
         "W:x3 W:kv1 W:kv2 W:ca a14 a15 f4 a16 f5 a17 f6 f7 f8 a18 a19 f9 f10 c0 f11 c2 "
         "W:cb W:kv3 W:kv4 W:g W:q c3 i0 i1 f12 c1 i2 f13 i3 f14 f15 c4 i4 f16 i5 f17 f18 c5 i6 f19 "
         "c6 i7 i8 i9 i10 c7 i11 c8 i12 i13 c9x i14 c9y i15 c9z i16 i17 c10x i18 c10y i19 c10z c11")
LOADS = "par b0 x0a x0b x0c b1 b2 x1 rows x2 kv0 x3 kv1 kv2 ca cb kv3 kv4 g q"
CFG = dict(
    ahead={"par": "b1", "x0c": "kv0", "b1": "kv1", "x1": "kv2", "kv0": "kv4", "x3": "q"},
    rate=70.0,
    cap=1.5,
    fwcost=40, ivcost=40, projcost=21,
    lag=8,
    early=16,
    quiet=8,
    scandue=80,
    gate=16, scangate=8, natlag=5, holdlag=3, scanlag=12,
)


def _dft_tables():
    g = np.arange(128)[:, None]
    m = np.arange(128)[None, :]
    fwd = np.zeros((4, 256, 128), np.float64)
    for r in range(4):
        th = np.pi * (((4 * g + 1) * (4 * m + r)) % 2048) / 1024.0
        c = np.cos(th).reshape(16, 8, 128)
        s = np.sin(th).reshape(16, 8, 128)
        fwd[r] = np.stack([c, s], axis=1).reshape(256, 128)
    inv = np.transpose(fwd, (0, 2, 1)) / 512.0
    perm = np.arange(128).reshape(4, 8, 2, 2).transpose(0, 2, 1, 3).reshape(128)
    fwd = fwd[:, :, perm]
    inv = inv.reshape(4, 128, 2, 128).transpose(0, 2, 1, 3)[..., perm]
    tab = np.concatenate([fwd.reshape(1024, 128), inv.reshape(1024, 128)], axis=0)
    tab = tab.reshape(64, 2, 8, 2, 128).transpose(0, 2, 1, 3, 4).reshape(2048, 128)
    return tab.astype(jnp.bfloat16)


def _lo(w):
    return pltpu.bitcast(w << 16, F32)


def _hi(w):
    return pltpu.bitcast(w & jnp.uint32(0xFFFF0000), F32)


def _rows16(a, b):
    return jnp.concatenate([a, b], axis=0).astype(BF16)


def _il(v):
    return pl.ds(16 * (v // 2) + v % 2, 8, stride=2)


def _get(ref, idx, v0):
    return jnp.concatenate([ref[idx + (_il(v), slice(None))] for v in range(v0, v0 + 8)], axis=0)


def _cmul(a, b):
    return a[0] * b[0] - a[1] * b[1], a[0] * b[1] + a[1] * b[0]


def _cadd(a, b):
    return a[0] + b[0], a[1] + b[1]


def _csub(a, b):
    return a[0] - b[0], a[1] - b[1]


def _lhs_sums(a11, a12, a21, a22):
    return a11 + a22, a21 + a22, a11 + a12, a21 - a11, a12 - a22


def _rhs_factors(b11, b12, b21, b22):
    return b11 + b22, b11, b12 - b22, b21 - b11, b22, b11 + b12, b21 + b22


def _load_groups():
    groups = {"par": ["lre", "lim", "ldt", "z"], "rows": ["dsk", "sd", "sh", "f"], "g": ["g"],
              "ca": [("c", g, c, j) for g in (0, 2) for j in range(NJ) for c in range(2)],
              "cb": [("c", 1, c, j) for j in range(NJ) for c in range(2)],
              "q": [("q", j) for j in range(NJ)],
              "x0a": [("x", 0, 0), ("x", 0, 2)], "x0b": [("x", 0, 1), ("x", 0, 3)], "x0c": [("x", 0, 4)]}
    for g in range(len(B_ROWS)):
        groups[f"b{g}"] = [("b", g, c, kt) for kt in range(NJ) for c in range(2)]
    for j in range(NJ):
        groups[f"kv{j}"] = [("k", j), ("v", j), ("ssm", j)]
    for p in range(1, NP):
        groups[f"x{p}"] = [("x", p, j) for j in range(NJ)]
    return groups


def _kernel(x_hbm, lre_hbm, lim_hbm, bre_hbm, bim_hbm, cre_hbm, cim_hbm, ldt_hbm, dsk_hbm,
            q_hbm, k_hbm, v_hbm, sh_hbm, ssm_hbm, sd_hbm, tab_hbm, z_hbm,
            o_hbm,
            xs, ks, vs, qs, ssm, bs, cs,
            lre_v, lim_v, ldt_v, dsk_v, sd_v, sh_v, tab_v, z_v,
            lamtab, fvec, rowp, kraw, oa, ob, wprev, sem, *rest):
    rest = list(rest)
    xsums, bfs, cps, hbs, kvbs, ktbs, uhs, khs, ybs, bus = (
        [rest.pop(0) for _ in range(n)] for n in (NP, NJ, 3, NP, NJ * NP, NJ * NP, NJ, NJ, NJ, NJ))

    def cols(j):
        return pl.ds(128 * j, 128)

    def rows(p):
        return pl.ds(T * p, T)

    copies = {"lre": (lre_hbm, lre_v), "lim": (lim_hbm, lim_v), "ldt": (ldt_hbm, ldt_v), "z": (z_hbm, z_v),
              "dsk": (dsk_hbm, dsk_v), "sd": (sd_hbm, sd_v), "sh": (sh_hbm, sh_v),
              "f": (tab_hbm.at[pl.ds(0, 1024), :], tab_v.at[pl.ds(0, 1024), :]),
              "g": (tab_hbm.at[pl.ds(1024, 1024), :], tab_v.at[pl.ds(1024, 1024), :])}
    for j in range(NJ):
        for c, (b_hbm, c_hbm) in enumerate(((bre_hbm, cre_hbm), (bim_hbm, cim_hbm))):
            for g, r in enumerate(C_ROWS):
                copies["c", g, c, j] = (c_hbm.at[r, cols(j)], cs.at[c, j, r, :])
            for g, r in enumerate(B_ROWS):
                copies["b", g, c, j] = (b_hbm.at[r, cols(j)], bs.at[c, j, r, :])
        copies["k", j] = (k_hbm.at[:, cols(j)], ks.at[j, pl.ds(HALO, S), :])
        copies["v", j] = (v_hbm.at[:, cols(j)], vs.at[j])
        copies["q", j] = (q_hbm.at[:, cols(j)], qs.at[j])
        copies["ssm", j] = (ssm_hbm.at[cols(j), :], ssm.at[cols(j), :])
        for p in range(NP):
            copies["x", p, j] = (x_hbm.at[rows(p), cols(j)], xs.at[j, rows(p), :])
            for g in range(2):
                r = pl.ds(T * p + T // 2 * g, T // 2)
                copies["oa", p, g, j] = (oa.at[j, r, :], o_hbm.at[r, cols(j)])
            copies["ob", p, j] = (ob.at[j, rows(p), :], o_hbm.at[rows(p), cols(NJ + j)])

    groups = _load_groups()
    words = ORDER.split()
    slot = {n: batch for batch, key in enumerate(("par", "b0", "x0a", "x0b")) for n in groups[key]}
    batch = 3
    for before, word in zip([""] + words, words):
        if word.startswith("W:"):
            batch += not before.startswith("W:")
            slot.update({n: batch for n in groups[word[2:]]})
    queue, pending = LOADS.split(), {}

    def start(name):
        c = pltpu.make_async_copy(*copies[name], sem.at[slot.get(name, batch + 1)])
        c.start()
        pending[name] = c

    def start_through(key):
        while key in queue:
            for name in groups[queue.pop(0)]:
                start(name)

    def wait(key):
        for name in groups[key]:
            pending.pop(name).wait()

    xw, kw, vw, qw, tabw, bw = (r.bitcast(U32) for r in (xs, ks, vs, qs, tab_v, bs))
    sub1 = lax.broadcasted_iota(jnp.int32, (8, 128), 0)

    def bcast(ref):
        return jnp.broadcast_to(ref[...].astype(F32).reshape(1, D), (8, D))

    def xvreg(p, j, b, m):
        return xw[j, pl.ds(T // 2 * p + 32 * b + m, 8, stride=4), :]

    def xrows(p, j, rb):
        return jnp.concatenate([xw[j, _il(T // 16 * p + 8 * rb + v), :] for v in (0, 2, 1, 3, 4, 6, 5, 7)], axis=0)

    aid = dict(never=None, scan=None, product=None)

    def hold(kind, ref, idx, stride):
        if aid[kind] is not None:
            r = idx + (stride, slice(None))
            ref[r] = jnp.where(aid["never"], aid[kind], ref[r])

    def discretise():
        lr, li = bcast(lre_v), bcast(lim_v)
        dt = jnp.exp(bcast(ldt_v)).astype(BF16).astype(F32)
        mag = jnp.exp(dt * lr)
        lam = (mag * jnp.cos(dt * li), mag * jnp.sin(dt * li))
        nr, ni = lam[0] - 1.0, lam[1]
        big = jnp.abs(lr) >= jnp.abs(li)
        ratio = jnp.where(big, li / lr, lr / li)
        den = jnp.where(big, lr + li * ratio, li + lr * ratio)
        fvec[0] = 2.0 * jnp.where(big, nr + ni * ratio, nr * ratio + ni) / den
        fvec[1] = 2.0 * jnp.where(big, ni - nr * ratio, ni * ratio - nr) / den
        pw = [lam]
        for i in range(1, 8):
            pw.append(_cmul(pw[(i - 1) // 2], pw[i - 1 - (i - 1) // 2]))
        mu1 = pw[7]
        mu2 = _cmul(mu1, mu1)
        mu4 = _cmul(mu2, mu2)
        sub = lax.broadcasted_iota(jnp.int32, (8, D), 0)
        tab = [c for z in pw for c in z]
        for d_, mu in ((1, mu1), (2, mu2), (4, mu4)):
            tab += [jnp.where(sub >= d_, mu[0], 0.0), jnp.where(sub >= d_, mu[1], 0.0)]
        for j in range(NJ):
            for i, t_ in enumerate(tab):
                lamtab[j, i] = t_[:, 128 * j:128 * (j + 1)]
            ks[j, pl.ds(0, HALO), :] = jnp.zeros((HALO, 128), BF16)

    def row_params():
        rowp[0] = bcast(dsk_v)
        rowp[1] = bcast(sd_v)
        sh = sh_v[...].astype(F32)
        for i in range(4):
            rowp[2 + i] = jnp.broadcast_to(sh[i:i + 1], (8, D))
        yield 100, []

    def x_sums(p, kts):
        for g in range(2):
            for kt in kts:
                for v in range(8):
                    fs = _lhs_sums(*(
                        pltpu.bitcast(xw[kt + 2 * cb, pl.ds(T // 2 * p + 64 * rb + 8 * v, 8), :], BF16).astype(F32)
                        for rb in (2 * g, 2 * g + 1) for cb in range(2)))
                    for n, f in enumerate(fs):
                        xsums[p][5 * g + n, kt, pl.ds(16 * v, 16), :] = f.astype(BF16)
                    yield 25, [f[8:] for f in fs]

    def b_factors(j):
        for s in range(8):
            r = pl.ds(128 * j + 16 * s, 16)
            for kt in range(2):
                fs = _rhs_factors(*(bs[c, kt + 2 * kb, r, :].astype(F32) for kb in range(2) for c in range(2)))
                for n, f in enumerate(fs):
                    bfs[j][2 * n + kt, pl.ds(16 * s, 16), :] = f.astype(BF16)
                yield 34, [fs[n][8:] for n in (0, 2, 3, 5, 6)]

    lasts = [None] * NJ

    def scan(p, j):
        def power(i):
            return lamtab[j, 2 * i], lamtab[j, 2 * i + 1]

        for b in range(T // 64):
            hold("scan", bus[j], (0,), pl.ds(T * p + 64 * b, 8, stride=9))
            hs = []
            for i in range(8):
                st = pl.ds(T * p + 64 * b + 32 * ((i // 2) % 2) + 2 * (i // 4) + i % 2, 8, stride=4)
                u = (bus[j][0, st, :], bus[j][1, st, :])
                hs.append(u if i == 0 else _cadd(_cmul(power(0), hs[-1]), u))
            yield 58, list(hs[7]), CFG["scangate"]
            e = tuple(jnp.where(sub1 == 7, c0, c1) for c0, c1 in zip(lasts[j] or (0.0, 0.0), hs[7]))
            e = tuple(pltpu.roll(c, 1, 0) for c in e)
            for n, d_ in enumerate((1, 2, 4)):
                e = _cadd(e, _cmul(power(8 + n), tuple(pltpu.roll(c, d_, 0) for c in e)))
            yield 36, list(e), CFG["scangate"]
            for i0 in (1, 0):
                for i in range(i0, 8, 2):
                    hs[i] = _cadd(hs[i], _cmul(power(i), e))
                    if i == 7:
                        lasts[j] = hs[7]
                blk = [jnp.concatenate([hs[i][c], hs[i + 4][c]], axis=0) for i in (i0, i0 + 2) for c in range(2)]
                fs = _lhs_sums(*blk) + (blk[0], blk[3])
                for n, f in enumerate(fs):
                    hbs[p][n, j, pl.ds(32 * b + 16 * i0, 16), :] = f.astype(BF16)
                yield 52, [fs[0][8:], fs[1][:8], fs[4][8:]], CFG["scangate"]

    def fold_c(j, i):
        f_r, f_i = (jnp.concatenate([fvec[c, :, cols(j)]] * 2, axis=0) for c in range(2))
        f_n = -f_i

        def fold(d_, s):
            a, b = (cs[c, j, pl.ds(128 * d_ + 16 * s, 16), :].astype(F32) for c in range(2))
            return a * f_r - b * f_i, a * f_n - b * f_r

        for s in range(8):
            if i < 2:
                (r0, i0), (r1, i1) = fold(2 * i, s), fold(2 * i + 1, s)
                fs = _rhs_factors(r0, r1, i0, i1)
            else:
                r0, i0 = fold(4, s)
                fs = (r0 - i0, i0, r0)
            for n, f in enumerate(fs):
                cps[i][n, j, pl.ds(16 * s, 16), :] = f.astype(BF16)
            yield (58, [fs[0][8:], fs[5][:8], fs[6][8:]]) if i < 2 else (28, [fs[0][8:]])

    def prep_kv(j, p):
        for mb in range(8):
            w = [rowp[2 + i, :, cols(j)] for i in range(4)]
            outs = [[] for _ in range(4)]
            for hf in range(2):
                at = T // 2 * p + 32 * mb + 16 * hf
                p0, p1, w0, w1 = (kw[j, pl.ds(HALO // 2 + at + o, 8, stride=2), :] for o in (-2, -1, 0, 1))
                kk = [_hi(p0), _lo(p1), _hi(p1), _lo(w0), _hi(w0), _lo(w1), _hi(w1)]
                v0, v1 = (vw[j, pl.ds(at + o, 8, stride=2), :] for o in (0, 1))
                vv = [_lo(v0), _hi(v0), _lo(v1), _hi(v1)]
                for r in range(4):
                    ksh = (kk[r] * w[3] + kk[r + 1] * w[2]) + (kk[r + 2] * w[1] + kk[r + 3] * w[0])
                    outs[r].append(ksh * vv[r])
                if hf == 0:
                    yield 47, [outs[r][0] for r in range(4)]
            for r in range(4):
                kvbs[j * NP + p][r, pl.ds(16 * mb, 16), :] = _rows16(*outs[r])
            yield 51, [outs[r][1] for r in range(4)]

    def prep_filter(j, p):
        raw = kraw.at[(j * NP + p) % 4]
        for a in range(4):
            raw[pl.ds(128 * a, 128), :] = ssm[cols(j), pl.ds(T * p + 128 * a, 128)].astype(F32).T
            for mb in (2 * a, 2 * a + 1):
                ws = [raw[pl.ds(64 * mb + r, 16, stride=4), :] for r in range(4)]
                for r in range(4):
                    ktbs[j * NP + p][r, pl.ds(16 * mb, 16), :] = ws[r].astype(BF16)
                yield 16, [w[8:] for w in ws]

    def bin_(ref, i, h, n):
        return tuple(ref[i, pl.ds(64 * h + 16 * n + c, 8, stride=2), :] for c in range(2))

    def product(j, i, a, prev):
        half = []
        for hs in ((0, 2), (1, 3)):
            y = []
            for h in hs:
                w = None
                for n in range(a + 1):
                    t_ = _cmul(bin_(khs[j], i, h, n), bin_(uhs[j], i, h, a - n))
                    w = t_ if w is None else _cadd(w, t_)
                y.append((w[0] + prev[h][1], w[1] - prev[h][0]) if a else w)
                prev[h] = w
                if a > 1 and h == hs[0]:
                    yield 8 * a + 8, list(y[0])
            half += [_cadd(*y), _csub(*y)]
            if hs[0] == 0 and a:
                yield (8 * a + 14 if a > 1 else 38), list(half[0])
        p_, q_, s_, t_ = half
        res = [_cadd(p_, s_), (q_[0] + t_[1], q_[1] - t_[0]), _csub(p_, s_), (q_[0] - t_[1], q_[1] + t_[0])]
        for r in range(4):
            ybs[j][a, r, pl.ds(16 * i, 16), :] = _rows16(*res[r])
        yield (46, 50, 36, 44)[a], [res[0][1], res[1][0]]

    def products(j, blocks, groups_):
        for i in groups_:
            hold("product", uhs[j], (i,), pl.ds(0, 8, stride=33))
            prev = [bin_(wprev, i, h, blocks[0] - 1) if blocks[0] else None for h in range(4)]
            for a in blocks:
                yield from product(j, i, a, prev)
            if a < NP - 1:
                for h in range(4):
                    for c in range(2):
                        wprev[i, pl.ds(64 * h + 16 * a + c, 8, stride=2), :] = prev[h][c]

    def mm(tie, lhs, rhs, dims):
        return lax.dot_general(pltpu.bitcast(tie(lhs), BF16), pltpu.bitcast(rhs, BF16), dims,
                               preferred_element_type=F32)

    def program(steps):
        m = {}
        for key, lhs, rhs, then in steps:
            def op(tie, key=key, lhs=lhs, rhs=rhs, then=then):
                d_ = mm(tie, lhs(), rhs(), NT)
                m[key] = m[key] + d_ if key in m else d_
                out = m[key][120:128]
                if then is not None:
                    then(m)
                return out
            yield CFG["projcost"], op

    def project_in(p, j):
        for g in range(2):
            def plain(rb, kt, g=g):
                return lambda: xrows(p, kt, 2 * g + rb)

            def put(rb, c, val, g=g):
                bus[j][c, pl.ds(T * p + 256 * g + 128 * rb, 128), :] = val

            def prod(n, key, then):
                def left(kt, g=g):
                    if n in (3, 4):
                        return plain(n - 3, 2 * (n - 3) + kt)
                    at = (5 * g + {1: 0, 2: 1, 5: 2, 6: 3, 7: 4}[n], kt)
                    return lambda: jnp.concatenate(
                        [xsums[p].bitcast(U32)[at + (_il(v), slice(None))] for v in (0, 2, 1, 3, 4, 6, 5, 7)], axis=0)
                return [(key, left(kt), lambda kt=kt: bfs[j].bitcast(U32)[2 * (n - 1) + kt], then if kt else None)
                        for kt in range(2)]

            lead = p == 0 and j in (0, 1, 3) and g == 0

            def after4(m, put=put):
                put(0, 1, m[3] + m[5] + m["l01"])
                m["t10"] = m["l10"] + m[4]
                m["t00"] = m[4] - m[5]

            def after2(m, put=put):
                put(1, 0, m["t10"] + m[2])
                m["t11"] = m[3] - m[2]

            def after1(m):
                m["t00"] = m["t00"] + m[1]
                m["t11"] = m["t11"] + m[1]

            def finish(m, put=put):
                put(0, 0, m["t00"] + m["l00"])
                put(1, 1, m["t11"] + m["l11"])

            def fifth(key, rb, c, then=None):
                return key, plain(rb, 4), lambda: bw[c, 4, pl.ds(64 * j, 64), :], then

            middle = (prod(4, 4, after4) + prod(2, 2, after2) + prod(1, 1, after1) + prod(7, "t00", None)
                      + prod(6, "t11", finish if lead else None))
            if lead:
                steps = ([fifth(f"l{rb}{c}", rb, c) for rb in range(2) for c in range(2)]
                         + prod(3, 3, None) + prod(5, 5, None) + middle)
            else:
                steps = (prod(3, 3, None) + prod(5, 5, None) + [fifth("l01", 0, 1), fifth("l10", 1, 0)] + middle
                         + [fifth("t00", 0, 0, lambda m, put=put: put(0, 0, m["t00"])),
                            fifth("t11", 1, 1, lambda m, put=put: put(1, 1, m["t11"]))])
            yield from program(steps)

    done = {}

    def project_out(p, unit, part):
        parts = [(0, unit, None), (1, unit, None), (0, 2, unit)] if unit < 2 else [(1, 2, 0), (1, 2, 1)]
        for g, i, half in [parts["xyz".index(part)]] if part else parts:
            def put(j, rb, val, g=g):
                dsk = rowp[0, :, cols(j)]
                for blk in range(4):
                    for late in range(2):
                        w = xvreg(p, j, 4 * g + blk, rb + 2 * late)
                        for i0, xv in enumerate((_lo(w), _hi(w))):
                            t0 = T * p + 64 * (4 * g + blk) + 2 * rb + 4 * late + i0
                            v = 4 * blk + 2 * i0 + late
                            oa[j, pl.ds(t0, 8, stride=8), :] = val[8 * v:8 * v + 8] + xv * dsk
                done[p, g, j] = done.get((p, g, j), 0) + 1
                if done[p, g, j] == 2:
                    start(("oa", p, g, j))

            def prod(ln, rn, key, then):
                return [(key, lambda kt=kt, g=g: hbs[p].bitcast(U32)[ln, kt, pl.ds(64 * g, 64), :],
                         lambda kt=kt, i=i: cps[i].bitcast(U32)[rn, kt], then if kt == NJ - 1 else None)
                        for kt in range(NJ)]

            if i < 2:
                def after4(m):
                    m["t00"] = m[4] - m[5]

                def after2(m, put=put, i=i):
                    put(2 * i, 1, m[2] + m[4])
                    m["t11"] = m[3] - m[2]

                def after1(m):
                    m["t00"] = m["t00"] + m[1]
                    m["t11"] = m["t11"] + m[1]

                steps = (prod(5, 2, 3, None)
                         + prod(2, 4, 5, lambda m, put=put, i=i: put(2 * i + 1, 0, m[3] + m[5]))
                         + prod(6, 3, 4, after4) + prod(1, 1, 2, after2) + prod(0, 0, 1, after1)
                         + prod(4, 6, "t00", lambda m, put=put, i=i: put(2 * i, 0, m["t00"]))
                         + prod(3, 5, "t11", lambda m, put=put, i=i: put(2 * i + 1, 1, m["t11"])))
            elif half == 0:
                steps = prod(5, 0, 0, None) + prod(2, 1, 0, lambda m, put=put: put(4, 0, m[0]))
            else:
                steps = prod(6, 0, 0, None) + prod(1, 2, 1, lambda m, put=put: put(4, 1, m[1] - m[0]))
            yield from program(steps)

    def forward(j, p):
        for src, dst in ((kvbs[j * NP + p], uhs[j]), (ktbs[j * NP + p], khs[j])):
            for hf in range(2):
                v = []
                for r in range(4):
                    def op(tie, src=src, dst=dst, hf=hf, r=r, v=v):
                        v.append(mm(tie, _get(tabw, (), 16 * r + 8 * hf), _get(src.bitcast(U32), (r,), 0), NN))
                        if r < 3:
                            return None
                        for i in range(8):
                            z = [(v[n][16 * i:16 * i + 8], v[n][16 * i + 8:16 * i + 16]) for n in range(4)]
                            a, b = _cadd(z[0], z[2]), _csub(z[0], z[2])
                            if dst is khs[j] and p == 0:
                                tap = rowp[1, :, cols(j)]
                                a, b = (a[0] + tap, a[1]), (b[0] + tap, b[1])
                            c, d_ = _cadd(z[1], z[3]), _csub(z[1], z[3])
                            res = [_cadd(a, c), (b[0] - d_[1], b[1] + d_[0]), _csub(a, c), (b[0] + d_[1], b[1] - d_[0])]
                            for h in range(4):
                                for e in range(2):
                                    dst[8 * hf + i, pl.ds(64 * h + 16 * p + e, 8, stride=2), :] = res[h][e]
                        return res[3][1] + res[2][0]
                    yield CFG["fwcost"], op

    def inverse(j, a):
        for r in range(4):
            acc = []
            for kt in range(2):
                def op(tie, r=r, kt=kt, acc=acc):
                    acc.append(mm(tie, _get(tabw, (), 64 + 16 * r + 8 * kt), _get(ybs[j].bitcast(U32), (a, r), 8 * kt), NN))
                    if kt == 0:
                        return None
                    y = acc[0] + acc[1]
                    for mb in range(16):
                        w = qw[j, pl.ds(T // 2 * a + 16 * mb + r // 2, 8, stride=2), :]
                        out = (_hi(w) if r % 2 else _lo(w)) * y[8 * mb:8 * mb + 8]
                        ob[j, pl.ds(T * a + 32 * mb + r, 8, stride=4), :] = out
                    if r == 3:
                        start(("ob", a, j))
                    return out
                yield CFG["ivcost"], op

    ops, first, last, wait_at, waits = [], {}, {}, {}, {}
    for word in words:
        if word.startswith("W:"):
            wait_at[word[2:]] = len(ops)
            waits.setdefault(len(ops), []).append(word[2:])
            continue
        k = int(word[1:].rstrip("xyz"))
        make, unit = {"a": (project_in, divmod(k, NJ)), "c": (project_out, divmod(k, 3)),
                      "f": (forward, divmod(k, NP)), "i": (inverse, divmod(k, NP))}[word[0]]
        key = (word[0],) + unit
        first.setdefault(key, len(ops))
        ops += list(make(*unit, word[1:].lstrip("0123456789")) if word[0] == "c" else make(*unit))
        last[key] = len(ops)

    lag = CFG["lag"]
    tasks = [[wait_at["rows"] + 4, wait_at["rows"], 100, row_params()]]
    for p in range(NP):
        if p:
            tasks.append([first["a", p, 0], wait_at[f"x{p}"], 800, x_sums(p, (0, 1))])
        for j in range(NJ):
            due = min(first["c", p, i] for i in range(3)) - CFG["scandue"] * p
            tasks.append([due, last["a", p, j] + lag, 1584, scan(p, j)])
            tasks.append([first["f", j, p], max(wait_at[f"kv{j}"], wait_at["rows"] + 4), 784, prep_kv(j, p)])
            tasks.append([first["f", j, p] + 8, wait_at[f"kv{j}"], 128, prep_filter(j, p)])
    for j in range(NJ):
        if j:
            tasks.append([first["a", 0, j], wait_at[f"b{(j + 1) // 2}"], 512, b_factors(j)])
        for i in range(3):
            due = min(first["c", p, n] for p in range(NP) for n in ((0,), (1,), (0, 1, 2))[i])
            tasks.append([due, wait_at["cb" if i == 1 else "ca"], 464 if i < 2 else 224, fold_c(j, i)])
        ready = max(last["f", j, p] for p in range(NP)) + lag
        for blocks, part in ([((0, 1), range(16)), ((2,), range(16)), ((3,), range(16))] if j == NJ - 1 else
                             [((0, 1, 2, 3), range(4 * i, 4 * i + 4)) for i in range(4)]):
            cost = len(part) * sum((48, 90, 112, 152)[a] for a in blocks) if j == NJ - 1 else 1632
            tasks.append([min(first["i", j, a] for a in blocks), ready, cost, products(j, blocks, part)])
    tasks.sort(key=lambda t_: t_[0])
    cum = [0.0]
    for n, (c, _) in enumerate(ops):
        quiet = any(n + ahead in waits for ahead in range(1, CFG["quiet"] + 1))
        cum.append(cum[-1] + (0.0 if quiet else max(CFG["rate"] - c, 0.0)))

    start_through("x0c")
    wait("par")
    start_through(CFG["ahead"]["par"])
    aid["never"] = jnp.full((8, 128), z_v[0], jnp.int32) != 0
    discretise()
    for key, task in (("b0", b_factors(0)), ("x0a", x_sums(0, (0,))), ("x0b", x_sums(0, (1,)))):
        wait(key)
        for _ in task:
            pass

    budget, back, later = 0.0, [], {}
    for n in range(0, len(ops), 4):
        for key in waits.get(n, ()):
            wait(key)
        for key in waits.get(n, ()):
            later.clear()
            start_through(CFG["ahead"].get(key))
        room = cum[n + 4] - cum[n]
        need = max([0.0] + [sum(t2[2] for t2 in tasks[:i + 1]) / max(cum[max(t_[0] - CFG["early"], 0)] - cum[n], room, 1)
                            for i, t_ in enumerate(tasks)])
        budget = min(budget, 0.0) + room * min(need, CFG["cap"])
        for kind, behind in (("product", CFG["holdlag"]), ("scan", CFG["scanlag"])):
            aid[kind] = back[-behind][-1] if len(back) >= behind else None
        steps = []
        for t_ in list(tasks):
            urgent = t_[0] < n + 4
            if t_[1] > n and not urgent:
                continue
            while budget > 0 or urgent:
                step = next(t_[3], None)
                if step is None:
                    tasks.remove(t_)
                    break
                if not urgent:
                    budget -= step[0]
                    t_[2] -= step[0]
                    steps.append((step[0], step[1][-2:], sum(step[2:])))
        total, acc = sum(t_[0] for t_ in steps), 0
        for i, (cost, vals, slack) in enumerate(steps):
            acc += cost
            later.setdefault(2 * n + CFG["gate"] + slack + int(8 * acc / (total + 1)), []).append((i % 4, vals))
        gates = [[[] for _ in range(8)] for _ in range(4)]
        for pos in range(8):
            for i, vals in later.pop(2 * n + pos, ()):
                gates[i][pos] += vals
        if len(back) >= CFG["natlag"]:
            for gate, val in zip(gates, back[-CFG["natlag"]]):
                gate[0].append(val)
        back.append([])
        for (_, op), gate in zip(ops[n:n + 4], gates):
            def tie(lhs, gate=gate):
                parts = [lhs[8 * i:8 * i + 8] for i in range(8)]
                for i, vals in enumerate(gate):
                    if vals:
                        both = functools.reduce(jnp.bitwise_or, [pltpu.bitcast(val, U32) for val in vals])
                        parts[i] = jnp.where(aid["never"], both, parts[i])
                return jnp.concatenate(parts, axis=0)

            out = op(tie)
            if out is not None:
                back[-1].append(out)
    assert not tasks and not queue
    for c in pending.values():
        c.wait()


@jax.jit
def pallas_concat_heads__ssm_conv_s5__ssm_conv_h3__prompt_kernel(
    A_x, A_Lambda_re, A_Lambda_im, A_B_re, A_B_im, A_C_re, A_C_im, A_log_dt, A_Dskip,
    B_q, B_k, B_v, B_shift_k, B_ssm_k, B_ssm_D,
):
    V = pltpu.VMEM
    scratch = [
        V((NJ, S, 128), BF16), V((NJ, S + HALO, 128), BF16), V((NJ, S, 128), BF16), V((NJ, S, 128), BF16),
        V((D, S), BF16), V((2, NJ, D, 128), BF16), V((2, NJ, D, 128), BF16),
        V((D,), BF16), V((D,), BF16), V((D,), BF16), V((D,), BF16), V((D,), BF16), V((4, D), BF16),
        V((2048, 128), BF16), pltpu.SMEM((1,), jnp.int32),
        V((NJ, 22, 8, 128), F32), V((2, 8, D), F32), V((6, 8, D), F32), V((4, T, 128), F32),
        V((NJ, S, 128), F32), V((NJ, S, 128), F32), V((16, 256, 128), F32),
        pltpu.SemaphoreType.DMA((12,)),
    ]
    scratch += [V((10, 2, 128, 128), BF16)] * NP + [V((14, 128, 128), BF16)] * NJ
    scratch += [V((7, NJ, 128, 128), BF16)] * 3 + [V((7, NJ, T // 2, 128), BF16)] * NP
    scratch += [V((4, 128, 128), BF16)] * (2 * NP * NJ)
    scratch += [V((16, 256, 128), F32)] * (2 * NJ) + [V((NP, 4, 256, 128), BF16)] * NJ
    scratch += [V((2, S, 128), F32)] * NJ
    out = pl.pallas_call(
        _kernel,
        out_shape=jax.ShapeDtypeStruct((S, 2 * D), F32),
        in_specs=[pl.BlockSpec(memory_space=pl.ANY)] * 17,
        out_specs=pl.BlockSpec(memory_space=pl.ANY),
        scratch_shapes=scratch,
        compiler_params=pltpu.CompilerParams(vmem_limit_bytes=110 * 1024 * 1024),
        name="s5_h3",
    )(A_x.reshape(S, D), A_Lambda_re, A_Lambda_im, A_B_re, A_B_im, A_C_re, A_C_im, A_log_dt, A_Dskip,
      B_q.reshape(S, D), B_k.reshape(S, D), B_v.reshape(S, D), B_shift_k.T, B_ssm_k, B_ssm_D,
      jnp.asarray(_dft_tables()), jnp.asarray(np.zeros((1,), np.int32)))
    return out.reshape(1, S, 2 * D)
```

```python
import functools

import numpy as np
import jax
import jax.numpy as jnp
from jax import lax
import jax.experimental.pallas as pl
import jax.experimental.pallas.tpu as pltpu

S, D = 2048, 640
T = 512
NP, NJ = 4, 5
NSEM = 6
HALO = 16
F32, BF16, U32 = jnp.float32, jnp.bfloat16, jnp.uint32
NT = (((1,), (1,)), ((), ()))
NN = (((1,), (0,)), ((), ()))
B_ROWS = (pl.ds(0, 128), pl.ds(128, 256), pl.ds(384, 256))

C_ROWS = (pl.ds(0, 256), pl.ds(256, 256), pl.ds(512, 128))

ORDER = ("W:x0c a0 W:b1 a1 a2 W:b2 W:x1 a3 a4 a5 a6 "
         "W:rows W:x2 W:kv0 a7 f0 a8 a9 a10 f1 f2 a11 f3 a12 a13 "
         "W:x3 W:kv1 W:kv2 W:ca a14 a15 f4 a16 f5 a17 f6 f7 f8 a18 a19 f9 c0 f10 c2 f11 c5 "
         "W:cb W:kv3 W:kv4 W:g W:q c3 i0 i1 f12 c1 i2 f13 i3 f14 f15 c4x i4 f16 c4y i5 c4z f17 f18 i6 f19 "
         "c6 i7 i8 i9 c7 i10 i11 c8 i12 i13 c9x i14 c9y i15 c9z i16 i17 c10x i18 c10y i19 c10z c11")
LOADS = "par b0 x0a x0b x0c b1 b2 x1 rows x2 kv0 x3 kv1 kv2 ca cb kv3 kv4 g q"
CFG = dict(
    ahead={"par": "b1", "x0c": "kv0", "b1": "kv1", "x1": "kv2", "kv0": "kv4", "x3": "q"},
    rate=70.0,
    cap=1.5,
    fwcost=40, ivcost=40, projcost=21,
    lag=8,
    early=16,
    quiet=8,
    scandue=80,
    held="kv c", gate=16, scangate=8, natlag=5, holdlag=5, scanlag=12,
)


def _dft_tables():
    g = np.arange(128)[:, None]
    m = np.arange(128)[None, :]
    fwd = np.zeros((4, 256, 128), np.float64)
    for r in range(4):
        th = np.pi * (((4 * g + 1) * (4 * m + r)) % 2048) / 1024.0
        c = np.cos(th).reshape(16, 8, 128)
        s = np.sin(th).reshape(16, 8, 128)
        fwd[r] = np.stack([c, s], axis=1).reshape(256, 128)
    inv = np.transpose(fwd, (0, 2, 1)) / 512.0
    perm = np.arange(128).reshape(4, 8, 2, 2).transpose(0, 2, 1, 3).reshape(128)
    fwd = fwd[:, :, perm]
    inv = inv.reshape(4, 128, 2, 128).transpose(0, 2, 1, 3)[..., perm]
    tab = np.concatenate([fwd.reshape(1024, 128), inv.reshape(1024, 128)], axis=0)
    tab = tab.reshape(64, 2, 8, 2, 128).transpose(0, 2, 1, 3, 4).reshape(2048, 128)
    return tab.astype(jnp.bfloat16)


def _lo(w):
    return pltpu.bitcast(w << 16, F32)


def _hi(w):
    return pltpu.bitcast(w & jnp.uint32(0xFFFF0000), F32)


def _rows16(a, b):
    return jnp.concatenate([a, b], axis=0).astype(BF16)


def _il(v):
    return pl.ds(16 * (v // 2) + v % 2, 8, stride=2)


def _get(ref, idx, v0):
    return jnp.concatenate([ref[idx + (_il(v), slice(None))] for v in range(v0, v0 + 8)], axis=0)


def _cmul(a, b):
    return a[0] * b[0] - a[1] * b[1], a[0] * b[1] + a[1] * b[0]


def _cadd(a, b):
    return a[0] + b[0], a[1] + b[1]


def _csub(a, b):
    return a[0] - b[0], a[1] - b[1]


def _lhs_sums(a11, a12, a21, a22):
    return a11 + a22, a21 + a22, a11 + a12, a21 - a11, a12 - a22


def _rhs_factors(b11, b12, b21, b22):
    return b11 + b22, b11, b12 - b22, b21 - b11, b22, b11 + b12, b21 + b22


def _load_groups():
    groups = {"par": ["lre", "lim", "ldt", "z"], "rows": ["dsk", "sd", "sh", "f"], "g": ["g"],
              "ca": [("c", g, c, j) for g in (0, 2) for j in range(NJ) for c in range(2)],
              "cb": [("c", 1, c, j) for j in range(NJ) for c in range(2)],
              "q": [("q", j) for j in range(NJ)],
              "x0a": [("x", 0, 0), ("x", 0, 2)], "x0b": [("x", 0, 1), ("x", 0, 3)], "x0c": [("x", 0, 4)]}
    for g in range(len(B_ROWS)):
        groups[f"b{g}"] = [("b", g, c, kt) for kt in range(NJ) for c in range(2)]
    for j in range(NJ):
        groups[f"kv{j}"] = [("k", j), ("v", j), ("ssm", j)]
    for p in range(1, NP):
        groups[f"x{p}"] = [("x", p, j) for j in range(NJ)]
    return groups


def _kernel(x_hbm, lre_hbm, lim_hbm, bre_hbm, bim_hbm, cre_hbm, cim_hbm, ldt_hbm, dsk_hbm,
            q_hbm, k_hbm, v_hbm, sh_hbm, ssm_hbm, sd_hbm, tab_hbm, z_hbm,
            o_hbm,
            xs, ks, vs, qs, ssm, bs, cs,
            lre_v, lim_v, ldt_v, dsk_v, sd_v, sh_v, tab_v, z_v,
            lamtab, fvec, rowp, kraw, oa, ob, wprev, sem, *rest):
    rest = list(rest)
    xsums, bfs, cps, hbs, kvbs, ktbs, uhs, khs, ybs, bus = (
        [rest.pop(0) for _ in range(n)] for n in (NP, NJ, 3, NP, NJ * NP, NJ * NP, NJ, NJ, NJ, NJ))

    def cols(j):
        return pl.ds(128 * j, 128)

    def rows(p):
        return pl.ds(T * p, T)

    copies = {"lre": (lre_hbm, lre_v), "lim": (lim_hbm, lim_v), "ldt": (ldt_hbm, ldt_v), "z": (z_hbm, z_v),
              "dsk": (dsk_hbm, dsk_v), "sd": (sd_hbm, sd_v), "sh": (sh_hbm, sh_v),
              "f": (tab_hbm.at[pl.ds(0, 1024), :], tab_v.at[pl.ds(0, 1024), :]),
              "g": (tab_hbm.at[pl.ds(1024, 1024), :], tab_v.at[pl.ds(1024, 1024), :])}
    for j in range(NJ):
        for c, (b_hbm, c_hbm) in enumerate(((bre_hbm, cre_hbm), (bim_hbm, cim_hbm))):
            for g, r in enumerate(C_ROWS):
                copies["c", g, c, j] = (c_hbm.at[r, cols(j)], cs.at[c, j, r, :])
            for g, r in enumerate(B_ROWS):
                copies["b", g, c, j] = (b_hbm.at[r, cols(j)], bs.at[c, j, r, :])
        copies["k", j] = (k_hbm.at[:, cols(j)], ks.at[j, pl.ds(HALO, S), :])
        copies["v", j] = (v_hbm.at[:, cols(j)], vs.at[j])
        copies["q", j] = (q_hbm.at[:, cols(j)], qs.at[j])
        copies["ssm", j] = (ssm_hbm.at[cols(j), :], ssm.at[cols(j), :])
        for p in range(NP):
            copies["x", p, j] = (x_hbm.at[rows(p), cols(j)], xs.at[j, rows(p), :])
            for g in range(2):
                r = pl.ds(T * p + T // 2 * g, T // 2)
                copies["oa", p, g, j] = (oa.at[j, r, :], o_hbm.at[r, cols(j)])
            copies["ob", p, j] = (ob.at[j, rows(p), :], o_hbm.at[rows(p), cols(NJ + j)])

    groups = _load_groups()
    words = ORDER.split()
    slot = {n: batch for batch, key in enumerate(("par", "b0", "x0a", "x0b")) for n in groups[key]}
    batch = 3
    for before, word in zip([""] + words, words):
        if word.startswith("W:"):
            batch += not before.startswith("W:")
            slot.update({n: batch for n in groups[word[2:]]})
    queue, pending = LOADS.split(), {}

    def start(name):
        c = pltpu.make_async_copy(*copies[name], sem.at[slot.get(name, batch + 1) % NSEM])
        c.start()
        pending[name] = c

    def start_through(key):
        while key in queue:
            for name in groups[queue.pop(0)]:
                start(name)

    def wait(key):
        for name in groups[key]:
            pending.pop(name).wait()

    xw, kw, vw, qw, tabw, bw = (r.bitcast(U32) for r in (xs, ks, vs, qs, tab_v, bs))
    sub1 = lax.broadcasted_iota(jnp.int32, (8, 128), 0)

    def bcast(ref):
        return jnp.broadcast_to(ref[...].astype(F32).reshape(1, D), (8, D))

    def xvreg(p, j, b, m):
        return xw[j, pl.ds(T // 2 * p + 32 * b + m, 8, stride=4), :]

    def xrows(p, j, rb):
        return jnp.concatenate([xw[j, _il(T // 16 * p + 8 * rb + v), :] for v in (0, 2, 1, 3, 4, 6, 5, 7)], axis=0)

    aid = dict(never=None, scan=None, product=None)

    def hold(kind, ref, idx, stride):
        if aid[kind] is not None:
            r = idx + (stride, slice(None))
            ref[r] = jnp.where(aid["never"], aid[kind], ref[r])

    def held(kind, val):
        if aid["product"] is None or kind not in CFG["held"]:
            return val
        return jnp.where(aid["never"], aid["product"], val)

    def discretise():
        lr, li = bcast(lre_v), bcast(lim_v)
        dt = jnp.exp(bcast(ldt_v)).astype(BF16).astype(F32)
        mag = jnp.exp(dt * lr)
        lam = (mag * jnp.cos(dt * li), mag * jnp.sin(dt * li))
        nr, ni = lam[0] - 1.0, lam[1]
        big = jnp.abs(lr) >= jnp.abs(li)
        ratio = jnp.where(big, li / lr, lr / li)
        den = jnp.where(big, lr + li * ratio, li + lr * ratio)
        fvec[0] = 2.0 * jnp.where(big, nr + ni * ratio, nr * ratio + ni) / den
        fvec[1] = 2.0 * jnp.where(big, ni - nr * ratio, ni * ratio - nr) / den
        pw = [lam]
        for i in range(1, 8):
            pw.append(_cmul(pw[(i - 1) // 2], pw[i - 1 - (i - 1) // 2]))
        mu1 = pw[7]
        mu2 = _cmul(mu1, mu1)
        mu4 = _cmul(mu2, mu2)
        sub = lax.broadcasted_iota(jnp.int32, (8, D), 0)
        tab = [c for z in pw for c in z]
        for d_, mu in ((1, mu1), (2, mu2), (4, mu4)):
            tab += [jnp.where(sub >= d_, mu[0], 0.0), jnp.where(sub >= d_, mu[1], 0.0)]
        for j in range(NJ):
            for i, t_ in enumerate(tab):
                lamtab[j, i] = t_[:, 128 * j:128 * (j + 1)]
            ks[j, pl.ds(0, HALO), :] = jnp.zeros((HALO, 128), BF16)

    def row_params():
        rowp[0] = bcast(dsk_v)
        rowp[1] = bcast(sd_v)
        sh = sh_v[...].astype(F32)
        for i in range(4):
            rowp[2 + i] = jnp.broadcast_to(sh[i:i + 1], (8, D))
        yield 100, []

    def x_sums(p, kts):
        for g in range(2):
            for kt in kts:
                for v in range(8):
                    fs = _lhs_sums(*(
                        pltpu.bitcast(xw[kt + 2 * cb, pl.ds(T // 2 * p + 64 * rb + 8 * v, 8), :], BF16).astype(F32)
                        for rb in (2 * g, 2 * g + 1) for cb in range(2)))
                    for n, f in enumerate(fs):
                        xsums[p][5 * g + n, kt, pl.ds(16 * v, 16), :] = f.astype(BF16)
                    yield 25, [f[8:] for f in fs]

    def b_factors(j):
        for s in range(8):
            r = pl.ds(128 * j + 16 * s, 16)
            for kt in range(2):
                fs = _rhs_factors(*(bs[c, kt + 2 * kb, r, :].astype(F32) for kb in range(2) for c in range(2)))
                for n, f in enumerate(fs):
                    bfs[j][2 * n + kt, pl.ds(16 * s, 16), :] = f.astype(BF16)
                yield 34, [fs[n][8:] for n in (0, 2, 3, 5, 6)]

    lasts = [None] * NJ

    def scan(p, j):
        def power(i):
            return lamtab[j, 2 * i], lamtab[j, 2 * i + 1]

        for b in range(T // 64):
            hold("scan", bus[j], (0,), pl.ds(T * p + 64 * b, 8, stride=9))
            hs = []
            for i in range(8):
                st = pl.ds(T * p + 64 * b + 32 * ((i // 2) % 2) + 2 * (i // 4) + i % 2, 8, stride=4)
                u = (bus[j][0, st, :], bus[j][1, st, :])
                hs.append(u if i == 0 else _cadd(_cmul(power(0), hs[-1]), u))
            yield 58, list(hs[7]), CFG["scangate"]
            e = tuple(jnp.where(sub1 == 7, c0, c1) for c0, c1 in zip(lasts[j] or (0.0, 0.0), hs[7]))
            e = tuple(pltpu.roll(c, 1, 0) for c in e)
            for n, d_ in enumerate((1, 2, 4)):
                e = _cadd(e, _cmul(power(8 + n), tuple(pltpu.roll(c, d_, 0) for c in e)))
            yield 36, list(e), CFG["scangate"]
            for i0 in (1, 0):
                for i in range(i0, 8, 2):
                    hs[i] = _cadd(hs[i], _cmul(power(i), e))
                    if i == 7:
                        lasts[j] = hs[7]
                blk = [jnp.concatenate([hs[i][c], hs[i + 4][c]], axis=0) for i in (i0, i0 + 2) for c in range(2)]
                fs = _lhs_sums(*blk) + (blk[0], blk[3])
                for n, f in enumerate(fs):
                    hbs[p][n, j, pl.ds(32 * b + 16 * i0, 16), :] = f.astype(BF16)
                yield 52, [fs[0][8:], fs[1][:8], fs[4][8:]], CFG["scangate"]

    def fold_c(j, i):
        f_r, f_i = (jnp.concatenate([fvec[c, :, cols(j)]] * 2, axis=0) for c in range(2))
        f_n = -f_i

        def fold(d_, s, f_r):
            a, b = (cs[c, j, pl.ds(128 * d_ + 16 * s, 16), :].astype(F32) for c in range(2))
            return a * f_r - b * f_i, a * f_n - b * f_r

        for s in range(8):
            g_r = jnp.concatenate([held("c", fvec[0, :, cols(j)])] * 2, axis=0)
            if i < 2:
                (r0, i0), (r1, i1) = fold(2 * i, s, g_r), fold(2 * i + 1, s, g_r)
                fs = _rhs_factors(r0, r1, i0, i1)
            else:
                r0, i0 = fold(4, s, g_r)
                fs = (r0 - i0, i0, r0)
            for n, f in enumerate(fs):
                cps[i][n, j, pl.ds(16 * s, 16), :] = f.astype(BF16)
            yield (58, [fs[0][8:], fs[5][:8], fs[6][8:]]) if i < 2 else (28, [fs[0][8:]])

    def prep_kv(j, p):
        for mb in range(8):
            w = [rowp[2 + i, :, cols(j)] for i in range(4)]
            w[0], w[2] = held("kv", w[0]), held("kv", w[2])
            outs = [[] for _ in range(4)]
            for hf in range(2):
                at = T // 2 * p + 32 * mb + 16 * hf
                p0, p1, w0, w1 = (kw[j, pl.ds(HALO // 2 + at + o, 8, stride=2), :] for o in (-2, -1, 0, 1))
                kk = [_hi(p0), _lo(p1), _hi(p1), _lo(w0), _hi(w0), _lo(w1), _hi(w1)]
                v0, v1 = (vw[j, pl.ds(at + o, 8, stride=2), :] for o in (0, 1))
                vv = [_lo(v0), _hi(v0), _lo(v1), _hi(v1)]
                for r in range(4):
                    ksh = (kk[r] * w[3] + kk[r + 1] * w[2]) + (kk[r + 2] * w[1] + kk[r + 3] * w[0])
                    outs[r].append(ksh * vv[r])
                if hf == 0:
                    yield 47, [outs[r][0] for r in range(4)]
            for r in range(4):
                kvbs[j * NP + p][r, pl.ds(16 * mb, 16), :] = _rows16(*outs[r])
            yield 51, [outs[r][1] for r in range(4)]

    def prep_filter(j, p):
        raw = kraw.at[(j * NP + p) % 4]
        for a in range(4):
            raw[pl.ds(128 * a, 128), :] = ssm[cols(j), pl.ds(T * p + 128 * a, 128)].astype(F32).T
            for mb in (2 * a, 2 * a + 1):
                ws = [raw[pl.ds(64 * mb + r, 16, stride=4), :] for r in range(4)]
                for r in range(4):
                    ktbs[j * NP + p][r, pl.ds(16 * mb, 16), :] = ws[r].astype(BF16)
                yield 16, [w[8:] for w in ws]

    def bin_(ref, i, h, n):
        return tuple(ref[i, pl.ds(64 * h + 16 * n + c, 8, stride=2), :] for c in range(2))

    def product(j, i, a, prev):
        half = []
        for hs in ((0, 2), (1, 3)):
            y = []
            for h in hs:
                w = None
                for n in range(a + 1):
                    t_ = _cmul(bin_(khs[j], i, h, n), bin_(uhs[j], i, h, a - n))
                    w = t_ if w is None else _cadd(w, t_)
                y.append((w[0] + prev[h][1], w[1] - prev[h][0]) if a else w)
                prev[h] = w
                if a > 1 and h == hs[0]:
                    yield 8 * a + 8, list(y[0])
            half += [_cadd(*y), _csub(*y)]
            if hs[0] == 0 and a:
                yield (8 * a + 14 if a > 1 else 38), list(half[0])
        p_, q_, s_, t_ = half
        res = [_cadd(p_, s_), (q_[0] + t_[1], q_[1] - t_[0]), _csub(p_, s_), (q_[0] - t_[1], q_[1] + t_[0])]
        for r in range(4):
            ybs[j][a, r, pl.ds(16 * i, 16), :] = _rows16(*res[r])
        yield (46, 50, 36, 44)[a], [res[0][1], res[1][0]]

    def products(j, blocks, groups_):
        for i in groups_:
            hold("product", uhs[j], (i,), pl.ds(0, 8, stride=33))
            prev = [bin_(wprev, i, h, blocks[0] - 1) if blocks[0] else None for h in range(4)]
            for a in blocks:
                yield from product(j, i, a, prev)
            if a < NP - 1:
                for h in range(4):
                    for c in range(2):
                        wprev[i, pl.ds(64 * h + 16 * a + c, 8, stride=2), :] = prev[h][c]

    def mm(tie, lhs, rhs, dims):
        return lax.dot_general(pltpu.bitcast(tie(lhs), BF16), pltpu.bitcast(rhs, BF16), dims,
                               preferred_element_type=F32)

    def program(steps):
        m = {}
        for key, lhs, rhs, then in steps:
            def op(tie, key=key, lhs=lhs, rhs=rhs, then=then):
                d_ = mm(tie, lhs(), rhs(), NT)
                m[key] = m[key] + d_ if key in m else d_
                out = m[key][120:128]
                if then is not None:
                    then(m)
                return out
            yield CFG["projcost"], op

    def project_in(p, j):
        for g in range(2):
            def plain(rb, kt, g=g):
                return lambda: xrows(p, kt, 2 * g + rb)

            def put(rb, c, val, g=g):
                bus[j][c, pl.ds(T * p + 256 * g + 128 * rb, 128), :] = val

            def prod(n, key, then):
                def left(kt, g=g):
                    if n in (3, 4):
                        return plain(n - 3, 2 * (n - 3) + kt)
                    at = (5 * g + {1: 0, 2: 1, 5: 2, 6: 3, 7: 4}[n], kt)
                    return lambda: jnp.concatenate(
                        [xsums[p].bitcast(U32)[at + (_il(v), slice(None))] for v in (0, 2, 1, 3, 4, 6, 5, 7)], axis=0)
                return [(key, left(kt), lambda kt=kt: bfs[j].bitcast(U32)[2 * (n - 1) + kt], then if kt else None)
                        for kt in range(2)]

            lead = p == 0 and j in (0, 1, 3) and g == 0

            def after4(m, put=put):
                put(0, 1, m[3] + m[5] + m["l01"])
                m["t10"] = m["l10"] + m[4]
                m["t00"] = m[4] - m[5]

            def after2(m, put=put):
                put(1, 0, m["t10"] + m[2])
                m["t11"] = m[3] - m[2]

            def after1(m):
                m["t00"] = m["t00"] + m[1]
                m["t11"] = m["t11"] + m[1]

            def finish(m, put=put):
                put(0, 0, m["t00"] + m["l00"])
                put(1, 1, m["t11"] + m["l11"])

            def fifth(key, rb, c, then=None):
                return key, plain(rb, 4), lambda: bw[c, 4, pl.ds(64 * j, 64), :], then

            middle = (prod(4, 4, after4) + prod(2, 2, after2) + prod(1, 1, after1) + prod(7, "t00", None)
                      + prod(6, "t11", finish if lead else None))
            if lead:
                steps = ([fifth(f"l{rb}{c}", rb, c) for rb in range(2) for c in range(2)]
                         + prod(3, 3, None) + prod(5, 5, None) + middle)
            else:
                steps = (prod(3, 3, None) + prod(5, 5, None) + [fifth("l01", 0, 1), fifth("l10", 1, 0)] + middle
                         + [fifth("t00", 0, 0, lambda m, put=put: put(0, 0, m["t00"])),
                            fifth("t11", 1, 1, lambda m, put=put: put(1, 1, m["t11"]))])
            yield from program(steps)

    done = {}

    def project_out(p, unit, part):
        parts = [(0, unit, None), (1, unit, None), (0, 2, unit)] if unit < 2 else [(1, 2, 0), (1, 2, 1)]
        for g, i, half in [parts["xyz".index(part)]] if part else parts:
            def put(j, rb, val, g=g):
                dsk = rowp[0, :, cols(j)]
                for blk in range(4):
                    for late in range(2):
                        w = xvreg(p, j, 4 * g + blk, rb + 2 * late)
                        for i0, xv in enumerate((_lo(w), _hi(w))):
                            t0 = T * p + 64 * (4 * g + blk) + 2 * rb + 4 * late + i0
                            v = 4 * blk + 2 * i0 + late
                            oa[j, pl.ds(t0, 8, stride=8), :] = val[8 * v:8 * v + 8] + xv * dsk
                done[p, g, j] = done.get((p, g, j), 0) + 1
                if done[p, g, j] == 2:
                    start(("oa", p, g, j))

            def prod(ln, rn, key, then):
                return [(key, lambda kt=kt, g=g: hbs[p].bitcast(U32)[ln, kt, pl.ds(64 * g, 64), :],
                         lambda kt=kt, i=i: cps[i].bitcast(U32)[rn, kt], then if kt == NJ - 1 else None)
                        for kt in range(NJ)]

            if i < 2:
                def after4(m):
                    m["t00"] = m[4] - m[5]

                def after2(m, put=put, i=i):
                    put(2 * i, 1, m[2] + m[4])
                    m["t11"] = m[3] - m[2]

                def after1(m):
                    m["t00"] = m["t00"] + m[1]
                    m["t11"] = m["t11"] + m[1]

                steps = (prod(5, 2, 3, None)
                         + prod(2, 4, 5, lambda m, put=put, i=i: put(2 * i + 1, 0, m[3] + m[5]))
                         + prod(6, 3, 4, after4) + prod(1, 1, 2, after2) + prod(0, 0, 1, after1)
                         + prod(4, 6, "t00", lambda m, put=put, i=i: put(2 * i, 0, m["t00"]))
                         + prod(3, 5, "t11", lambda m, put=put, i=i: put(2 * i + 1, 1, m["t11"])))
            elif half == 0:
                steps = prod(5, 0, 0, None) + prod(2, 1, 0, lambda m, put=put: put(4, 0, m[0]))
            else:
                steps = prod(6, 0, 0, None) + prod(1, 2, 1, lambda m, put=put: put(4, 1, m[1] - m[0]))
            yield from program(steps)

    def forward(j, p):
        for src, dst in ((kvbs[j * NP + p], uhs[j]), (ktbs[j * NP + p], khs[j])):
            for hf in range(2):
                v = []
                for r in range(4):
                    def op(tie, src=src, dst=dst, hf=hf, r=r, v=v):
                        v.append(mm(tie, _get(tabw, (), 16 * r + 8 * hf), _get(src.bitcast(U32), (r,), 0), NN))
                        if r < 3:
                            return None
                        for i in range(8):
                            z = [(v[n][16 * i:16 * i + 8], v[n][16 * i + 8:16 * i + 16]) for n in range(4)]
                            a, b = _cadd(z[0], z[2]), _csub(z[0], z[2])
                            if dst is khs[j] and p == 0:
                                tap = rowp[1, :, cols(j)]
                                a, b = (a[0] + tap, a[1]), (b[0] + tap, b[1])
                            c, d_ = _cadd(z[1], z[3]), _csub(z[1], z[3])
                            res = [_cadd(a, c), (b[0] - d_[1], b[1] + d_[0]), _csub(a, c), (b[0] + d_[1], b[1] - d_[0])]
                            for h in range(4):
                                for e in range(2):
                                    dst[8 * hf + i, pl.ds(64 * h + 16 * p + e, 8, stride=2), :] = res[h][e]
                        return res[3][1] + res[2][0]
                    yield CFG["fwcost"], op

    def inverse(j, a):
        for r in range(4):
            acc = []
            for kt in range(2):
                def op(tie, r=r, kt=kt, acc=acc):
                    acc.append(mm(tie, _get(tabw, (), 64 + 16 * r + 8 * kt), _get(ybs[j].bitcast(U32), (a, r), 8 * kt), NN))
                    if kt == 0:
                        return None
                    y = acc[0] + acc[1]
                    for mb in range(16):
                        w = qw[j, pl.ds(T // 2 * a + 16 * mb + r // 2, 8, stride=2), :]
                        out = (_hi(w) if r % 2 else _lo(w)) * y[8 * mb:8 * mb + 8]
                        ob[j, pl.ds(T * a + 32 * mb + r, 8, stride=4), :] = out
                    if r == 3:
                        start(("ob", a, j))
                    return out
                yield CFG["ivcost"], op

    ops, first, last, wait_at, waits = [], {}, {}, {}, {}
    for word in words:
        if word.startswith("W:"):
            wait_at[word[2:]] = len(ops)
            waits.setdefault(len(ops), []).append(word[2:])
            continue
        k = int(word[1:].rstrip("xyz"))
        make, unit = {"a": (project_in, divmod(k, NJ)), "c": (project_out, divmod(k, 3)),
                      "f": (forward, divmod(k, NP)), "i": (inverse, divmod(k, NP))}[word[0]]
        key = (word[0],) + unit
        first.setdefault(key, len(ops))
        ops += list(make(*unit, word[1:].lstrip("0123456789")) if word[0] == "c" else make(*unit))
        last[key] = len(ops)

    lag = CFG["lag"]
    tasks = [[wait_at["rows"] + 4, wait_at["rows"], 100, row_params()]]
    for p in range(NP):
        if p:
            tasks.append([first["a", p, 0], wait_at[f"x{p}"], 800, x_sums(p, (0, 1))])
        for j in range(NJ):
            due = min(first["c", p, i] for i in range(3)) - CFG["scandue"] * p
            tasks.append([due, last["a", p, j] + lag, 1584, scan(p, j)])
            tasks.append([first["f", j, p], max(wait_at[f"kv{j}"], wait_at["rows"] + 4), 784, prep_kv(j, p)])
            tasks.append([first["f", j, p] + 8, wait_at[f"kv{j}"], 128, prep_filter(j, p)])
    for j in range(NJ):
        if j:
            tasks.append([first["a", 0, j], wait_at[f"b{(j + 1) // 2}"], 512, b_factors(j)])
        for i in range(3):
            due = min(first["c", p, n] for p in range(NP) for n in ((0,), (1,), (0, 1, 2))[i])
            tasks.append([due, wait_at["cb" if i == 1 else "ca"], 464 if i < 2 else 224, fold_c(j, i)])
        ready = max(last["f", j, p] for p in range(NP)) + lag
        for blocks, part in ([((0, 1), range(16)), ((2,), range(16)), ((3,), range(16))] if j == NJ - 1 else
                             [((0, 1, 2, 3), range(4 * i, 4 * i + 4)) for i in range(4)]):
            cost = len(part) * sum((48, 90, 112, 152)[a] for a in blocks) if j == NJ - 1 else 1632
            tasks.append([min(first["i", j, a] for a in blocks), ready, cost, products(j, blocks, part)])
    tasks.sort(key=lambda t_: t_[0])
    cum = [0.0]
    for n, (c, _) in enumerate(ops):
        quiet = any(n + ahead in waits for ahead in range(1, CFG["quiet"] + 1))
        cum.append(cum[-1] + (0.0 if quiet else max(CFG["rate"] - c, 0.0)))

    start_through("x0c")
    wait("par")
    start_through(CFG["ahead"]["par"])
    aid["never"] = jnp.full((8, 128), z_v[0], jnp.int32) != 0
    discretise()
    for key, task in (("b0", b_factors(0)), ("x0a", x_sums(0, (0,))), ("x0b", x_sums(0, (1,)))):
        wait(key)
        for _ in task:
            pass

    budget, back, later = 0.0, [], {}
    for n in range(0, len(ops), 4):
        for key in waits.get(n, ()):
            wait(key)
        for key in waits.get(n, ()):
            later.clear()
            start_through(CFG["ahead"].get(key))
        room = cum[n + 4] - cum[n]
        need = max([0.0] + [sum(t2[2] for t2 in tasks[:i + 1]) / max(cum[max(t_[0] - CFG["early"], 0)] - cum[n], room, 1)
                            for i, t_ in enumerate(tasks)])
        budget = min(budget, 0.0) + room * min(need, CFG["cap"])
        for kind, behind in (("product", CFG["holdlag"]), ("scan", CFG["scanlag"])):
            aid[kind] = back[-behind][-1] if len(back) >= behind else None
        steps = []
        for t_ in list(tasks):
            urgent = t_[0] < n + 4
            if t_[1] > n and not urgent:
                continue
            while budget > 0 or urgent:
                step = next(t_[3], None)
                if step is None:
                    tasks.remove(t_)
                    break
                if not urgent:
                    budget -= step[0]
                    t_[2] -= step[0]
                    steps.append((step[0], step[1][-2:], sum(step[2:])))
        total, acc = sum(t_[0] for t_ in steps), 0
        for i, (cost, vals, slack) in enumerate(steps):
            acc += cost
            later.setdefault(2 * n + CFG["gate"] + slack + int(8 * acc / (total + 1)), []).append((i % 4, vals))
        gates = [[[] for _ in range(8)] for _ in range(4)]
        for pos in range(8):
            for i, vals in later.pop(2 * n + pos, ()):
                gates[i][pos] += vals
        if len(back) >= CFG["natlag"]:
            for gate, val in zip(gates, back[-CFG["natlag"]]):
                gate[0].append(val)
        back.append([])
        for (_, op), gate in zip(ops[n:n + 4], gates):
            def tie(lhs, gate=gate):
                parts = [lhs[8 * i:8 * i + 8] for i in range(8)]
                for i, vals in enumerate(gate):
                    if vals:
                        both = functools.reduce(jnp.bitwise_or, [pltpu.bitcast(val, U32) for val in vals])
                        parts[i] = jnp.where(aid["never"], both, parts[i])
                return jnp.concatenate(parts, axis=0)

            out = op(tie)
            if out is not None:
                back[-1].append(out)
    assert not tasks and not queue
    for c in pending.values():
        c.wait()


@jax.jit
def pallas_concat_heads__ssm_conv_s5__ssm_conv_h3__prompt_kernel(
    A_x, A_Lambda_re, A_Lambda_im, A_B_re, A_B_im, A_C_re, A_C_im, A_log_dt, A_Dskip,
    B_q, B_k, B_v, B_shift_k, B_ssm_k, B_ssm_D,
):
    V = pltpu.VMEM
    scratch = [
        V((NJ, S, 128), BF16), V((NJ, S + HALO, 128), BF16), V((NJ, S, 128), BF16), V((NJ, S, 128), BF16),
        V((D, S), BF16), V((2, NJ, D, 128), BF16), V((2, NJ, D, 128), BF16),
        V((D,), BF16), V((D,), BF16), V((D,), BF16), V((D,), BF16), V((D,), BF16), V((4, D), BF16),
        V((2048, 128), BF16), pltpu.SMEM((1,), jnp.int32),
        V((NJ, 22, 8, 128), F32), V((2, 8, D), F32), V((6, 8, D), F32), V((4, T, 128), F32),
        V((NJ, S, 128), F32), V((NJ, S, 128), F32), V((16, 256, 128), F32),
        pltpu.SemaphoreType.DMA((NSEM,)),
    ]
    scratch += [V((10, 2, 128, 128), BF16)] * NP + [V((14, 128, 128), BF16)] * NJ
    scratch += [V((7, NJ, 128, 128), BF16)] * 3 + [V((7, NJ, T // 2, 128), BF16)] * NP
    scratch += [V((4, 128, 128), BF16)] * (2 * NP * NJ)
    scratch += [V((16, 256, 128), F32)] * (2 * NJ) + [V((NP, 4, 256, 128), BF16)] * NJ
    scratch += [V((2, S, 128), F32)] * NJ
    out = pl.pallas_call(
        _kernel,
        out_shape=jax.ShapeDtypeStruct((S, 2 * D), F32),
        in_specs=[pl.BlockSpec(memory_space=pl.ANY)] * 17,
        out_specs=pl.BlockSpec(memory_space=pl.ANY),
        scratch_shapes=scratch,
        compiler_params=pltpu.CompilerParams(vmem_limit_bytes=110 * 1024 * 1024),
        name="s5_h3",
    )(A_x.reshape(S, D), A_Lambda_re, A_Lambda_im, A_B_re, A_B_im, A_C_re, A_C_im, A_log_dt, A_Dskip,
      B_q.reshape(S, D), B_k.reshape(S, D), B_v.reshape(S, D), B_shift_k.T, B_ssm_k, B_ssm_D,
      jnp.asarray(_dft_tables()), jnp.asarray(np.zeros((1,), np.int32)))
    return out.reshape(1, S, 2 * D)
```

```python
import functools

import numpy as np
import jax
import jax.numpy as jnp
from jax import lax
import jax.experimental.pallas as pl
import jax.experimental.pallas.tpu as pltpu

S, D = 2048, 640
T = 512
NP, NJ = 4, 5
NSEM = 6
HALO = 16
F32, BF16, U32 = jnp.float32, jnp.bfloat16, jnp.uint32
NT = (((1,), (1,)), ((), ()))
NN = (((1,), (0,)), ((), ()))
B_ROWS = (pl.ds(0, 128), pl.ds(128, 256), pl.ds(384, 256))

C_ROWS = (pl.ds(0, 256), pl.ds(256, 256), pl.ds(512, 128))

ORDER = ("W:x0c a0 W:b1 a1 a2 W:b2 W:x1 a3 a4 a5 a6 "
         "W:rows W:x2 W:kv0 a7 f0 a8 a9 a10 f1 f2 a11 f3 a12 a13 "
         "W:x3 W:kv1 W:kv2 W:ca a14 a15 f4 a16 f5 a17 f6 f7 f8 a18 a19 f9 c0 f10 c2 f11 c5 "
         "W:cb W:kv3 W:kv4 W:g W:q c3 i0 i1 f12 c1 i2 f13 i3 f14 f15 c4x i4 f16 c4y i5 c4z f17 f18 i6 f19 "
         "c6 i7 i8 i9 c7 i10 i11 c8 i12 i13 c9x i14 c9y i15 c9z i16 i17 c10x i18 c10y i19 c10z c11")
LOADS = "par b0 x0a x0b x0c b1 b2 x1 rows x2 kv0 x3 kv1 kv2 ca cb kv3 kv4 g q"
CFG = dict(
    ahead={"par": "b1", "x0c": "kv0", "b1": "kv1", "x1": "kv2", "kv0": "kv4", "x3": "q"},
    rate=72.0,
    cap=1.5,
    fwcost=40, ivcost=40, projcost=21,
    lag=8,
    early=16,
    quiet=8,
    scandue=80,
    held="kv c", gate=16, scangate=8, natlag=5, holdlag=5, scanlag=12,
)


def _dft_tables():
    g = np.arange(128)[:, None]
    m = np.arange(128)[None, :]
    fwd = np.zeros((4, 256, 128), np.float64)
    for r in range(4):
        th = np.pi * (((4 * g + 1) * (4 * m + r)) % 2048) / 1024.0
        c = np.cos(th).reshape(16, 8, 128)
        s = np.sin(th).reshape(16, 8, 128)
        fwd[r] = np.stack([c, s], axis=1).reshape(256, 128)
    inv = np.transpose(fwd, (0, 2, 1)) / 512.0
    perm = np.arange(128).reshape(4, 8, 2, 2).transpose(0, 2, 1, 3).reshape(128)
    fwd = fwd[:, :, perm]
    inv = inv.reshape(4, 128, 2, 128).transpose(0, 2, 1, 3)[..., perm]
    tab = np.concatenate([fwd.reshape(1024, 128), inv.reshape(1024, 128)], axis=0)
    tab = tab.reshape(64, 2, 8, 2, 128).transpose(0, 2, 1, 3, 4).reshape(2048, 128)
    return tab.astype(jnp.bfloat16)


def _lo(w):
    return pltpu.bitcast(w << 16, F32)


def _hi(w):
    return pltpu.bitcast(w & jnp.uint32(0xFFFF0000), F32)


def _rows16(a, b):
    return jnp.concatenate([a, b], axis=0).astype(BF16)


def _il(v):
    return pl.ds(16 * (v // 2) + v % 2, 8, stride=2)


def _get(ref, idx, v0):
    return jnp.concatenate([ref[idx + (_il(v), slice(None))] for v in range(v0, v0 + 8)], axis=0)


def _cmul(a, b):
    return a[0] * b[0] - a[1] * b[1], a[0] * b[1] + a[1] * b[0]


def _cadd(a, b):
    return a[0] + b[0], a[1] + b[1]


def _csub(a, b):
    return a[0] - b[0], a[1] - b[1]


def _lhs_sums(a11, a12, a21, a22):
    return a11 + a22, a21 + a22, a11 + a12, a21 - a11, a12 - a22


def _rhs_factors(b11, b12, b21, b22):
    return b11 + b22, b11, b12 - b22, b21 - b11, b22, b11 + b12, b21 + b22


def _load_groups():
    groups = {"par": ["lre", "lim", "ldt", "z"], "rows": ["dsk", "sd", "sh", "f"], "g": ["g"],
              "ca": [("c", g, c, j) for g in (0, 2) for j in range(NJ) for c in range(2)],
              "cb": [("c", 1, c, j) for j in range(NJ) for c in range(2)],
              "q": [("q", j) for j in range(NJ)],
              "x0a": [("x", 0, 0), ("x", 0, 2)], "x0b": [("x", 0, 1), ("x", 0, 3)], "x0c": [("x", 0, 4)]}
    for g in range(len(B_ROWS)):
        groups[f"b{g}"] = [("b", g, c, kt) for kt in range(NJ) for c in range(2)]
    for j in range(NJ):
        groups[f"kv{j}"] = [("k", j), ("v", j), ("ssm", j)]
    for p in range(1, NP):
        groups[f"x{p}"] = [("x", p, j) for j in range(NJ)]
    return groups


def _kernel(x_hbm, lre_hbm, lim_hbm, bre_hbm, bim_hbm, cre_hbm, cim_hbm, ldt_hbm, dsk_hbm,
            q_hbm, k_hbm, v_hbm, sh_hbm, ssm_hbm, sd_hbm, tab_hbm, z_hbm,
            o_hbm,
            xs, ks, vs, qs, ssm, bs, cs,
            lre_v, lim_v, ldt_v, dsk_v, sd_v, sh_v, tab_v, z_v,
            lamtab, fvec, rowp, kraw, oa, ob, wprev, sem, *rest):
    rest = list(rest)
    xsums, bfs, cps, hbs, kvbs, ktbs, uhs, khs, ybs, bus = (
        [rest.pop(0) for _ in range(n)] for n in (NP, NJ, 3, NP, NJ * NP, NJ * NP, NJ, NJ, NJ, NJ))

    def cols(j):
        return pl.ds(128 * j, 128)

    def rows(p):
        return pl.ds(T * p, T)

    copies = {"lre": (lre_hbm, lre_v), "lim": (lim_hbm, lim_v), "ldt": (ldt_hbm, ldt_v), "z": (z_hbm, z_v),
              "dsk": (dsk_hbm, dsk_v), "sd": (sd_hbm, sd_v), "sh": (sh_hbm, sh_v),
              "f": (tab_hbm.at[pl.ds(0, 1024), :], tab_v.at[pl.ds(0, 1024), :]),
              "g": (tab_hbm.at[pl.ds(1024, 1024), :], tab_v.at[pl.ds(1024, 1024), :])}
    for j in range(NJ):
        for c, (b_hbm, c_hbm) in enumerate(((bre_hbm, cre_hbm), (bim_hbm, cim_hbm))):
            for g, r in enumerate(C_ROWS):
                copies["c", g, c, j] = (c_hbm.at[r, cols(j)], cs.at[c, j, r, :])
            for g, r in enumerate(B_ROWS):
                copies["b", g, c, j] = (b_hbm.at[r, cols(j)], bs.at[c, j, r, :])
        copies["k", j] = (k_hbm.at[:, cols(j)], ks.at[j, pl.ds(HALO, S), :])
        copies["v", j] = (v_hbm.at[:, cols(j)], vs.at[j])
        copies["q", j] = (q_hbm.at[:, cols(j)], qs.at[j])
        copies["ssm", j] = (ssm_hbm.at[cols(j), :], ssm.at[cols(j), :])
        for p in range(NP):
            copies["x", p, j] = (x_hbm.at[rows(p), cols(j)], xs.at[j, rows(p), :])
            for g in range(2):
                r = pl.ds(T * p + T // 2 * g, T // 2)
                copies["oa", p, g, j] = (oa.at[j, r, :], o_hbm.at[r, cols(j)])
            copies["ob", p, j] = (ob.at[j, rows(p), :], o_hbm.at[rows(p), cols(NJ + j)])

    groups = _load_groups()
    words = ORDER.split()
    slot = {n: batch for batch, key in enumerate(("par", "b0", "x0a", "x0b")) for n in groups[key]}
    batch = 3
    for before, word in zip([""] + words, words):
        if word.startswith("W:"):
            batch += not before.startswith("W:")
            slot.update({n: batch for n in groups[word[2:]]})
    queue, pending = LOADS.split(), {}

    def start(name):
        c = pltpu.make_async_copy(*copies[name], sem.at[slot.get(name, batch + 1) % NSEM])
        c.start()
        pending[name] = c

    def start_through(key):
        while key in queue:
            for name in groups[queue.pop(0)]:
                start(name)

    def wait(key):
        for name in groups[key]:
            pending.pop(name).wait()

    xw, kw, vw, qw, tabw, bw = (r.bitcast(U32) for r in (xs, ks, vs, qs, tab_v, bs))
    sub1 = lax.broadcasted_iota(jnp.int32, (8, 128), 0)

    def bcast(ref):
        return jnp.broadcast_to(ref[...].astype(F32).reshape(1, D), (8, D))

    def xvreg(p, j, b, m):
        return xw[j, pl.ds(T // 2 * p + 32 * b + m, 8, stride=4), :]

    def xrows(p, j, rb):
        return jnp.concatenate([xw[j, _il(T // 16 * p + 8 * rb + v), :] for v in (0, 2, 1, 3, 4, 6, 5, 7)], axis=0)

    aid = dict(never=None, scan=None, product=None)

    def hold(kind, ref, idx, stride):
        if aid[kind] is not None:
            r = idx + (stride, slice(None))
            ref[r] = jnp.where(aid["never"], aid[kind], ref[r])

    def held(kind, val):
        if aid["product"] is None or kind not in CFG["held"]:
            return val
        return jnp.where(aid["never"], aid["product"], val)

    def discretise():
        lr, li = bcast(lre_v), bcast(lim_v)
        dt = jnp.exp(bcast(ldt_v)).astype(BF16).astype(F32)
        mag = jnp.exp(dt * lr)
        lam = (mag * jnp.cos(dt * li), mag * jnp.sin(dt * li))
        nr, ni = lam[0] - 1.0, lam[1]
        big = jnp.abs(lr) >= jnp.abs(li)
        ratio = jnp.where(big, li / lr, lr / li)
        den = jnp.where(big, lr + li * ratio, li + lr * ratio)
        fvec[0] = 2.0 * jnp.where(big, nr + ni * ratio, nr * ratio + ni) / den
        fvec[1] = 2.0 * jnp.where(big, ni - nr * ratio, ni * ratio - nr) / den
        pw = [lam]
        for i in range(1, 8):
            pw.append(_cmul(pw[(i - 1) // 2], pw[i - 1 - (i - 1) // 2]))
        mu1 = pw[7]
        mu2 = _cmul(mu1, mu1)
        mu4 = _cmul(mu2, mu2)
        sub = lax.broadcasted_iota(jnp.int32, (8, D), 0)
        tab = [c for z in pw for c in z]
        for d_, mu in ((1, mu1), (2, mu2), (4, mu4)):
            tab += [jnp.where(sub >= d_, mu[0], 0.0), jnp.where(sub >= d_, mu[1], 0.0)]
        for j in range(NJ):
            for i, t_ in enumerate(tab):
                lamtab[j, i] = t_[:, 128 * j:128 * (j + 1)]
            ks[j, pl.ds(0, HALO), :] = jnp.zeros((HALO, 128), BF16)

    def row_params():
        rowp[0] = bcast(dsk_v)
        rowp[1] = bcast(sd_v)
        sh = sh_v[...].astype(F32)
        for i in range(4):
            rowp[2 + i] = jnp.broadcast_to(sh[i:i + 1], (8, D))
        yield 100, []

    def x_sums(p, kts):
        for g in range(2):
            for kt in kts:
                for v in range(8):
                    fs = _lhs_sums(*(
                        pltpu.bitcast(xw[kt + 2 * cb, pl.ds(T // 2 * p + 64 * rb + 8 * v, 8), :], BF16).astype(F32)
                        for rb in (2 * g, 2 * g + 1) for cb in range(2)))
                    for n, f in enumerate(fs):
                        xsums[p][5 * g + n, kt, pl.ds(16 * v, 16), :] = f.astype(BF16)
                    yield 25, [f[8:] for f in fs]

    def b_factors(j):
        for s in range(8):
            r = pl.ds(128 * j + 16 * s, 16)
            for kt in range(2):
                fs = _rhs_factors(*(bs[c, kt + 2 * kb, r, :].astype(F32) for kb in range(2) for c in range(2)))
                for n, f in enumerate(fs):
                    bfs[j][2 * n + kt, pl.ds(16 * s, 16), :] = f.astype(BF16)
                yield 34, [fs[n][8:] for n in (0, 2, 3, 5, 6)]

    lasts = [None] * NJ

    def scan(p, j):
        def power(i):
            return lamtab[j, 2 * i], lamtab[j, 2 * i + 1]

        for b in range(T // 64):
            hold("scan", bus[j], (0,), pl.ds(T * p + 64 * b, 8, stride=9))
            hs = []
            for i in range(8):
                st = pl.ds(T * p + 64 * b + 32 * ((i // 2) % 2) + 2 * (i // 4) + i % 2, 8, stride=4)
                u = (bus[j][0, st, :], bus[j][1, st, :])
                hs.append(u if i == 0 else _cadd(_cmul(power(0), hs[-1]), u))
            yield 58, list(hs[7]), CFG["scangate"]
            e = tuple(jnp.where(sub1 == 7, c0, c1) for c0, c1 in zip(lasts[j] or (0.0, 0.0), hs[7]))
            e = tuple(pltpu.roll(c, 1, 0) for c in e)
            for n, d_ in enumerate((1, 2, 4)):
                e = _cadd(e, _cmul(power(8 + n), tuple(pltpu.roll(c, d_, 0) for c in e)))
            yield 36, list(e), CFG["scangate"]
            for i0 in (1, 0):
                for i in range(i0, 8, 2):
                    hs[i] = _cadd(hs[i], _cmul(power(i), e))
                    if i == 7:
                        lasts[j] = hs[7]
                blk = [jnp.concatenate([hs[i][c], hs[i + 4][c]], axis=0) for i in (i0, i0 + 2) for c in range(2)]
                fs = _lhs_sums(*blk) + (blk[0], blk[3])
                for n, f in enumerate(fs):
                    hbs[p][n, j, pl.ds(32 * b + 16 * i0, 16), :] = f.astype(BF16)
                yield 52, [fs[0][8:], fs[1][:8], fs[4][8:]], CFG["scangate"]

    def fold_c(j, i):
        f_r, f_i = (jnp.concatenate([fvec[c, :, cols(j)]] * 2, axis=0) for c in range(2))
        f_n = -f_i

        def fold(d_, s, f_r):
            a, b = (cs[c, j, pl.ds(128 * d_ + 16 * s, 16), :].astype(F32) for c in range(2))
            return a * f_r - b * f_i, a * f_n - b * f_r

        for s in range(8):
            g_r = jnp.concatenate([held("c", fvec[0, :, cols(j)])] * 2, axis=0)
            if i < 2:
                (r0, i0), (r1, i1) = fold(2 * i, s, g_r), fold(2 * i + 1, s, g_r)
                fs = _rhs_factors(r0, r1, i0, i1)
            else:
                r0, i0 = fold(4, s, g_r)
                fs = (r0 - i0, i0, r0)
            for n, f in enumerate(fs):
                cps[i][n, j, pl.ds(16 * s, 16), :] = f.astype(BF16)
            yield (58, [fs[0][8:], fs[5][:8], fs[6][8:]]) if i < 2 else (28, [fs[0][8:]])

    def prep_kv(j, p):
        for mb in range(8):
            w = [rowp[2 + i, :, cols(j)] for i in range(4)]
            w[0], w[2] = held("kv", w[0]), held("kv", w[2])
            outs = [[] for _ in range(4)]
            for hf in range(2):
                at = T // 2 * p + 32 * mb + 16 * hf
                p0, p1, w0, w1 = (kw[j, pl.ds(HALO // 2 + at + o, 8, stride=2), :] for o in (-2, -1, 0, 1))
                kk = [_hi(p0), _lo(p1), _hi(p1), _lo(w0), _hi(w0), _lo(w1), _hi(w1)]
                v0, v1 = (vw[j, pl.ds(at + o, 8, stride=2), :] for o in (0, 1))
                vv = [_lo(v0), _hi(v0), _lo(v1), _hi(v1)]
                for r in range(4):
                    ksh = (kk[r] * w[3] + kk[r + 1] * w[2]) + (kk[r + 2] * w[1] + kk[r + 3] * w[0])
                    outs[r].append(ksh * vv[r])
                if hf == 0:
                    yield 47, [outs[r][0] for r in range(4)]
            for r in range(4):
                kvbs[j * NP + p][r, pl.ds(16 * mb, 16), :] = _rows16(*outs[r])
            yield 51, [outs[r][1] for r in range(4)]

    def prep_filter(j, p):
        raw = kraw.at[(j * NP + p) % 4]
        for a in range(4):
            raw[pl.ds(128 * a, 128), :] = ssm[cols(j), pl.ds(T * p + 128 * a, 128)].astype(F32).T
            for mb in (2 * a, 2 * a + 1):
                ws = [raw[pl.ds(64 * mb + r, 16, stride=4), :] for r in range(4)]
                for r in range(4):
                    ktbs[j * NP + p][r, pl.ds(16 * mb, 16), :] = ws[r].astype(BF16)
                yield 16, [w[8:] for w in ws]

    def bin_(ref, i, h, n):
        return tuple(ref[i, pl.ds(64 * h + 16 * n + c, 8, stride=2), :] for c in range(2))

    def product(j, i, a, prev):
        half = []
        for hs in ((0, 2), (1, 3)):
            y = []
            for h in hs:
                w = None
                for n in range(a + 1):
                    t_ = _cmul(bin_(khs[j], i, h, n), bin_(uhs[j], i, h, a - n))
                    w = t_ if w is None else _cadd(w, t_)
                y.append((w[0] + prev[h][1], w[1] - prev[h][0]) if a else w)
                prev[h] = w
                if a > 1 and h == hs[0]:
                    yield 8 * a + 8, list(y[0])
            half += [_cadd(*y), _csub(*y)]
            if hs[0] == 0 and a:
                yield (8 * a + 14 if a > 1 else 38), list(half[0])
        p_, q_, s_, t_ = half
        res = [_cadd(p_, s_), (q_[0] + t_[1], q_[1] - t_[0]), _csub(p_, s_), (q_[0] - t_[1], q_[1] + t_[0])]
        for r in range(4):
            ybs[j][a, r, pl.ds(16 * i, 16), :] = _rows16(*res[r])
        yield (46, 50, 36, 44)[a], [res[0][1], res[1][0]]

    def products(j, blocks, groups_):
        for i in groups_:
            hold("product", uhs[j], (i,), pl.ds(0, 8, stride=33))
            prev = [bin_(wprev, i, h, blocks[0] - 1) if blocks[0] else None for h in range(4)]
            for a in blocks:
                yield from product(j, i, a, prev)
            if a < NP - 1:
                for h in range(4):
                    for c in range(2):
                        wprev[i, pl.ds(64 * h + 16 * a + c, 8, stride=2), :] = prev[h][c]

    def mm(tie, lhs, rhs, dims):
        return lax.dot_general(pltpu.bitcast(tie(lhs), BF16), pltpu.bitcast(rhs, BF16), dims,
                               preferred_element_type=F32)

    def program(steps):
        m = {}
        for key, lhs, rhs, then in steps:
            def op(tie, key=key, lhs=lhs, rhs=rhs, then=then):
                d_ = mm(tie, lhs(), rhs(), NT)
                m[key] = m[key] + d_ if key in m else d_
                out = m[key][120:128]
                if then is not None:
                    then(m)
                return out
            yield CFG["projcost"], op

    def project_in(p, j):
        for g in range(2):
            def plain(rb, kt, g=g):
                return lambda: xrows(p, kt, 2 * g + rb)

            def put(rb, c, val, g=g):
                bus[j][c, pl.ds(T * p + 256 * g + 128 * rb, 128), :] = val

            def prod(n, key, then):
                def left(kt, g=g):
                    if n in (3, 4):
                        return plain(n - 3, 2 * (n - 3) + kt)
                    at = (5 * g + {1: 0, 2: 1, 5: 2, 6: 3, 7: 4}[n], kt)
                    return lambda: jnp.concatenate(
                        [xsums[p].bitcast(U32)[at + (_il(v), slice(None))] for v in (0, 2, 1, 3, 4, 6, 5, 7)], axis=0)
                return [(key, left(kt), lambda kt=kt: bfs[j].bitcast(U32)[2 * (n - 1) + kt], then if kt else None)
                        for kt in range(2)]

            lead = p == 0 and j in (0, 1, 3) and g == 0

            def after5(m, put=put, lead=lead):
                m["t01"] = m[3] + m[5]
                if lead:
                    put(0, 1, m["t01"] + m["l01"])

            def after4(m):
                m["t00"] = m[4] - m[5]

            def after2(m, put=put, lead=lead):
                m["t10"] = m[4] + m[2]
                m["t11"] = m[3] - m[2]
                if lead:
                    put(1, 0, m["t10"] + m["l10"])

            def after1(m):
                m["t00"] = m["t00"] + m[1]
                m["t11"] = m["t11"] + m[1]

            def finish(m, put=put):
                put(0, 0, m["t00"] + m["l00"])
                put(1, 1, m["t11"] + m["l11"])

            def fifth(key, rb, c, store=True):
                then = (lambda m, put=put: put(rb, c, m[key])) if store else None
                return [(key, plain(rb, 4), lambda: bw[c, 4, pl.ds(64 * j, 64), :], then)]

            if lead:
                steps = (sum((fifth(f"l{rb}{c}", rb, c, False) for rb in range(2) for c in range(2)), [])
                         + prod(3, 3, None) + prod(5, 5, after5) + prod(4, 4, after4) + prod(2, 2, after2)
                         + prod(1, 1, after1) + prod(7, "t00", None) + prod(6, "t11", finish))
            else:
                steps = (prod(3, 3, None) + prod(5, 5, after5) + fifth("t01", 0, 1) + prod(4, 4, after4)
                         + prod(2, 2, after2) + fifth("t10", 1, 0) + prod(1, 1, after1) + prod(7, "t00", None)
                         + fifth("t00", 0, 0) + prod(6, "t11", None) + fifth("t11", 1, 1))
            yield from program(steps)

    done = {}

    def project_out(p, unit, part):
        parts = [(0, unit, None), (1, unit, None), (0, 2, unit)] if unit < 2 else [(1, 2, 0), (1, 2, 1)]
        for g, i, half in [parts["xyz".index(part)]] if part else parts:
            def put(j, rb, val, g=g):
                dsk = rowp[0, :, cols(j)]
                for blk in range(4):
                    for late in range(2):
                        w = xvreg(p, j, 4 * g + blk, rb + 2 * late)
                        for i0, xv in enumerate((_lo(w), _hi(w))):
                            t0 = T * p + 64 * (4 * g + blk) + 2 * rb + 4 * late + i0
                            v = 4 * blk + 2 * i0 + late
                            oa[j, pl.ds(t0, 8, stride=8), :] = val[8 * v:8 * v + 8] + xv * dsk
                done[p, g, j] = done.get((p, g, j), 0) + 1
                if done[p, g, j] == 2:
                    start(("oa", p, g, j))

            def prod(ln, rn, key, then):
                return [(key, lambda kt=kt, g=g: hbs[p].bitcast(U32)[ln, kt, pl.ds(64 * g, 64), :],
                         lambda kt=kt, i=i: cps[i].bitcast(U32)[rn, kt], then if kt == NJ - 1 else None)
                        for kt in range(NJ)]

            if i < 2:
                def after4(m):
                    m["t00"] = m[4] - m[5]

                def after2(m, put=put, i=i):
                    put(2 * i, 1, m[2] + m[4])
                    m["t11"] = m[3] - m[2]

                def after1(m):
                    m["t00"] = m["t00"] + m[1]
                    m["t11"] = m["t11"] + m[1]

                steps = (prod(5, 2, 3, None)
                         + prod(2, 4, 5, lambda m, put=put, i=i: put(2 * i + 1, 0, m[3] + m[5]))
                         + prod(6, 3, 4, after4) + prod(1, 1, 2, after2) + prod(0, 0, 1, after1)
                         + prod(4, 6, "t00", lambda m, put=put, i=i: put(2 * i, 0, m["t00"]))
                         + prod(3, 5, "t11", lambda m, put=put, i=i: put(2 * i + 1, 1, m["t11"])))
            elif half == 0:
                steps = prod(5, 0, 0, None) + prod(2, 1, 0, lambda m, put=put: put(4, 0, m[0]))
            else:
                steps = prod(6, 0, 0, None) + prod(1, 2, 1, lambda m, put=put: put(4, 1, m[1] - m[0]))
            yield from program(steps)

    def forward(j, p):
        for src, dst in ((kvbs[j * NP + p], uhs[j]), (ktbs[j * NP + p], khs[j])):
            for hf in range(2):
                v = []
                for r in range(4):
                    def op(tie, src=src, dst=dst, hf=hf, r=r, v=v):
                        v.append(mm(tie, _get(tabw, (), 16 * r + 8 * hf), _get(src.bitcast(U32), (r,), 0), NN))
                        if r < 3:
                            return None
                        for i in range(8):
                            z = [(v[n][16 * i:16 * i + 8], v[n][16 * i + 8:16 * i + 16]) for n in range(4)]
                            a, b = _cadd(z[0], z[2]), _csub(z[0], z[2])
                            if dst is khs[j] and p == 0:
                                tap = rowp[1, :, cols(j)]
                                a, b = (a[0] + tap, a[1]), (b[0] + tap, b[1])
                            c, d_ = _cadd(z[1], z[3]), _csub(z[1], z[3])
                            res = [_cadd(a, c), (b[0] - d_[1], b[1] + d_[0]), _csub(a, c), (b[0] + d_[1], b[1] - d_[0])]
                            for h in range(4):
                                for e in range(2):
                                    dst[8 * hf + i, pl.ds(64 * h + 16 * p + e, 8, stride=2), :] = res[h][e]
                        return res[3][1] + res[2][0]
                    yield CFG["fwcost"], op

    def inverse(j, a):
        for r in range(4):
            acc = []
            for kt in range(2):
                def op(tie, r=r, kt=kt, acc=acc):
                    acc.append(mm(tie, _get(tabw, (), 64 + 16 * r + 8 * kt), _get(ybs[j].bitcast(U32), (a, r), 8 * kt), NN))
                    if kt == 0:
                        return None
                    y = acc[0] + acc[1]
                    for mb in range(16):
                        w = qw[j, pl.ds(T // 2 * a + 16 * mb + r // 2, 8, stride=2), :]
                        out = (_hi(w) if r % 2 else _lo(w)) * y[8 * mb:8 * mb + 8]
                        ob[j, pl.ds(T * a + 32 * mb + r, 8, stride=4), :] = out
                    if r == 3:
                        start(("ob", a, j))
                    return out
                yield CFG["ivcost"], op

    ops, first, last, wait_at, waits = [], {}, {}, {}, {}
    for word in words:
        if word.startswith("W:"):
            wait_at[word[2:]] = len(ops)
            waits.setdefault(len(ops), []).append(word[2:])
            continue
        k = int(word[1:].rstrip("xyz"))
        make, unit = {"a": (project_in, divmod(k, NJ)), "c": (project_out, divmod(k, 3)),
                      "f": (forward, divmod(k, NP)), "i": (inverse, divmod(k, NP))}[word[0]]
        key = (word[0],) + unit
        first.setdefault(key, len(ops))
        ops += list(make(*unit, word[1:].lstrip("0123456789")) if word[0] == "c" else make(*unit))
        last[key] = len(ops)

    lag = CFG["lag"]
    tasks = [[wait_at["rows"] + 4, wait_at["rows"], 100, row_params()]]
    for p in range(NP):
        if p:
            tasks.append([first["a", p, 0], wait_at[f"x{p}"], 800, x_sums(p, (0, 1))])
        for j in range(NJ):
            due = min(first["c", p, i] for i in range(3)) - CFG["scandue"] * p
            tasks.append([due, last["a", p, j] + lag, 1584, scan(p, j)])
            tasks.append([first["f", j, p], max(wait_at[f"kv{j}"], wait_at["rows"] + 4), 784, prep_kv(j, p)])
            tasks.append([first["f", j, p] + 8, wait_at[f"kv{j}"], 128, prep_filter(j, p)])
    for j in range(NJ):
        if j:
            tasks.append([first["a", 0, j], wait_at[f"b{(j + 1) // 2}"], 512, b_factors(j)])
        for i in range(3):
            due = min(first["c", p, n] for p in range(NP) for n in ((0,), (1,), (0, 1, 2))[i])
            tasks.append([due, wait_at["cb" if i == 1 else "ca"], 464 if i < 2 else 224, fold_c(j, i)])
        ready = max(last["f", j, p] for p in range(NP)) + lag
        for blocks, part in ([((0, 1), range(16)), ((2,), range(16)), ((3,), range(16))] if j == NJ - 1 else
                             [((0, 1, 2, 3), range(4 * i, 4 * i + 4)) for i in range(4)]):
            cost = len(part) * sum((48, 90, 112, 152)[a] for a in blocks) if j == NJ - 1 else 1632
            tasks.append([min(first["i", j, a] for a in blocks), ready, cost, products(j, blocks, part)])
    tasks.sort(key=lambda t_: t_[0])
    cum = [0.0]
    for n, (c, _) in enumerate(ops):
        quiet = any(n + ahead in waits for ahead in range(1, CFG["quiet"] + 1))
        cum.append(cum[-1] + (0.0 if quiet else max(CFG["rate"] - c, 0.0)))

    start_through("x0c")
    wait("par")
    start_through(CFG["ahead"]["par"])
    aid["never"] = jnp.full((8, 128), z_v[0], jnp.int32) != 0
    discretise()
    for key, task in (("b0", b_factors(0)), ("x0a", x_sums(0, (0,))), ("x0b", x_sums(0, (1,)))):
        wait(key)
        for _ in task:
            pass

    budget, back, later = 0.0, [], {}
    for n in range(0, len(ops), 4):
        for key in waits.get(n, ()):
            wait(key)
        for key in waits.get(n, ()):
            later.clear()
            start_through(CFG["ahead"].get(key))
        room = cum[n + 4] - cum[n]
        need = max([0.0] + [sum(t2[2] for t2 in tasks[:i + 1]) / max(cum[max(t_[0] - CFG["early"], 0)] - cum[n], room, 1)
                            for i, t_ in enumerate(tasks)])
        budget = min(budget, 0.0) + room * min(need, CFG["cap"])
        for kind, behind in (("product", CFG["holdlag"]), ("scan", CFG["scanlag"])):
            aid[kind] = back[-behind][-1] if len(back) >= behind else None
        steps = []
        for t_ in list(tasks):
            urgent = t_[0] < n + 4
            if t_[1] > n and not urgent:
                continue
            while budget > 0 or urgent:
                step = next(t_[3], None)
                if step is None:
                    tasks.remove(t_)
                    break
                if not urgent:
                    budget -= step[0]
                    t_[2] -= step[0]
                    steps.append((step[0], step[1][-2:], sum(step[2:])))
        total, acc = sum(t_[0] for t_ in steps), 0
        for i, (cost, vals, slack) in enumerate(steps):
            acc += cost
            later.setdefault(2 * n + CFG["gate"] + slack + int(8 * acc / (total + 1)), []).append((i % 4, vals))
        gates = [[[] for _ in range(8)] for _ in range(4)]
        for pos in range(8):
            for i, vals in later.pop(2 * n + pos, ()):
                gates[i][pos] += vals
        if len(back) >= CFG["natlag"]:
            for gate, val in zip(gates, back[-CFG["natlag"]]):
                gate[0].append(val)
        back.append([])
        for (_, op), gate in zip(ops[n:n + 4], gates):
            def tie(lhs, gate=gate):
                parts = [lhs[8 * i:8 * i + 8] for i in range(8)]
                for i, vals in enumerate(gate):
                    if vals:
                        both = functools.reduce(jnp.bitwise_or, [pltpu.bitcast(val, U32) for val in vals])
                        parts[i] = jnp.where(aid["never"], both, parts[i])
                return jnp.concatenate(parts, axis=0)

            out = op(tie)
            if out is not None:
                back[-1].append(out)
    assert not tasks and not queue
    for c in pending.values():
        c.wait()


@jax.jit
def pallas_concat_heads__ssm_conv_s5__ssm_conv_h3__prompt_kernel(
    A_x, A_Lambda_re, A_Lambda_im, A_B_re, A_B_im, A_C_re, A_C_im, A_log_dt, A_Dskip,
    B_q, B_k, B_v, B_shift_k, B_ssm_k, B_ssm_D,
):
    V = pltpu.VMEM
    scratch = [
        V((NJ, S, 128), BF16), V((NJ, S + HALO, 128), BF16), V((NJ, S, 128), BF16), V((NJ, S, 128), BF16),
        V((D, S), BF16), V((2, NJ, D, 128), BF16), V((2, NJ, D, 128), BF16),
        V((D,), BF16), V((D,), BF16), V((D,), BF16), V((D,), BF16), V((D,), BF16), V((4, D), BF16),
        V((2048, 128), BF16), pltpu.SMEM((1,), jnp.int32),
        V((NJ, 22, 8, 128), F32), V((2, 8, D), F32), V((6, 8, D), F32), V((4, T, 128), F32),
        V((NJ, S, 128), F32), V((NJ, S, 128), F32), V((16, 256, 128), F32),
        pltpu.SemaphoreType.DMA((NSEM,)),
    ]
    scratch += [V((10, 2, 128, 128), BF16)] * NP + [V((14, 128, 128), BF16)] * NJ
    scratch += [V((7, NJ, 128, 128), BF16)] * 3 + [V((7, NJ, T // 2, 128), BF16)] * NP
    scratch += [V((4, 128, 128), BF16)] * (2 * NP * NJ)
    scratch += [V((16, 256, 128), F32)] * (2 * NJ) + [V((NP, 4, 256, 128), BF16)] * NJ
    scratch += [V((2, S, 128), F32)] * NJ
    out = pl.pallas_call(
        _kernel,
        out_shape=jax.ShapeDtypeStruct((S, 2 * D), F32),
        in_specs=[pl.BlockSpec(memory_space=pl.ANY)] * 17,
        out_specs=pl.BlockSpec(memory_space=pl.ANY),
        scratch_shapes=scratch,
        compiler_params=pltpu.CompilerParams(vmem_limit_bytes=110 * 1024 * 1024),
        name="s5_h3",
    )(A_x.reshape(S, D), A_Lambda_re, A_Lambda_im, A_B_re, A_B_im, A_C_re, A_C_im, A_log_dt, A_Dskip,
      B_q.reshape(S, D), B_k.reshape(S, D), B_v.reshape(S, D), B_shift_k.T, B_ssm_k, B_ssm_D,
      jnp.asarray(_dft_tables()), jnp.asarray(np.zeros((1,), np.int32)))
    return out.reshape(1, S, 2 * D)
```

```python
import functools

import numpy as np
import jax
import jax.numpy as jnp
from jax import lax
import jax.experimental.pallas as pl
import jax.experimental.pallas.tpu as pltpu

S, D = 2048, 640
T = 512
NP, NJ = 4, 5
NSEM = 6
HALO = 16
F32, BF16, U32 = jnp.float32, jnp.bfloat16, jnp.uint32
NT = (((1,), (1,)), ((), ()))
NN = (((1,), (0,)), ((), ()))
B_ROWS = (pl.ds(0, 128), pl.ds(128, 256), pl.ds(384, 256))
C_ROWS = (pl.ds(0, 256), pl.ds(256, 256), pl.ds(512, 128))

ORDER = ("W:x0c a0 W:b1 a1 a2 W:b2 W:x1 a3 a4 a5 a6 "
         "W:rows W:x2 W:kv0 a7 f0 a8 a9 a10 f1 a11 f2 f3 a12 a13 "
         "W:x3 W:kv1 W:kv2 W:ca a14 a15 f4 a16 f5 a17 f6 f7 a18 f8 f9 a19 c0 f10 c2 f11 c5 "
         "W:cb W:kv3 W:kv4 W:g W:q c3 i0 i1 f12 c1 i2 f13 f14 i3 f15 c4x i4 f16 c4y i5 c4z f17 f18 i6 f19 "
         "c6 i7 i8 c7 i9 i10 i11 c8 i12 i13 c9x i14 c9y i15 c9z i16 i17 c10x i18 c10y i19 c10z c11")
LOADS = "par b0 x0a x0b x0c b1 b2 x1 rows x2 kv0 x3 kv1 kv2 ca cb kv3 kv4 g q"
CFG = dict(
    ahead={"par": "b1", "x0c": "kv0", "b1": "kv1", "x1": "kv2", "kv0": "kv4", "x3": "q"},
    rate=72.0,
    cap=1.5,
    fwcost=40, ivcost=40, projcost=22,
    lag=8,
    early=16,
    quiet=8,
    scandue=80,
    gate=16, scangate=8,
    natlag=3,
    holdlag=5, scanlag=12,
)


def _dft_tables():
    g = np.arange(128)[:, None]
    m = np.arange(128)[None, :]
    fwd = np.zeros((4, 256, 128), np.float64)
    for r in range(4):
        th = np.pi * (((4 * g + 1) * (4 * m + r)) % 2048) / 1024.0
        c = np.cos(th).reshape(16, 8, 128)
        s = np.sin(th).reshape(16, 8, 128)
        fwd[r] = np.stack([c, s], axis=1).reshape(256, 128)
    inv = np.transpose(fwd, (0, 2, 1)) / 512.0
    perm = np.arange(128).reshape(4, 8, 2, 2).transpose(0, 2, 1, 3).reshape(128)
    fwd = fwd[:, :, perm]
    inv = inv.reshape(4, 128, 2, 128).transpose(0, 2, 1, 3)[..., perm]
    tab = np.concatenate([fwd.reshape(1024, 128), inv.reshape(1024, 128)], axis=0)
    tab = tab.reshape(64, 2, 8, 2, 128).transpose(0, 2, 1, 3, 4).reshape(2048, 128)
    return tab.astype(jnp.bfloat16)


def _lo(w):
    return pltpu.bitcast(w << 16, F32)


def _hi(w):
    return pltpu.bitcast(w & jnp.uint32(0xFFFF0000), F32)


def _rows16(a, b):
    return jnp.concatenate([a, b], axis=0).astype(BF16)


def _il(v):
    return pl.ds(16 * (v // 2) + v % 2, 8, stride=2)


def _get(ref, idx, v0):
    return jnp.concatenate([ref[idx + (_il(v), slice(None))] for v in range(v0, v0 + 8)], axis=0)


def _cmul(a, b):
    return a[0] * b[0] - a[1] * b[1], a[0] * b[1] + a[1] * b[0]


def _cadd(a, b):
    return a[0] + b[0], a[1] + b[1]


def _csub(a, b):
    return a[0] - b[0], a[1] - b[1]


def _lhs_sums(a11, a12, a21, a22):
    return a11 + a22, a21 + a22, a11 + a12, a21 - a11, a12 - a22


def _rhs_factors(b11, b12, b21, b22):
    return b11 + b22, b11, b12 - b22, b21 - b11, b22, b11 + b12, b21 + b22


def _load_groups():
    groups = {"par": ["lre", "lim", "ldt", "z"], "rows": ["dsk", "sd", "sh", "f"], "g": ["g"],
              "ca": [("c", g, c, j) for g in (0, 2) for j in range(NJ) for c in range(2)],
              "cb": [("c", 1, c, j) for j in range(NJ) for c in range(2)],
              "q": [("q", j) for j in range(NJ)],
              "x0a": [("x", 0, 0), ("x", 0, 2)], "x0b": [("x", 0, 1), ("x", 0, 3)], "x0c": [("x", 0, 4)]}
    for g in range(len(B_ROWS)):
        groups[f"b{g}"] = [("b", g, c, kt) for kt in range(NJ) for c in range(2)]
    for j in range(NJ):
        groups[f"kv{j}"] = [("k", j), ("v", j), ("ssm", j)]
    for p in range(1, NP):
        groups[f"x{p}"] = [("x", p, j) for j in range(NJ)]
    return groups


def _kernel(x_hbm, lre_hbm, lim_hbm, bre_hbm, bim_hbm, cre_hbm, cim_hbm, ldt_hbm, dsk_hbm,
            q_hbm, k_hbm, v_hbm, sh_hbm, ssm_hbm, sd_hbm, tab_hbm, z_hbm,
            o_hbm,
            xs, ks, vs, qs, ssm, bs, cs,
            lre_v, lim_v, ldt_v, dsk_v, sd_v, sh_v, tab_v, z_v,
            lamtab, fvec, rowp, kraw, oa, ob, wprev, sem, *rest):
    rest = list(rest)
    xsums, bfs, cps, hbs, kvbs, ktbs, uhs, khs, ybs, bus = (
        [rest.pop(0) for _ in range(n)] for n in (NP, NJ, 3, NP, NJ * NP, NJ * NP, NJ, NJ, NJ, NJ))

    def cols(j):
        return pl.ds(128 * j, 128)

    def rows(p):
        return pl.ds(T * p, T)

    copies = {"lre": (lre_hbm, lre_v), "lim": (lim_hbm, lim_v), "ldt": (ldt_hbm, ldt_v), "z": (z_hbm, z_v),
              "dsk": (dsk_hbm, dsk_v), "sd": (sd_hbm, sd_v), "sh": (sh_hbm, sh_v),
              "f": (tab_hbm.at[pl.ds(0, 1024), :], tab_v.at[pl.ds(0, 1024), :]),
              "g": (tab_hbm.at[pl.ds(1024, 1024), :], tab_v.at[pl.ds(1024, 1024), :])}
    for j in range(NJ):
        for c, (b_hbm, c_hbm) in enumerate(((bre_hbm, cre_hbm), (bim_hbm, cim_hbm))):
            for g, r in enumerate(C_ROWS):
                copies["c", g, c, j] = (c_hbm.at[r, cols(j)], cs.at[c, j, r, :])
            for g, r in enumerate(B_ROWS):
                copies["b", g, c, j] = (b_hbm.at[r, cols(j)], bs.at[c, j, r, :])
        copies["k", j] = (k_hbm.at[:, cols(j)], ks.at[j, pl.ds(HALO, S), :])
        copies["v", j] = (v_hbm.at[:, cols(j)], vs.at[j])
        copies["q", j] = (q_hbm.at[:, cols(j)], qs.at[j])
        copies["ssm", j] = (ssm_hbm.at[cols(j), :], ssm.at[cols(j), :])
        for p in range(NP):
            copies["x", p, j] = (x_hbm.at[rows(p), cols(j)], xs.at[j, rows(p), :])
            for g in range(2):
                r = pl.ds(T * p + T // 2 * g, T // 2)
                copies["oa", p, g, j] = (oa.at[j, r, :], o_hbm.at[r, cols(j)])
            copies["ob", p, j] = (ob.at[j, rows(p), :], o_hbm.at[rows(p), cols(NJ + j)])

    groups = _load_groups()
    words = ORDER.split()
    slot = {n: batch for batch, key in enumerate(("par", "b0", "x0a", "x0b")) for n in groups[key]}
    batch = 3
    for before, word in zip([""] + words, words):
        if word.startswith("W:"):
            batch += not before.startswith("W:")
            slot.update({n: batch for n in groups[word[2:]]})
    queue, pending = LOADS.split(), {}

    def start(name):
        c = pltpu.make_async_copy(*copies[name], sem.at[slot.get(name, batch + 1) % NSEM])
        c.start()
        pending[name] = c

    def start_through(key):
        while key in queue:
            for name in groups[queue.pop(0)]:
                start(name)

    def wait(key):
        for name in groups[key]:
            pending.pop(name).wait()

    xw, kw, vw, qw, tabw, bw = (r.bitcast(U32) for r in (xs, ks, vs, qs, tab_v, bs))
    sub1 = lax.broadcasted_iota(jnp.int32, (8, 128), 0)

    def bcast(ref):
        return jnp.broadcast_to(ref[...].astype(F32).reshape(1, D), (8, D))

    def xvreg(p, j, b, m):
        return xw[j, pl.ds(T // 2 * p + 32 * b + m, 8, stride=4), :]

    def xrows(p, j, rb):
        return jnp.concatenate([xw[j, _il(T // 16 * p + 8 * rb + v), :] for v in (0, 2, 1, 3, 4, 6, 5, 7)], axis=0)

    aid = dict(never=None, scan=None, product=None)

    def hold(kind, ref, idx, stride):
        if aid[kind] is not None:
            r = idx + (stride, slice(None))
            ref[r] = jnp.where(aid["never"], aid[kind], ref[r])

    def held(val):
        if aid["product"] is None:
            return val
        return jnp.where(aid["never"], aid["product"], val)

    def discretise():
        lr, li = bcast(lre_v), bcast(lim_v)
        dt = jnp.exp(bcast(ldt_v)).astype(BF16).astype(F32)
        mag = jnp.exp(dt * lr)
        lam = (mag * jnp.cos(dt * li), mag * jnp.sin(dt * li))
        nr, ni = lam[0] - 1.0, lam[1]
        big = jnp.abs(lr) >= jnp.abs(li)
        ratio = jnp.where(big, li / lr, lr / li)
        den = jnp.where(big, lr + li * ratio, li + lr * ratio)
        fvec[0] = 2.0 * jnp.where(big, nr + ni * ratio, nr * ratio + ni) / den
        fvec[1] = 2.0 * jnp.where(big, ni - nr * ratio, ni * ratio - nr) / den
        pw = [lam]
        for i in range(1, 8):
            pw.append(_cmul(pw[(i - 1) // 2], pw[i - 1 - (i - 1) // 2]))
        mu1 = pw[7]
        mu2 = _cmul(mu1, mu1)
        mu4 = _cmul(mu2, mu2)
        sub = lax.broadcasted_iota(jnp.int32, (8, D), 0)
        tab = [c for z in pw for c in z]
        for d_, mu in ((1, mu1), (2, mu2), (4, mu4)):
            tab += [jnp.where(sub >= d_, mu[0], 0.0), jnp.where(sub >= d_, mu[1], 0.0)]
        for j in range(NJ):
            for i, t_ in enumerate(tab):
                lamtab[j, i] = t_[:, 128 * j:128 * (j + 1)]
            ks[j, pl.ds(0, HALO), :] = jnp.zeros((HALO, 128), BF16)

    def row_params():
        rowp[0] = bcast(dsk_v)
        rowp[1] = bcast(sd_v)
        sh = sh_v[...].astype(F32)
        for i in range(4):
            rowp[2 + i] = jnp.broadcast_to(sh[i:i + 1], (8, D))
        yield 100, []

    def x_sums(p, kts):
        for g in range(2):
            for kt in kts:
                for v in range(8):
                    fs = _lhs_sums(*(
                        pltpu.bitcast(xw[kt + 2 * cb, pl.ds(T // 2 * p + 64 * rb + 8 * v, 8), :], BF16).astype(F32)
                        for rb in (2 * g, 2 * g + 1) for cb in range(2)))
                    for n, f in enumerate(fs):
                        xsums[p][5 * g + n, kt, pl.ds(16 * v, 16), :] = f.astype(BF16)
                    yield 25, [f[8:] for f in fs]

    def b_factors(j):
        for s in range(8):
            r = pl.ds(128 * j + 16 * s, 16)
            for kt in range(2):
                fs = _rhs_factors(*(bs[c, kt + 2 * kb, r, :].astype(F32) for kb in range(2) for c in range(2)))
                for n, f in enumerate(fs):
                    bfs[j][2 * n + kt, pl.ds(16 * s, 16), :] = f.astype(BF16)
                yield 34, [fs[n][8:] for n in (0, 2, 3, 5, 6)]

    lasts = [None] * NJ

    def scan(p, j):
        def power(i):
            return lamtab[j, 2 * i], lamtab[j, 2 * i + 1]

        for b in range(T // 64):
            hold("scan", bus[j], (0,), pl.ds(T * p + 64 * b, 8, stride=9))
            hs = []
            for i in range(8):
                st = pl.ds(T * p + 64 * b + 32 * ((i // 2) % 2) + 2 * (i // 4) + i % 2, 8, stride=4)
                u = (bus[j][0, st, :], bus[j][1, st, :])
                hs.append(u if i == 0 else _cadd(_cmul(power(0), hs[-1]), u))
            yield 58, list(hs[7]), CFG["scangate"]
            e = tuple(jnp.where(sub1 == 7, c0, c1) for c0, c1 in zip(lasts[j] or (0.0, 0.0), hs[7]))
            e = tuple(pltpu.roll(c, 1, 0) for c in e)
            for n, d_ in enumerate((1, 2, 4)):
                e = _cadd(e, _cmul(power(8 + n), tuple(pltpu.roll(c, d_, 0) for c in e)))
            yield 36, list(e), CFG["scangate"]
            for i0 in (1, 0):
                for i in range(i0, 8, 2):
                    hs[i] = _cadd(hs[i], _cmul(power(i), e))
                    if i == 7:
                        lasts[j] = hs[7]
                blk = [jnp.concatenate([hs[i][c], hs[i + 4][c]], axis=0) for i in (i0, i0 + 2) for c in range(2)]
                fs = _lhs_sums(*blk) + (blk[0], blk[3])
                for n, f in enumerate(fs):
                    hbs[p][n, j, pl.ds(32 * b + 16 * i0, 16), :] = f.astype(BF16)
                yield 52, [fs[0][8:], fs[1][:8], fs[4][8:]], CFG["scangate"]

    def fold_c(j, i):
        f_r, f_i = (jnp.concatenate([fvec[c, :, cols(j)]] * 2, axis=0) for c in range(2))
        f_n = -f_i

        def fold(d_, s, f_r):
            a, b = (cs[c, j, pl.ds(128 * d_ + 16 * s, 16), :].astype(F32) for c in range(2))
            return a * f_r - b * f_i, a * f_n - b * f_r

        for s in range(8):
            g_r = jnp.concatenate([held(fvec[0, :, cols(j)])] * 2, axis=0)
            if i < 2:
                (r0, i0), (r1, i1) = fold(2 * i, s, g_r), fold(2 * i + 1, s, g_r)
                fs = _rhs_factors(r0, r1, i0, i1)
            else:
                r0, i0 = fold(4, s, g_r)
                fs = (r0 - i0, i0, r0)
            for n, f in enumerate(fs):
                cps[i][n, j, pl.ds(16 * s, 16), :] = f.astype(BF16)
            yield (58, [fs[0][8:], fs[5][:8], fs[6][8:]]) if i < 2 else (28, [fs[0][8:]])

    def prep_kv(j, p):
        for mb in range(8):
            w = [rowp[2 + i, :, cols(j)] for i in range(4)]
            w[0], w[2] = held(w[0]), held(w[2])
            outs = [[] for _ in range(4)]
            for hf in range(2):
                at = T // 2 * p + 32 * mb + 16 * hf
                p0, p1, w0, w1 = (kw[j, pl.ds(HALO // 2 + at + o, 8, stride=2), :] for o in (-2, -1, 0, 1))
                kk = [_hi(p0), _lo(p1), _hi(p1), _lo(w0), _hi(w0), _lo(w1), _hi(w1)]
                v0, v1 = (vw[j, pl.ds(at + o, 8, stride=2), :] for o in (0, 1))
                vv = [_lo(v0), _hi(v0), _lo(v1), _hi(v1)]
                for r in range(4):
                    ksh = (kk[r] * w[3] + kk[r + 1] * w[2]) + (kk[r + 2] * w[1] + kk[r + 3] * w[0])
                    outs[r].append(ksh * vv[r])
                if hf == 0:
                    yield 47, [outs[r][0] for r in range(4)]
            for r in range(4):
                kvbs[j * NP + p][r, pl.ds(16 * mb, 16), :] = _rows16(*outs[r])
            yield 51, [outs[r][1] for r in range(4)]

    def prep_filter(j, p):
        raw = kraw.at[(j * NP + p) % 4]
        for a in range(4):
            raw[pl.ds(128 * a, 128), :] = ssm[cols(j), pl.ds(T * p + 128 * a, 128)].astype(F32).T
            for mb in (2 * a, 2 * a + 1):
                ws = [raw[pl.ds(64 * mb + r, 16, stride=4), :] for r in range(4)]
                for r in range(4):
                    ktbs[j * NP + p][r, pl.ds(16 * mb, 16), :] = ws[r].astype(BF16)
                yield 16, [w[8:] for w in ws]

    def bin_(ref, i, h, n):
        return tuple(ref[i, pl.ds(64 * h + 16 * n + c, 8, stride=2), :] for c in range(2))

    def product(j, i, a, prev):
        half = []
        for hs in ((0, 2), (1, 3)):
            y = []
            for h in hs:
                w = None
                for n in range(a + 1):
                    t_ = _cmul(bin_(khs[j], i, h, n), bin_(uhs[j], i, h, a - n))
                    w = t_ if w is None else _cadd(w, t_)
                y.append((w[0] + prev[h][1], w[1] - prev[h][0]) if a else w)
                prev[h] = w
                if a > 1 and h == hs[0]:
                    yield 8 * a + 8, list(y[0])
            half += [_cadd(*y), _csub(*y)]
            if hs[0] == 0 and a:
                yield (8 * a + 14 if a > 1 else 38), list(half[0])
        p_, q_, s_, t_ = half
        res = [_cadd(p_, s_), (q_[0] + t_[1], q_[1] - t_[0]), _csub(p_, s_), (q_[0] - t_[1], q_[1] + t_[0])]
        for r in range(4):
            ybs[j][a, r, pl.ds(16 * i, 16), :] = _rows16(*res[r])
        yield (46, 50, 36, 44)[a], [res[0][1], res[1][0]]

    def products(j, blocks, groups_):
        for i in groups_:
            hold("product", uhs[j], (i,), pl.ds(0, 8, stride=33))
            prev = [bin_(wprev, i, h, blocks[0] - 1) if blocks[0] else None for h in range(4)]
            for a in blocks:
                yield from product(j, i, a, prev)
            if a < NP - 1:
                for h in range(4):
                    for c in range(2):
                        wprev[i, pl.ds(64 * h + 16 * a + c, 8, stride=2), :] = prev[h][c]

    def mm(tie, lhs, rhs, dims):
        return lax.dot_general(pltpu.bitcast(tie(lhs), BF16), pltpu.bitcast(rhs, BF16), dims,
                               preferred_element_type=F32)

    def program(steps):
        m = {}
        for key, lhs, rhs, then in steps:
            def op(tie, key=key, lhs=lhs, rhs=rhs, then=then):
                d_ = mm(tie, lhs(), rhs(), NT)
                m[key] = m[key] + d_ if key in m else d_
                out = m[key][120:128]
                if then is not None:
                    then(m)
                return out
            yield CFG["projcost"], op

    def project_in(p, j):
        for g in range(2):
            def plain(rb, kt, g=g):
                return lambda: xrows(p, kt, 2 * g + rb)

            def put(rb, c, val, g=g):
                bus[j][c, pl.ds(T * p + 256 * g + 128 * rb, 128), :] = val

            def prod(n, key, then):
                def left(kt, g=g):
                    if n in (3, 4):
                        return plain(n - 3, 2 * (n - 3) + kt)
                    at = (5 * g + {1: 0, 2: 1, 5: 2, 6: 3, 7: 4}[n], kt)
                    return lambda: jnp.concatenate(
                        [xsums[p].bitcast(U32)[at + (_il(v), slice(None))] for v in (0, 2, 1, 3, 4, 6, 5, 7)], axis=0)
                return [(key, left(kt), lambda kt=kt: bfs[j].bitcast(U32)[2 * (n - 1) + kt], then if kt else None)
                        for kt in range(2)]

            lead = p == 0 and j in (0, 1, 3) and g == 0

            def after5(m, put=put, lead=lead):
                m["t01"] = m[3] + m[5]
                if lead:
                    put(0, 1, m["t01"] + m["l01"])

            def after4(m):
                m["t00"] = m[4] - m[5]

            def after2(m, put=put, lead=lead):
                m["t10"] = m[4] + m[2]
                m["t11"] = m[3] - m[2]
                if lead:
                    put(1, 0, m["t10"] + m["l10"])

            def after1(m):
                m["t00"] = m["t00"] + m[1]
                m["t11"] = m["t11"] + m[1]

            def finish(m, put=put):
                put(0, 0, m["t00"] + m["l00"])
                put(1, 1, m["t11"] + m["l11"])

            def fifth(key, rb, c, store=True):
                then = (lambda m, put=put: put(rb, c, m[key])) if store else None
                return [(key, plain(rb, 4), lambda: bw[c, 4, pl.ds(64 * j, 64), :], then)]

            if lead:
                steps = (sum((fifth(f"l{rb}{c}", rb, c, False) for rb in range(2) for c in range(2)), [])
                         + prod(3, 3, None) + prod(5, 5, after5) + prod(4, 4, after4) + prod(2, 2, after2)
                         + prod(1, 1, after1) + prod(7, "t00", None) + prod(6, "t11", finish))
            else:
                steps = (prod(3, 3, None) + prod(5, 5, after5) + fifth("t01", 0, 1) + prod(4, 4, after4)
                         + prod(2, 2, after2) + fifth("t10", 1, 0) + prod(1, 1, after1) + prod(7, "t00", None)
                         + fifth("t00", 0, 0) + prod(6, "t11", None) + fifth("t11", 1, 1))
            yield from program(steps)

    done = {}

    def project_out(p, unit, part):
        parts = [(0, unit, None), (1, unit, None), (0, 2, unit)] if unit < 2 else [(1, 2, 0), (1, 2, 1)]
        for g, i, half in [parts["xyz".index(part)]] if part else parts:
            def put(j, rb, val, g=g):
                dsk = rowp[0, :, cols(j)]
                for blk in range(4):
                    for late in range(2):
                        w = xvreg(p, j, 4 * g + blk, rb + 2 * late)
                        for i0, xv in enumerate((_lo(w), _hi(w))):
                            t0 = T * p + 64 * (4 * g + blk) + 2 * rb + 4 * late + i0
                            v = 4 * blk + 2 * i0 + late
                            oa[j, pl.ds(t0, 8, stride=8), :] = val[8 * v:8 * v + 8] + xv * dsk
                done[p, g, j] = done.get((p, g, j), 0) + 1
                if done[p, g, j] == 2:
                    start(("oa", p, g, j))

            def prod(ln, rn, key, then):
                return [(key, lambda kt=kt, g=g: hbs[p].bitcast(U32)[ln, kt, pl.ds(64 * g, 64), :],
                         lambda kt=kt, i=i: cps[i].bitcast(U32)[rn, kt], then if kt == NJ - 1 else None)
                        for kt in range(NJ)]

            if i < 2:
                def after4(m):
                    m["t00"] = m[4] - m[5]

                def after2(m, put=put, i=i):
                    put(2 * i, 1, m[2] + m[4])
                    m["t11"] = m[3] - m[2]

                def after1(m):
                    m["t00"] = m["t00"] + m[1]
                    m["t11"] = m["t11"] + m[1]

                steps = (prod(5, 2, 3, None)
                         + prod(2, 4, 5, lambda m, put=put, i=i: put(2 * i + 1, 0, m[3] + m[5]))
                         + prod(6, 3, 4, after4) + prod(1, 1, 2, after2) + prod(0, 0, 1, after1)
                         + prod(4, 6, "t00", lambda m, put=put, i=i: put(2 * i, 0, m["t00"]))
                         + prod(3, 5, "t11", lambda m, put=put, i=i: put(2 * i + 1, 1, m["t11"])))
            elif half == 0:
                steps = prod(5, 0, 0, None) + prod(2, 1, 0, lambda m, put=put: put(4, 0, m[0]))
            else:
                steps = prod(6, 0, 0, None) + prod(1, 2, 1, lambda m, put=put: put(4, 1, m[1] - m[0]))
            yield from program(steps)

    def forward(j, p):
        for src, dst in ((kvbs[j * NP + p], uhs[j]), (ktbs[j * NP + p], khs[j])):
            for hf in range(2):
                v = []
                for r in range(4):
                    def op(tie, src=src, dst=dst, hf=hf, r=r, v=v):
                        v.append(mm(tie, _get(tabw, (), 16 * r + 8 * hf), _get(src.bitcast(U32), (r,), 0), NN))
                        if r < 3:
                            return None
                        for i in range(8):
                            z = [(v[n][16 * i:16 * i + 8], v[n][16 * i + 8:16 * i + 16]) for n in range(4)]
                            a, b = _cadd(z[0], z[2]), _csub(z[0], z[2])
                            if dst is khs[j] and p == 0:
                                tap = rowp[1, :, cols(j)]
                                a, b = (a[0] + tap, a[1]), (b[0] + tap, b[1])
                            c, d_ = _cadd(z[1], z[3]), _csub(z[1], z[3])
                            res = [_cadd(a, c), (b[0] - d_[1], b[1] + d_[0]), _csub(a, c), (b[0] + d_[1], b[1] - d_[0])]
                            for h in range(4):
                                for e in range(2):
                                    dst[8 * hf + i, pl.ds(64 * h + 16 * p + e, 8, stride=2), :] = res[h][e]
                        return res[3][1] + res[2][0]
                    yield CFG["fwcost"], op

    def inverse(j, a):
        for r in range(4):
            acc = []
            for kt in range(2):
                def op(tie, r=r, kt=kt, acc=acc):
                    acc.append(mm(tie, _get(tabw, (), 64 + 16 * r + 8 * kt), _get(ybs[j].bitcast(U32), (a, r), 8 * kt), NN))
                    if kt == 0:
                        return None
                    y = acc[0] + acc[1]
                    for mb in range(16):
                        w = qw[j, pl.ds(T // 2 * a + 16 * mb + r // 2, 8, stride=2), :]
                        out = (_hi(w) if r % 2 else _lo(w)) * y[8 * mb:8 * mb + 8]
                        ob[j, pl.ds(T * a + 32 * mb + r, 8, stride=4), :] = out
                    if r == 3:
                        start(("ob", a, j))
                    return out
                yield CFG["ivcost"], op

    ops, first, last, wait_at, waits = [], {}, {}, {}, {}
    for word in words:
        if word.startswith("W:"):
            wait_at[word[2:]] = len(ops)
            waits.setdefault(len(ops), []).append(word[2:])
            continue
        k = int(word[1:].rstrip("xyz"))
        make, unit = {"a": (project_in, divmod(k, NJ)), "c": (project_out, divmod(k, 3)),
                      "f": (forward, divmod(k, NP)), "i": (inverse, divmod(k, NP))}[word[0]]
        key = (word[0],) + unit
        first.setdefault(key, len(ops))
        ops += list(make(*unit, word[1:].lstrip("0123456789")) if word[0] == "c" else make(*unit))
        last[key] = len(ops)

    lag = CFG["lag"]
    tasks = [[wait_at["rows"] + 4, wait_at["rows"], 100, row_params()]]
    for p in range(NP):
        if p:
            tasks.append([first["a", p, 0], wait_at[f"x{p}"], 800, x_sums(p, (0, 1))])
        for j in range(NJ):
            due = min(first["c", p, i] for i in range(3)) - CFG["scandue"] * p
            tasks.append([due, last["a", p, j] + lag, 1584, scan(p, j)])
            tasks.append([first["f", j, p], max(wait_at[f"kv{j}"], wait_at["rows"] + 4), 784, prep_kv(j, p)])
            tasks.append([first["f", j, p] + 8, wait_at[f"kv{j}"], 128, prep_filter(j, p)])
    for j in range(NJ):
        if j:
            tasks.append([first["a", 0, j], wait_at[f"b{(j + 1) // 2}"], 512, b_factors(j)])
        for i in range(3):
            due = min(first["c", p, n] for p in range(NP) for n in ((0,), (1,), (0, 1, 2))[i])
            tasks.append([due, wait_at["cb" if i == 1 else "ca"], 464 if i < 2 else 224, fold_c(j, i)])
        ready = max(last["f", j, p] for p in range(NP)) + lag
        for blocks, part in ([((0, 1), range(16)), ((2,), range(16)), ((3,), range(16))] if j == NJ - 1 else
                             [((0, 1, 2, 3), range(4 * i, 4 * i + 4)) for i in range(4)]):
            cost = len(part) * sum((48, 90, 112, 152)[a] for a in blocks) if j == NJ - 1 else 1632
            tasks.append([min(first["i", j, a] for a in blocks), ready, cost, products(j, blocks, part)])
    tasks.sort(key=lambda t_: t_[0])
    cum = [0.0]
    for n, (c, _) in enumerate(ops):
        quiet = any(n + ahead in waits for ahead in range(1, CFG["quiet"] + 1))
        cum.append(cum[-1] + (0.0 if quiet else max(CFG["rate"] - c, 0.0)))

    start_through("x0c")
    wait("par")
    start_through(CFG["ahead"]["par"])
    aid["never"] = jnp.full((8, 128), z_v[0], jnp.int32) != 0
    discretise()
    for key, task in (("b0", b_factors(0)), ("x0a", x_sums(0, (0,))), ("x0b", x_sums(0, (1,)))):
        wait(key)
        for _ in task:
            pass

    budget, back, later = 0.0, [], {}
    for n in range(0, len(ops), 4):
        for key in waits.get(n, ()):
            wait(key)
        for key in waits.get(n, ()):
            later.clear()
            start_through(CFG["ahead"].get(key))
        room = cum[n + 4] - cum[n]
        need = max([0.0] + [sum(t2[2] for t2 in tasks[:i + 1]) / max(cum[max(t_[0] - CFG["early"], 0)] - cum[n], room, 1)
                            for i, t_ in enumerate(tasks)])
        budget = min(budget, 0.0) + room * min(need, CFG["cap"])
        for kind, behind in (("product", CFG["holdlag"]), ("scan", CFG["scanlag"])):
            aid[kind] = back[-behind][-1] if len(back) >= behind else None
        steps = []
        for t_ in list(tasks):
            urgent = t_[0] < n + 4
            if t_[1] > n and not urgent:
                continue
            while budget > 0 or urgent:
                step = next(t_[3], None)
                if step is None:
                    tasks.remove(t_)
                    break
                if not urgent:
                    budget -= step[0]
                    t_[2] -= step[0]
                    steps.append((step[0], step[1][-2:], sum(step[2:])))
        total, acc = sum(t_[0] for t_ in steps), 0
        for i, (cost, vals, slack) in enumerate(steps):
            acc += cost
            later.setdefault(2 * n + CFG["gate"] + slack + int(8 * acc / (total + 1)), []).append((i % 4, vals))
        gates = [[[] for _ in range(8)] for _ in range(4)]
        for pos in range(8):
            for i, vals in later.pop(2 * n + pos, ()):
                gates[i][pos] += vals
        if len(back) >= CFG["natlag"]:
            for gate, val in zip(gates, back[-CFG["natlag"]]):
                gate[0].append(val)
        back.append([])
        for (_, op), gate in zip(ops[n:n + 4], gates):
            def tie(lhs, gate=gate):
                parts = [lhs[8 * i:8 * i + 8] for i in range(8)]
                for i, vals in enumerate(gate):
                    if vals:
                        both = functools.reduce(jnp.bitwise_or, [pltpu.bitcast(val, U32) for val in vals])
                        parts[i] = jnp.where(aid["never"], both, parts[i])
                return jnp.concatenate(parts, axis=0)

            out = op(tie)
            if out is not None:
                back[-1].append(out)
    assert not tasks and not queue
    for c in pending.values():
        c.wait()


@jax.jit
def pallas_concat_heads__ssm_conv_s5__ssm_conv_h3__prompt_kernel(
    A_x, A_Lambda_re, A_Lambda_im, A_B_re, A_B_im, A_C_re, A_C_im, A_log_dt, A_Dskip,
    B_q, B_k, B_v, B_shift_k, B_ssm_k, B_ssm_D,
):
    V = pltpu.VMEM
    scratch = [
        V((NJ, S, 128), BF16), V((NJ, S + HALO, 128), BF16), V((NJ, S, 128), BF16), V((NJ, S, 128), BF16),
        V((D, S), BF16), V((2, NJ, D, 128), BF16), V((2, NJ, D, 128), BF16),
        V((D,), BF16), V((D,), BF16), V((D,), BF16), V((D,), BF16), V((D,), BF16), V((4, D), BF16),
        V((2048, 128), BF16), pltpu.SMEM((1,), jnp.int32),
        V((NJ, 22, 8, 128), F32), V((2, 8, D), F32), V((6, 8, D), F32), V((4, T, 128), F32),
        V((NJ, S, 128), F32), V((NJ, S, 128), F32), V((16, 256, 128), F32),
        pltpu.SemaphoreType.DMA((NSEM,)),
    ]
    scratch += [V((10, 2, 128, 128), BF16)] * NP + [V((14, 128, 128), BF16)] * NJ
    scratch += [V((7, NJ, 128, 128), BF16)] * 3 + [V((7, NJ, T // 2, 128), BF16)] * NP
    scratch += [V((4, 128, 128), BF16)] * (2 * NP * NJ)
    scratch += [V((16, 256, 128), F32)] * (2 * NJ) + [V((NP, 4, 256, 128), BF16)] * NJ
    scratch += [V((2, S, 128), F32)] * NJ
    out = pl.pallas_call(
        _kernel,
        out_shape=jax.ShapeDtypeStruct((S, 2 * D), F32),
        in_specs=[pl.BlockSpec(memory_space=pl.ANY)] * 17,
        out_specs=pl.BlockSpec(memory_space=pl.ANY),
        scratch_shapes=scratch,
        compiler_params=pltpu.CompilerParams(vmem_limit_bytes=110 * 1024 * 1024),
        name="s5_h3",
    )(A_x.reshape(S, D), A_Lambda_re, A_Lambda_im, A_B_re, A_B_im, A_C_re, A_C_im, A_log_dt, A_Dskip,
      B_q.reshape(S, D), B_k.reshape(S, D), B_v.reshape(S, D), B_shift_k.T, B_ssm_k, B_ssm_D,
      jnp.asarray(_dft_tables()), jnp.asarray(np.zeros((1,), np.int32)))
    return out.reshape(1, S, 2 * D)
```
